```python
import jax
import jax.numpy as jnp

def _softmax(x, axis=-1):
    return jax.nn.softmax(x, axis=axis)

def _gelu(x):
    return jax.nn.gelu(x, approximate=True)

def _silu(x):
    return jax.nn.silu(x)

def _sigmoid(x):
    return jax.nn.sigmoid(x)

def _layernorm(x, axis=-1, eps=1e-05):
    m = jnp.mean(x, axis=axis, keepdims=True)
    v = jnp.var(x, axis=axis, keepdims=True)
    return (x - m) / jnp.sqrt(v + eps)

def _scatter_add(tgt, idx, src, axis=0):
    return tgt.at[idx].add(src)

def _segment_sum(src, seg, n):
    return jax.ops.segment_sum(src, seg, n)

class _Rng:

    def __init__(self, key):
        self._k = key

    def _next(self):
        self._k, sub = jax.random.split(self._k)
        return sub

    def normal(self, shape):
        return jax.random.normal(self._next(), shape, dtype=jnp.bfloat16)

    def randint(self, lo, hi, shape):
        return jax.random.randint(self._next(), shape, lo, hi, dtype=jnp.int32)

    def uniform(self, shape, lo=0.0, hi=1.0):
        return jax.random.uniform(self._next(), shape, jnp.bfloat16, lo, hi)

    def permutation(self, n):
        return jax.random.permutation(self._next(), n)
kernel_name = 'adaLN_cond__ssm_conv_h3__mixer_gmlp__prompt'

def setup_inputs():
    _rng = _Rng(jax.random.key(int.from_bytes(__import__("os").urandom(4), "little")))
    _w = lambda a: (lambda t: t.astype(jnp.bfloat16) if jnp.issubdtype(t.dtype, jnp.floating) else t)(jnp.asarray(a))

    def _A_setup():
        B, S, D = (1, 2048, 640)
        ks = 4
        return {'q': _w((lambda *s: _rng.normal(s) * 0.05)(B, S, D)), 'k': _w((lambda *s: _rng.normal(s) * 0.05)(B, S, D)), 'v': _w((lambda *s: _rng.normal(s) * 0.05)(B, S, D)), 'shift_k': _w((lambda *s: _rng.normal(s) * 0.05)(D, ks) * 0.5), 'ssm_k': _w((lambda *s: _rng.normal(s) * 0.05)(D, S) * (1.0 / S ** 0.5)), 'ssm_D': _w((lambda *s: _rng.normal(s) * 0.05)(D))}
    _A_in = _A_setup()

    def _B_setup():
        B, S, D, F = (1, 2048, 640, 1728)
        Fh = F // 2
        return {'x': _w((lambda *s: _rng.normal(s) * 0.05)(B, S, D)), 'w_in': _w((lambda *s: _rng.normal(s) * 0.05)(D, 2 * Fh)), 'w_sp': _w(0.01 * (lambda *s: _rng.normal(s) * 0.05)(S, S)), 'b_sp': _w(1.0 + 0.01 * (lambda *s: _rng.normal(s) * 0.05)(S)), 'w_out': _w((lambda *s: _rng.normal(s) * 0.05)(Fh, D))}
    _B_in = _B_setup()
    return {'A_q': _A_in['q'], 'A_k': _A_in['k'], 'A_v': _A_in['v'], 'A_shift_k': _A_in['shift_k'], 'A_ssm_k': _A_in['ssm_k'], 'A_ssm_D': _A_in['ssm_D'], 'B_x': _B_in['x'], 'B_w_in': _B_in['w_in'], 'B_w_sp': _B_in['w_sp'], 'B_b_sp': _B_in['b_sp'], 'B_w_out': _B_in['w_out'], 'c': _w((lambda *s: _rng.normal(s) * 0.05)(1, 640)), 'w_mod': _w((lambda *s: _rng.normal(s) * 0.05)(640, 6 * 640) * 640 ** (-0.5))}

def reference(A_q, A_k, A_v, A_shift_k, A_ssm_k, A_ssm_D, B_x, B_w_in, B_w_sp, B_b_sp, B_w_out, c, w_mod):

    def _A_ref(q, k, v, shift_k, ssm_k, ssm_D):
        B, S, D = q.shape
        ks = shift_k.shape[-1]
        k_pad = jnp.pad(k, ((0, 0), (ks - 1, 0), (0, 0)))
        k_shift = jnp.zeros_like(k)
        for t in range(ks):
            k_shift = k_shift + k_pad[:, t:t + S, :] * shift_k[:, ks - 1 - t][None, None, :]
        kv = k_shift * v
        L = 2 * S
        kv_pad = jnp.pad(kv, ((0, 0), (0, S), (0, 0)))
        kf_pad = jnp.pad(ssm_k, ((0, 0), (0, S)))
        kv_f = (lambda x, axes=(-2, -1): jnp.fft.rfft2(x.astype(jnp.float32), axes=axes))(kv_pad[:, None, :, :], axes=(1, 2))
        kf_f = (lambda x, axes=(-2, -1): jnp.fft.rfft2(x.astype(jnp.float32), axes=axes))(kf_pad[:, None, :], axes=(1, 2))
        kf_f = (lambda x, *d: x.transpose(*d))(kf_f, 1, 2, 0)
        y_f = kv_f * kf_f[None, :, :, :]
        y = (lambda x, s, axes=(-2, -1): jnp.fft.irfft2(x, s=s, axes=axes).astype(jnp.bfloat16))(y_f, (1, L), axes=(1, 2))[:, 0, :S, :]
        y = y + kv * ssm_D[None, None, :]
        return q * y

    def _B_ref(x, w_in, w_sp, b_sp, w_out):
        B, S, D = x.shape
        F = w_in.shape[-1]
        Fh = F // 2
        z = _gelu(jnp.einsum('bsd,df->bsf', x, w_in))
        z1 = z[..., :Fh].copy()
        z2 = _layernorm(z[..., Fh:], axis=-1)
        g = jnp.einsum('ts,bsf->btf', w_sp, z2) + b_sp[None, :, None]
        return jnp.einsum('bsf,fd->bsd', z1 * g, w_out)
    x = A_q
    mod = (_silu(c) @ w_mod).reshape(c.shape[0], 6, 1, -1)
    sa, ca, ga, sb, cb, gb = (mod[:, 0].copy(), mod[:, 1].copy(), mod[:, 2].copy(), mod[:, 3].copy(), mod[:, 4].copy(), mod[:, 5].copy())
    h = _layernorm(x, axis=-1) * (1 + ca) + sa
    x = x + ga * _A_ref(h, A_k, A_v, A_shift_k, A_ssm_k, A_ssm_D)
    h = _layernorm(x, axis=-1) * (1 + cb) + sb
    x = x + gb * _B_ref(h, B_w_in, B_w_sp, B_b_sp, B_w_out)
    return x
```

```python
import functools
import math

import numpy as np
import jax
import jax.numpy as jnp
from jax import lax
import jax.experimental.pallas as pl
import jax.experimental.pallas.tpu as pltpu

S, D, FH = 2048, 640, 864
CH = 512
NA = S // CH
N2 = 64
N1 = CH // N2
NCB = D // 128
EPS = 1e-5
F32, BF16 = jnp.float32, jnp.bfloat16

_C8 = math.cos(math.pi / 8)
_T8 = math.tan(math.pi / 8)
_R2 = math.sqrt(0.5)


def _dft_mats():
    ang = [1 / 16 + m / 4 for m in range(4)] + [1 / 8, 1 / 8 + 1 / 2, 1 / 4]
    idx = np.arange(128)
    pos = (idx // 16) * 8 + idx % 8
    part = (idx // 8) % 2
    mats = []
    for b, a in enumerate(ang):
        th = 2 * np.pi * (a + pos[:, None]) * pos[None, :] / N2
        po, pi = part[:, None], part[None, :]
        m = np.where(po == pi, np.cos(th), np.where(po == 1, np.sin(th), -np.sin(th)))
        mats.append(m * ((_C8 if b < 4 else 1.0) / 8))
    n = pos + 64 * part
    th = 2 * np.pi * pos[:, None] * n[None, :] / 128
    m = np.where(part[:, None] == 0, np.cos(th), np.sin(th))
    m[8, :] = 1.0 - 2.0 * (n % 2)
    mats.append(m / 8)
    return np.stack(mats).astype(np.float32)


def _outer_fwd(u):
    t0r, t0i = u[0] * (1 / _C8), u[4] * (1 / _C8)
    t2r, t2i = (u[2] - u[6]) * (_R2 / _C8), (u[2] + u[6]) * (_R2 / _C8)
    t1r, t1i = u[1] - _T8 * u[5], u[5] + _T8 * u[1]
    t3r, t3i = _T8 * u[3] - u[7], _T8 * u[7] + u[3]
    ar, ai, br, bi = t0r + t2r, t0i + t2i, t0r - t2r, t0i - t2i
    cr, ci, dr, di = t1r + t3r, t1i + t3i, t1r - t3r, t1i - t3i
    out = [(ar + cr, ai + ci), (br - di, bi + dr), (ar - cr, ai - ci), (br + di, bi - dr)]
    p = [u[j] + u[j + 4] for j in range(4)]
    q = [u[j] - u[j + 4] for j in range(4)]
    er, ei = (q[1] - q[3]) * _R2, (q[1] + q[3]) * _R2
    out += [(q[0] + er, q[2] + ei), (q[0] - er, q[2] - ei)]
    out += [(p[0] - p[2], p[1] - p[3]), (p[0] + p[2], p[1] + p[3])]
    return out


def _outer_inv(B):
    ar, ai = B[0][0] + B[2][0], B[0][1] + B[2][1]
    cr, ci = B[0][0] - B[2][0], B[0][1] - B[2][1]
    br, bi = B[1][0] + B[3][0], B[1][1] + B[3][1]
    dr, di = B[1][0] - B[3][0], B[1][1] - B[3][1]
    g0r, g0i, g2r, g2i = ar + br, ai + bi, ar - br, ai - bi
    g1r, g1i, g3r, g3i = cr + di, ci - dr, cr - di, ci + dr
    nr = [g0r * (1 / _C8), g1r + _T8 * g1i, (g2r + g2i) * (_R2 / _C8), _T8 * g3r + g3i]
    ni = [g0i * (1 / _C8), g1i - _T8 * g1r, (g2i - g2r) * (_R2 / _C8), _T8 * g3i - g3r]
    fr, fi = B[4][0] - B[5][0], B[4][1] - B[5][1]
    q = [B[4][0] + B[5][0], (fr + fi) * _R2, B[4][1] + B[5][1], (fi - fr) * _R2]
    p = [B[7][0] + B[6][0], B[7][1] + B[6][1], B[7][0] - B[6][0], B[7][1] - B[6][1]]
    return ([p[j] + q[j] + nr[j] for j in range(4)]
            + [p[j] - q[j] + ni[j] for j in range(4)])


def _gelu(x):
    c0 = math.sqrt(2 / math.pi)
    t = jnp.tanh(x * (c0 + (c0 * 0.044715) * (x * x)))
    hx = 0.5 * x
    return hx + hx * t


def _ln_rows(x):
    m = jnp.sum(x, axis=-1, keepdims=True) * (1.0 / x.shape[-1])
    d = x - m
    v = jnp.sum(d * d, axis=-1, keepdims=True) * (1.0 / x.shape[-1])
    return d * lax.rsqrt(v + EPS)


def _nt(a, b):
    return lax.dot_general(a, b, (((1,), (1,)), ((), ())), preferred_element_type=F32)


R1 = 512
R2 = 512


def _kernel(q_h, k_h, v_h, sh_h, sk_h, sd_h, wi_h, ws_h, b_h, wo_h, c_h, wm_h, vf_h, o_h,
            q_v, k_v, v_v, sh_v, sk_v, sd_v, wi_v, ws_v, b_v, wo_v, c_v, wm_v, vf_v,
            kf_v, au_v, bi_v, y_v, h_v, z1_v, z2_v, o_v, sems):
    copies = {}

    def start(name, src, dst):
        cp = pltpu.make_async_copy(src, dst, sems.at[len(copies)])
        cp.start()
        copies[name] = cp

    for cb in range(NCB):
        lanes = pl.ds(cb * 128, 128)
        start(("sk", cb), sk_h.at[lanes, :], sk_v.at[cb])
        if cb == 0:
            start("sd", sd_h, sd_v)
            start("sh", sh_h, sh_v)
        start(("k", cb), k_h.at[:, lanes], k_v.at[cb])
        start(("v", cb), v_h.at[:, lanes], v_v.at[cb])
        if cb == 0:
            start("vf", vf_h, vf_v)
    start("c", c_h, c_v)
    start("wm", wm_h.at[:, pl.ds(0, 5 * D)], wm_v.at[:, pl.ds(0, 5 * D)])
    start(("q", 0), q_h.at[pl.ds(0, R1)], q_v.at[pl.ds(0, R1)])
    start("wi", wi_h, wi_v)
    for i in range(1, S // R1):
        start(("q", i), q_h.at[pl.ds(i * R1, R1)], q_v.at[pl.ds(i * R1, R1)])
    start("wg", wm_h.at[:, pl.ds(5 * D, D)], wm_v.at[:, pl.ds(5 * D, D)])
    start("b", b_h, b_v)
    start("wo", wo_h, wo_v)
    for i in range(S // R2):
        start(("ws", i), ws_h.at[pl.ds(i * R2, R2)], ws_v.at[pl.ds(i * R2, R2)])

    kf_v[0:8, :] = jnp.zeros((8, 128), F32)
    row8 = lax.broadcasted_iota(jnp.int32, (8, 128), 0)

    def put(slot, a, g, res):
        for b in range(8):
            au_v[b, pl.ds(16 * g, 16), pl.ds((slot * NA + a) * 128, 128)] = (
                jnp.concatenate(res[b], axis=0).astype(BF16))

    def fwd(cb):
        lanes = pl.ds(cb * 128, 128)
        dskip = sd_v[...].astype(F32)[cb:cb + 1]
        for a in range(NA):
            kt = sk_v[cb, :, pl.ds(a * CH, CH)].T.astype(F32)
            for g in range(N2 // 8):
                u = [kt[j * N2 + 8 * g:j * N2 + 8 * g + 8] for j in range(N1)]
                if a == 0 and g == 0:
                    u[0] = u[0] + jnp.where(row8 == 0, dskip, 0.0)
                put(1, a, g, _outer_fwd(u))
        kf_v[pl.ds(8, S), :] = k_v[cb].astype(F32)
        w = [jnp.broadcast_to(sh_v[j:j + 1, lanes].astype(F32), (8, 128)) for j in range(4)]
        for a in range(NA):
            for g2 in range(N2 // 16):
                vv = [v_v[cb, pl.ds(a * CH + j * N2 + 16 * g2, 16), :].astype(F32) for j in range(N1)]
                for h in range(2):
                    u = []
                    for j in range(N1):
                        r = 8 + a * CH + j * N2 + 16 * g2 + 8 * h
                        ks = kf_v[pl.ds(r, 8), :] * w[0]
                        for t in range(1, 4):
                            ks = ks + kf_v[pl.ds(r - t, 8), :] * w[t]
                        u.append(ks * vv[j][8 * h:8 * h + 8])
                    put(0, a, 2 * g2 + h, _outer_fwd(u))

    def mid(cb):
        for b in range(8):
            f = jnp.dot(vf_v[b], au_v[b], preferred_element_type=F32)
            cols = [[] for _ in range(NA)]
            for g in range(8):
                def part(i, c):
                    return f[16 * g + 8 * c:16 * g + 8 * c + 8, 128 * i:128 * i + 128]
                ur = [part(a, 0) for a in range(NA)]
                ui = [part(a, 1) for a in range(NA)]
                kr = [part(NA + a, 0) for a in range(NA)]
                ki = [part(NA + a, 1) for a in range(NA)]
                if b < 4:
                    kr = [kr[0]] + [kr[a] - kr[a - 1] for a in range(1, NA)]
                    ki = [ki[0]] + [ki[a] - ki[a - 1] for a in range(1, NA)]
                else:
                    kr = [kr[0]] + [kr[a] + kr[a - 1] for a in range(1, NA)]
                    ki = [ki[0]] + [ki[a] + ki[a - 1] for a in range(1, NA)]
                for a in range(NA):
                    add = lambda xs: functools.reduce(lambda x, y: x + y, xs)
                    rr = add([kr[j] * ur[a - j] for j in range(a + 1)])
                    ii = add([ki[j] * ui[a - j] for j in range(a + 1)])
                    ri = add([kr[j] * ui[a - j] + ki[j] * ur[a - j] for j in range(a + 1)])
                    if b == 7 and g == 0:
                        yr = jnp.where(row8 == 0, 0.5 * rr, rr - ii)
                        yi = jnp.where(row8 == 0, 0.5 * ii, ri)
                    else:
                        yr, yi = rr - ii, ri
                    cols[a] += [yr, yi]
            yf = jnp.concatenate([jnp.concatenate(c, axis=0).astype(BF16) for c in cols], axis=1)
            bi_v[b] = jnp.dot(vf_v[8 + b], yf, preferred_element_type=F32)

    def inv(cb):
        for a in range(NA):
            for g in range(N2 // 8):
                res = [(bi_v[b, pl.ds(16 * g, 8), pl.ds(128 * a, 128)],
                        bi_v[b, pl.ds(16 * g + 8, 8), pl.ds(128 * a, 128)]) for b in range(8)]
                ys = _outer_inv(res)
                for j in range(N1):
                    y_v[pl.ds(a * CH + j * N2 + 8 * g, 8), pl.ds(cb * 128, 128)] = ys[j]

    copies["sd"].wait()
    copies["sh"].wait()
    for cb in range(NCB):
        copies[("sk", cb)].wait()
        copies[("k", cb)].wait()
        copies[("v", cb)].wait()
        fwd(cb)
        if cb == 0:
            copies["vf"].wait()
        mid(cb)
        inv(cb)

    copies["c"].wait()
    copies["wm"].wait()
    cc = c_v[...].astype(F32)
    sc = jnp.broadcast_to(cc / (1.0 + jnp.exp(-cc)), (16, D)).astype(BF16)
    mod = jnp.dot(sc, wm_v[:, pl.ds(0, 5 * D)], preferred_element_type=F32)[0:1]
    sa, ca, ga, sb, cb_ = (mod[:, i * D:(i + 1) * D] for i in range(5))
    m1, m0 = ga * (1.0 + ca), ga * sa
    cb1 = 1.0 + cb_

    copies["wi"].wait()

    for i in range(S // R1):
        copies[("q", i)].wait()
        rows = pl.ds(i * R1, R1)
        x = q_v[rows, :].astype(F32)
        x1 = x + (_ln_rows(x) * m1 + m0) * y_v[rows, :]
        y_v[rows, :] = x1
        h2 = (_ln_rows(x1) * cb1 + sb).astype(BF16)
        z2 = _gelu(_nt(wi_v[pl.ds(FH, FH), :], h2))
        m = jnp.sum(z2, axis=0, keepdims=True) * (1.0 / FH)
        d = z2 - m
        var = jnp.sum(d * d, axis=0, keepdims=True) * (1.0 / FH)
        z2_v[:, rows] = (d * lax.rsqrt(var + EPS)).astype(BF16)
        z1_v[:, rows] = _gelu(_nt(wi_v[pl.ds(0, FH), :], h2)).astype(BF16)

    copies["wg"].wait()
    copies["b"].wait()
    copies["wo"].wait()
    gb = jnp.dot(sc, wm_v[:, pl.ds(5 * D, D)], preferred_element_type=F32)[0:1]
    outs = []
    bf = b_v[...].astype(F32)
    for i in range(S // R2):
        copies[("ws", i)].wait()
        rows = pl.ds(i * R2, R2)
        bb = jnp.concatenate([bf[j:j + 1] for j in range(i * R2 // 128, (i + 1) * R2 // 128)], axis=1)
        g = _nt(z2_v[...], ws_v[rows, :]) + bb
        p = (z1_v[:, rows].astype(F32) * g).astype(BF16)
        o = lax.dot_general(p, wo_v[...], (((0,), (0,)), ((), ())), preferred_element_type=F32)
        o_v[rows, :] = (y_v[rows, :] + gb * o).astype(BF16)
        cp = pltpu.make_async_copy(o_v.at[rows], o_h.at[rows], sems.at[len(copies) + i])
        cp.start()
        outs.append(cp)
    for cp in outs:
        cp.wait()


@jax.jit
def pallas_adaLN_cond__ssm_conv_h3__mixer_gmlp__prompt_kernel(
    A_q, A_k, A_v, A_shift_k, A_ssm_k, A_ssm_D, B_x, B_w_in, B_w_sp, B_b_sp, B_w_out, c, w_mod,
):
    del B_x
    vf = _dft_mats()
    vf = np.concatenate([vf, vf.transpose(0, 2, 1)]).astype(BF16)
    vm = pltpu.VMEM
    scratch = [
        vm((S, D), BF16), vm((NCB, S, 128), BF16), vm((NCB, S, 128), BF16), vm((4, D), BF16),
        vm((NCB, 128, S), BF16), vm((NCB, 128), BF16), vm((2 * FH, D), BF16), vm((S, S), BF16),
        vm((S // 128, 128), BF16), vm((FH, D), BF16), vm((1, D), BF16), vm((D, 6 * D), BF16),
        vm((16, 128, 128), BF16),
        vm((S + 8, 128), F32), vm((8, 128, 2 * NA * 128), BF16), vm((8, 128, NA * 128), F32),
        vm((S, D), F32), vm((R1, D), BF16), vm((FH, S), BF16),
        vm((FH, S), BF16), vm((S, D), BF16),
        pltpu.SemaphoreType.DMA((48,)),
    ]
    out = pl.pallas_call(
        _kernel,
        out_shape=jax.ShapeDtypeStruct((S, D), BF16),
        in_specs=[pl.BlockSpec(memory_space=pltpu.HBM)] * 13,
        out_specs=pl.BlockSpec(memory_space=pltpu.HBM),
        scratch_shapes=scratch,
        compiler_params=pltpu.CompilerParams(vmem_limit_bytes=110 * 1024 * 1024),
    )(A_q.reshape(S, D), A_k.reshape(S, D), A_v.reshape(S, D), A_shift_k.T, A_ssm_k,
      A_ssm_D.reshape(NCB, 128), B_w_in.T, B_w_sp, B_b_sp.reshape(S // 128, 128), B_w_out, c, w_mod, vf)
    return out.reshape(1, S, D)
```

```python
import functools
import math

import numpy as np
import jax
import jax.numpy as jnp
from jax import lax
import jax.experimental.pallas as pl
import jax.experimental.pallas.tpu as pltpu

S, D, FH = 2048, 640, 864
FM = FH // 2
TAPS = 4
CH = 512
NA = S // CH
N2 = 64
N1 = CH // N2
NCB = D // 128
RB = 512
NB = S // RB
EPS = 1e-5
F32, BF16 = jnp.float32, jnp.bfloat16

_C8 = math.cos(math.pi / 8)
_T8 = math.tan(math.pi / 8)
_R2 = math.sqrt(0.5)
_G0 = math.sqrt(2 / math.pi)
_GA = (_G0 * 0.044715) ** (1 / 3)

TU = (-1, -1, 0, 4, 16, 32, 35, 38)
TK = (40, 41, 42, 43, 44, 45, 46, 47)
TI = (-1, -1, -1, -1, -1, -1, -1, -1, 0, 2, 4, 6, 16, 17, 32, 33, 34, 35, 36, 37, 38, 39, 40, 41)
P0, PS = 2, 12
G0, GS = 170, 6
G1, GT = 384, 6
SU = 48
HD = 256


def _dft_mats():
    ang = [1 / 16 + m / 4 for m in range(4)] + [1 / 8, 1 / 8 + 1 / 2, 1 / 4]
    idx = np.arange(128)
    pos = (idx // 16) * 8 + idx % 8
    part = (idx // 8) % 2
    mats = []
    for b, a in enumerate(ang):
        th = 2 * np.pi * (a + pos[:, None]) * pos[None, :] / N2
        po, pi = part[:, None], part[None, :]
        m = np.where(po == pi, np.cos(th), np.where(po == 1, np.sin(th), -np.sin(th)))
        mats.append(m * ((_C8 if b < 4 else 1.0) / 8))
    n = pos + 64 * part
    th = 2 * np.pi * pos[:, None] * n[None, :] / 128
    m = np.where(part[:, None] == 0, np.cos(th), np.sin(th))
    m[8, :] = 1.0 - 2.0 * (n % 2)
    mats.append(m / 8)
    return np.stack(mats).astype(np.float32)


def _outer_fwd(u):
    t0r, t0i = u[0] * (1 / _C8), u[4] * (1 / _C8)
    t2r, t2i = (u[2] - u[6]) * (_R2 / _C8), (u[2] + u[6]) * (_R2 / _C8)
    t1r, t1i = u[1] - _T8 * u[5], u[5] + _T8 * u[1]
    t3r, t3i = _T8 * u[3] - u[7], _T8 * u[7] + u[3]
    ar, ai, br, bi = t0r + t2r, t0i + t2i, t0r - t2r, t0i - t2i
    cr, ci, dr, di = t1r + t3r, t1i + t3i, t1r - t3r, t1i - t3i
    out = [(ar + cr, ai + ci), (br - di, bi + dr), (ar - cr, ai - ci), (br + di, bi - dr)]
    p = [u[j] + u[j + 4] for j in range(4)]
    q = [u[j] - u[j + 4] for j in range(4)]
    er, ei = (q[1] - q[3]) * _R2, (q[1] + q[3]) * _R2
    out += [(q[0] + er, q[2] + ei), (q[0] - er, q[2] - ei)]
    out += [(p[0] - p[2], p[1] - p[3]), (p[0] + p[2], p[1] + p[3])]
    return out


def _outer_inv(B):
    ar, ai = B[0][0] + B[2][0], B[0][1] + B[2][1]
    cr, ci = B[0][0] - B[2][0], B[0][1] - B[2][1]
    br, bi = B[1][0] + B[3][0], B[1][1] + B[3][1]
    dr, di = B[1][0] - B[3][0], B[1][1] - B[3][1]
    g0r, g0i, g2r, g2i = ar + br, ai + bi, ar - br, ai - bi
    g1r, g1i, g3r, g3i = cr + di, ci - dr, cr - di, ci + dr
    nr = [g0r * (1 / _C8), g1r + _T8 * g1i, (g2r + g2i) * (_R2 / _C8), _T8 * g3r + g3i]
    ni = [g0i * (1 / _C8), g1i - _T8 * g1r, (g2i - g2r) * (_R2 / _C8), _T8 * g3i - g3r]
    fr, fi = B[4][0] - B[5][0], B[4][1] - B[5][1]
    q = [B[4][0] + B[5][0], (fr + fi) * _R2, B[4][1] + B[5][1], (fi - fr) * _R2]
    p = [B[7][0] + B[6][0], B[7][1] + B[6][1], B[7][0] - B[6][0], B[7][1] - B[6][1]]
    return ([p[j] + q[j] + nr[j] for j in range(4)]
            + [p[j] - q[j] + ni[j] for j in range(4)])


def _gelu_scaled(x):
    t = jnp.tanh(x * (_G0 / _GA + x * x))
    return x + x * t


def _ln_rows(x):
    m = jnp.sum(x, axis=-1, keepdims=True) * (1.0 / x.shape[-1])
    d = x - m
    v = jnp.sum(d * d, axis=-1, keepdims=True) * (1.0 / x.shape[-1])
    return d * lax.rsqrt(v + EPS)


def _ld(ref, *idx):
    return pltpu.bitcast(ref.bitcast(jnp.uint32)[idx], BF16)


def _nn(a, b):
    return jnp.dot(a, b, preferred_element_type=F32)


def _nt(a, b):
    return lax.dot_general(a, b, (((1,), (1,)), ((), ())), preferred_element_type=F32)


def _ds(start, size, align):
    return pl.ds(start if isinstance(start, int) else pl.multiple_of(start, align), size)


def _add(xs):
    return functools.reduce(lambda x, y: x + y, xs)


def _kernel(q_h, k_h, v_h, sh_h, sk_h, sd_h, wi_h, ws_h, b_h, wo_h, c_h, wm_h, vf_h, o_h,
            q_v, k_v, v_v, sh_v, sk_v, sd_v, wi_v, ws_v, b_v, wo_v, c_v, wm_v, vf_v,
            kf_v, au0_v, au1_v, fa_v, fb_v, ya_v, yb_v, bm0_v, bp0_v, bm1_v, bp1_v,
            y_v, x1_v, h0_v, h1_v, z1_v, z2_v, bf_v, o_v, tie_v, zero_s,
            sems, osem, *lists):
    au_v, h_v, zf_v, ps_v = (au0_v, au1_v), (h0_v, h1_v), lists[:4], lists[4:]
    copies = {}

    def start(name, src, dst):
        copies[name] = pltpu.make_async_copy(src, dst, sems.at[NCB * NA + len(copies)])
        copies[name].start()

    def wait(*names):
        for name in names:
            copies[name].wait()

    def conv_inputs(cb, a):
        rows, lanes, sem = _ds(a * CH, CH, CH), pl.ds(cb * 128, 128), sems.at[cb * NA + a]
        return (pltpu.make_async_copy(k_h.at[rows, lanes], k_v.at[cb, rows], sem),
                pltpu.make_async_copy(v_h.at[rows, lanes], v_v.at[cb, rows], sem),
                pltpu.make_async_copy(sk_h.at[lanes, rows], sk_v.at[cb, a], sem))

    def fetch(stage):
        if stage < NCB:
            for a in range(NA):
                for cp in conv_inputs(stage, a):
                    cp.start()
        if stage == 0:
            start("vf", vf_h, vf_v)
        if stage == NCB:
            start("c", c_h, c_v)
            start("wm", wm_h.at[:, pl.ds(0, 5 * D)], wm_v.at[:, pl.ds(0, 5 * D)])
            start("q0", q_h.at[pl.ds(0, HD)], q_v.at[pl.ds(0, HD)])
            start("w2", wi_h.at[pl.ds(FH, FH)], wi_v.at[pl.ds(0, FH)])
            if HD < RB:
                start("q1", q_h.at[pl.ds(HD, RB - HD)], q_v.at[pl.ds(HD, RB - HD)])
            start("w1", wi_h.at[pl.ds(0, FH)], wi_v.at[pl.ds(FH, FH)])
            start("q2", q_h.at[pl.ds(RB, S - RB)], q_v.at[pl.ds(RB, S - RB)])
        if stage == NCB + 2:
            start("wg", wm_h.at[:, pl.ds(5 * D, D)], wm_v.at[:, pl.ds(5 * D, D)])
            start("b", b_h, b_v)
            start("wo", wo_h, wo_v)
            for j in range(S // 128):
                start(("ws", j), ws_h.at[:, pl.ds(128 * j, 128)], ws_v.at[j])

    start("sh", sh_h, sh_v)
    start("sd", sd_h, sd_v)
    fetch(0)
    fetch(1)
    for ref in (fb_v, ya_v, tie_v):
        ref[...] = jnp.zeros(ref.shape, ref.dtype)
    kf_v[CH:CH + 8, :] = jnp.zeros((8, 128), F32)
    zero_s[0] = 0
    row8 = lax.broadcasted_iota(jnp.int32, (8, 128), 0)

    def tie(after, x):
        if after is None:
            return x
        never = jnp.concatenate([tie_v[...]] * (x.shape[0] // 8), axis=0) != 0
        return jnp.where(never, after, x)

    def put(cb, slot, g, res):
        for b in range(8):
            au_v[cb % 2][b, slot, pl.ds(16 * g, 16), :] = jnp.concatenate(res[b], axis=0).astype(BF16)

    def split_filter(cb, a, after):
        kt = sk_v[cb, a].T.astype(F32)
        for g in range(N2 // 8):
            u = [kt[j * N2 + 8 * g:j * N2 + 8 * g + 8] for j in range(N1)]
            if g == 0:
                u[0] = u[0] + jnp.where(row8 + a == 0, sd_v[...].astype(F32)[cb:cb + 1], 0.0)
            u[:4] = [tie(after(g), x) for x in u[:4]]
            put(cb, NA + a, g, _outer_fwd(u))

    def split_signal(cb, a, after):
        kf_v[0:8, :] = jnp.where(a == 0, 0.0, kf_v[CH:CH + 8, :])
        kf_v[pl.ds(8, CH), :] = k_v[cb, _ds(a * CH, CH, CH), :].astype(F32)
        taps = [jnp.broadcast_to(sh_v[j:j + 1, pl.ds(cb * 128, 128)].astype(F32), (8, 128))
                for j in range(TAPS)]
        for g2 in range(N2 // 16):
            vv = [v_v[cb, _ds(a * CH + j * N2 + 16 * g2, 16, 16), :].astype(F32) for j in range(N1)]
            for g in (2 * g2, 2 * g2 + 1):
                w = [tie(after(g), t) for t in taps]
                u = [_add([kf_v[pl.ds(8 + j * N2 + 8 * g - t, 8), :] * w[t] for t in range(TAPS)])
                     * vv[j][8 * (g % 2):8 * (g % 2) + 8] for j in range(N1)]
                put(cb, a, g, _outer_fwd(u))

    def spectra(cb, b, half, f_ref):
        rhs = jnp.concatenate([_ld(au_v[cb % 2], b, half * NA + a) for a in range(NA)], axis=1)
        f = _nn(_ld(vf_v, b), rhs)
        for a in range(NA):
            f_ref[half * NA + a] = f[:, 128 * a:128 * a + 128]
        return f

    def product(f_ref, y_ref, plus, real_rows=None):
        for g in range(8):
            ur, ui, kr, ki = ([f_ref[o + a, pl.ds(16 * g + 8 * c, 8), :] for a in range(NA)]
                              for o in (0, NA) for c in (0, 1))
            kr, ki = ([k[0]] + [k[a] + k[a - 1] if plus else k[a] - k[a - 1] for a in range(1, NA)]
                      for k in (kr, ki))
            for a in range(NA):
                yi = _add([kr[j] * ui[a - j] + ki[j] * ur[a - j] for j in range(a + 1)])
                if real_rows is not None and g == 0:
                    rr = _add([kr[j] * ur[a - j] for j in range(a + 1)])
                    ii = _add([ki[j] * ui[a - j] for j in range(a + 1)])
                    yr = jnp.where(real_rows, 0.5 * rr, rr - ii)
                    yi = jnp.where(real_rows, 0.5 * ii, yi)
                else:
                    yr = _add([kr[j] * ur[a - j] - ki[j] * ui[a - j] for j in range(a + 1)])
                y_ref[a, pl.ds(16 * g, 16), :] = jnp.concatenate([yr, yi], axis=0).astype(BF16)

    def residues(y_ref, b, dst):
        r = _nn(_ld(vf_v, 8 + b), jnp.concatenate([_ld(y_ref, a) for a in range(NA)], axis=1))
        for a in range(NA):
            dst[a] = r[:, 128 * a:128 * a + 128]
        return r

    def stash(t):
        return ((bm0_v.at[t], bp0_v.at[t]) if t < 16 else (bm1_v.at[t - 16], bp1_v.at[t - 16]))

    def merge(cb, a, after=lambda g: None):
        src = [stash(1 + 4 * cb + b)[s] for s in (0, 1) for b in range(4)]
        for g in range(N2 // 8):
            res = [[ref[a, pl.ds(16 * g + 8 * c, 8), :] for c in (0, 1)] for ref in src]
            res[0] = [tie(after(g), x) for x in res[0]]
            res[1] = [tie(after(g), x) for x in res[1]]
            for j, y in enumerate(_outer_inv(res)):
                y_v[cb, _ds(a * CH + j * N2 + 8 * g, 8, 8), :] = y

    def transform(cb, a, dst, active=True):
        pa = (a + 3) % 4
        res = []
        if active:
            res += [spectra(cb, a, 1, fa_v), spectra(cb, a, 0, fa_v)]
        product(fb_v, yb_v, True, row8 + (3 - pa) == 0)
        res.append(residues(ya_v, pa, dst[0]))
        if active:
            res += [spectra(cb, 4 + a, 1, fb_v), spectra(cb, 4 + a, 0, fb_v)]
            product(fa_v, ya_v, False)
        res.append(residues(yb_v, 4 + pa, dst[1]))
        return lambda p: None if p < 0 else res[p // 8][16 * (p % 8):16 * (p % 8) + 8, 0:128]

    def conv_step(cb, a):
        if cb < NCB:
            for cp in conv_inputs(cb, a):
                cp.wait()
        at = lambda p: None
        if 0 < cb < NCB:
            at = transform(cb - 1, a, (bm0_v.at[4 * cb - 4 + a], bp0_v.at[4 * cb - 4 + a]))
        if cb < NCB:
            split_signal(cb, a, lambda g: at(TU[g]))
            split_filter(cb, a, lambda g: at(TK[g]))
        else:
            at = transform(cb - 1, a, (bm1_v.at[a], bp1_v.at[a]))
            for c in range(3):
                merge(c, a, lambda g: at(TI[8 * c + g]))

    wait("sh", "sd")
    for cb in range(NCB + 1):
        if cb == 1:
            wait("vf")
        fetch(cb + 2)
        pl.loop(0, NA)(functools.partial(conv_step, cb))

    wait("c", "wm")
    transform(NCB, 0, stash(20), active=False)
    cc = c_v[...].astype(F32)
    sc = jnp.broadcast_to(cc / (1.0 + jnp.exp(-cc)), (16, D)).astype(BF16)
    mod = _nn(sc, wm_v[:, pl.ds(0, 5 * D)])
    sa, ca, ga, sb, cb_ = (mod[:, i * D:(i + 1) * D] for i in range(5))
    m1, m0 = ga * (1.0 + ca), ga * sa
    n1, n0 = _GA * (1.0 + cb_), _GA * sb
    zero = zero_s[0]
    for cb in (3, 4):
        for a in range(NA):
            merge(cb, a + zero)

    TB = RB // 128
    PER = 2 * FH // 16

    def hidden(r, after=None):
        rows = _ds(r, 16, 16)
        x = q_v[rows, :].astype(F32)
        x = jnp.concatenate([tie(after, x[:, :128]), x[:, 128:]], axis=1)
        x1 = x + (_ln_rows(x) * m1 + m0) * jnp.concatenate([y_v[j, rows, :] for j in range(NCB)], axis=1)
        x1_v[rows, :] = x1
        return _ln_rows(x1) * n1 + n0

    def keep_hidden(h_ref, r, h):
        for j in range(NCB):
            h_ref[j, _ds(r, 16, 16), :] = h[:, 128 * j:128 * j + 128].astype(BF16)

    def act(h_ref, f0, n, extra=()):
        h = jnp.concatenate([_ld(h_ref, j, pl.ds(0, (RB - 16 * len(extra)) // 2)) for j in range(NCB)], axis=1)
        if extra:
            h = jnp.concatenate([h, jnp.concatenate(extra, axis=0).astype(BF16)], axis=0)
        return _gelu_scaled(_nt(wi_v[pl.ds(f0, n), :], h))

    def keep_gate(z2, zero):
        stats = []
        for t in range(TB):
            z = z2[:, 128 * t:128 * t + 128]
            zf_v[t][pl.ds(zero, FH), :] = z
            c = jnp.broadcast_to(jnp.sum(z[0:8], axis=0, keepdims=True) * 0.125, (8, 128))
            s1 = s2 = None
            for n, f in enumerate(range(0, FH, SU)):
                for r in range(f, f + SU, 8):
                    d = z[r:r + 8] - c
                    s1, s2 = (d, d * d) if s1 is None else (s1 + d, s2 + d * d)
                ps_v[t][pl.ds(16 * n + zero, 16), :] = jnp.concatenate([s1, s2], axis=0)
            m = jnp.sum(ps_v[t][pl.ds(16 * n, 8), :], axis=0, keepdims=True) * (1.0 / FH)
            var = jnp.sum(ps_v[t][pl.ds(16 * n + 8, 8), :], axis=0, keepdims=True) * (1.0 / FH) - m * m
            rstd = lax.rsqrt(jnp.maximum(var, 0.0) + EPS * (2 * _GA) ** 2)
            stats.append((jnp.broadcast_to(m + c[0:1], (16, 128)), jnp.broadcast_to(rstd, (16, 128))))
        return stats

    def norm_gate(i, pair, stats, after):
        for n, f in enumerate(range(0, FM, 16)):
            means = [tie(after(n), stats[2 * pair + c][0]) for c in (0, 1)]
            a11, a12, a21, a22 = [
                (zf_v[2 * pair + c][pl.ds(r + f, 16), :] - means[c]) * stats[2 * pair + c][1]
                for r in (0, FM) for c in (0, 1)]
            for k, a in enumerate((a11 + a22, a21 + a22, a11, a22, a11 + a12, a21 - a11, a12 - a22)):
                z2_v[k, 2 * i + pair, pl.ds(f, 16), :] = a.astype(BF16)

    def keep_value(i, z1):
        for t in range(TB):
            z1_v[i * TB + t] = z1[:, 128 * t:128 * t + 128].astype(BF16)

    def rows_of(z):
        per = z.shape[0] // 16
        return lambda p: z[16 * (p % per):16 * (p % per) + 16, 128 * (p // per):128 * (p // per) + 128]

    wait("q0")
    for r in range(0, HD, 16):
        keep_hidden(h0_v, r, hidden(r))
    wait("w2")
    if HD < RB:
        wait("q1")
    zero = pl.multiple_of(zero_s[0], 16)
    extra = [hidden(r) for r in range(HD, RB, 16)]
    for n, h in enumerate(extra):
        keep_hidden(h0_v, HD + 16 * n, h)
    stats = keep_gate(act(h0_v, 0, FH, extra), zero)
    wait("w1", "q2")
    z = act(h0_v, FH, FH)
    at = rows_of(z)
    keep_value(0, z)
    for pair in (0, 1):
        norm_gate(0, pair, stats, lambda n: at(2 + 2 * (27 * pair + n)))
    for n in range(RB // 16):
        keep_hidden(h1_v, 16 * n + zero, hidden(RB + 16 * n, at(n * 5)))
    for i in range(1, NB):
        z = act(h_v[i % 2], 0, 2 * FH)
        at = rows_of(z)
        keep_value(i, z[FH:])
        stats = keep_gate(z[:FH], zero)
        norm_gate(i, 0, stats, lambda n: at(G0 + n * GS))
        norm_gate(i, 1, stats, lambda n: at(G1 + (n * GT) // 4))
        if i + 1 < NB:
            for n in range(RB // 16):
                keep_hidden(h_v[(i + 1) % 2], 16 * n + zero,
                            hidden((i + 1) * RB + 16 * n, at(P0 + n * PS)))

    wait("wg", "b", "wo", *[("ws", j) for j in range(S // 128)])
    gb = _nn(sc, wm_v[:, pl.ds(5 * D, D)]) * (0.5 / _GA)
    bf_v[...] = b_v[...].astype(F32)
    H = RB // 2

    def mix(i):
        def w(c, r):
            return [_ld(ws_v, 2 * j + c, _ds((i * RB + r * H) // 2, H // 2, H // 2)) for j in range(S // 256)]

        def comb(x, y, sign):
            return [(a.astype(F32) + b.astype(F32) if sign > 0 else a.astype(F32) - b.astype(F32)).astype(BF16)
                    for a, b in zip(x, y)]

        def prod(n, rhs):
            lhs = jnp.concatenate([_ld(z2_v, n, j) for j in range(S // 256)], axis=1)
            return _nt(lhs, jnp.concatenate(rhs, axis=1))

        def gate(r, c, g):
            tiles = [i * TB + c * (H // 128) + t for t in range(H // 128)]
            bias = jnp.concatenate([bf_v[pl.ds(j, 1), :] for j in tiles], axis=1)
            z1 = jnp.concatenate([z1_v[j, pl.ds(FM * r, FM), :] for j in tiles], axis=1).astype(F32)
            return z1 * (g + bias)

        s2 = prod(1, w(0, 0))
        s5 = prod(4, w(1, 1))
        s4 = prod(3, comb(w(1, 0), w(0, 0), -1))
        p21 = gate(1, 0, s2 + s4)
        d11 = s4 - s5
        s1 = prod(0, comb(w(0, 0), w(1, 1), 1))
        d11, d22 = d11 + s1, s1 - s2
        p11 = gate(0, 0, d11 + prod(6, comb(w(1, 0), w(1, 1), 1)))
        s3 = prod(2, comb(w(0, 1), w(1, 1), -1))
        p12 = gate(0, 1, s3 + s5)
        p22 = gate(1, 1, (d22 + s3) + prod(5, comb(w(0, 0), w(0, 1), 1)))
        return [jnp.concatenate(p, axis=0).astype(BF16) for p in ((p11, p21), (p12, p22))]

    def flush(k):
        rows = _ds(k * H, H, H)
        return pltpu.make_async_copy(o_v.at[rows], o_h.at[rows], osem.at[k])

    def mix_step(i):
        for c, p in enumerate(mix(i)):
            rows = _ds(i * RB + c * H, H, H)
            o = lax.dot_general(p, wo_v[...], (((0,), (0,)), ((), ())), preferred_element_type=F32)
            o_v[rows, :] = (x1_v[rows, :] + jnp.concatenate([gb] * (H // 16), axis=0) * o).astype(BF16)
            flush(2 * i + c).start()

    pl.loop(0, NB)(mix_step)
    for k in range(2 * NB):
        flush(k).wait()


@jax.jit
def pallas_adaLN_cond__ssm_conv_h3__mixer_gmlp__prompt_kernel(
    A_q, A_k, A_v, A_shift_k, A_ssm_k, A_ssm_D, B_x, B_w_in, B_w_sp, B_b_sp, B_w_out, c, w_mod,
):
    del B_x
    vf = _dft_mats()
    vf = np.concatenate([vf, vf.transpose(0, 2, 1)]).astype(BF16)
    vm = pltpu.VMEM
    tile = (128, 128)
    scratch = [
        vm((S, D), BF16), vm((NCB, S, 128), BF16), vm((NCB, S, 128), BF16), vm((TAPS, D), BF16),
        vm((NCB, NA, 128, CH), BF16), vm((NCB, 128), BF16), vm((2 * FH, D), BF16),
        vm((S // 128, S, 128), BF16), vm((S // 128, 128), BF16), vm((FH, D), BF16), vm((1, D), BF16),
        vm((D, 6 * D), BF16), vm((16, *tile), BF16),
        vm((CH + 8, 128), F32), vm((8, 2 * NA, *tile), BF16), vm((8, 2 * NA, *tile), BF16),
        vm((2 * NA, *tile), F32), vm((2 * NA, *tile), F32), vm((NA, *tile), BF16), vm((NA, *tile), BF16),
        vm((16, NA, *tile), F32), vm((16, NA, *tile), F32), vm((5, NA, *tile), F32), vm((5, NA, *tile), F32),
        vm((NCB, S, 128), F32), vm((S, D), F32), vm((NCB, RB, 128), BF16), vm((NCB, RB, 128), BF16),
        vm((S // 128, FH, 128), BF16), vm((7, S // 256, FM, 128), BF16), vm((S // 128, 128), F32),
        vm((S, D), BF16), vm((8, 128), jnp.int32), pltpu.SMEM((1,), jnp.int32),
        pltpu.SemaphoreType.DMA((NCB * NA + 32,)),
        pltpu.SemaphoreType.DMA((2 * NB,)),
    ] + [vm((FH, 128), F32)] * 4 + [vm((FH // SU * 16, 128), F32)] * 4
    out = pl.pallas_call(
        _kernel,
        out_shape=jax.ShapeDtypeStruct((S, D), BF16),
        in_specs=[pl.BlockSpec(memory_space=pltpu.HBM)] * 13,
        out_specs=pl.BlockSpec(memory_space=pltpu.HBM),
        scratch_shapes=scratch,
        compiler_params=pltpu.CompilerParams(vmem_limit_bytes=110 * 1024 * 1024),
    )(A_q.reshape(S, D), A_k.reshape(S, D), A_v.reshape(S, D), A_shift_k.T, A_ssm_k,
      A_ssm_D.reshape(NCB, 128), B_w_in.T, B_w_sp, B_b_sp.reshape(S // 128, 128), B_w_out, c, w_mod, vf)
    return out.reshape(1, S, D)
```

```python
import functools
import math

import numpy as np
import jax
import jax.numpy as jnp
from jax import lax
import jax.experimental.pallas as pl
import jax.experimental.pallas.tpu as pltpu

S, D, FH = 2048, 640, 864
FM, DM = FH // 2, D // 2
KO = FH // 256
FT, FB = 224, 208
TAPS = 4
CH = 512
NA = S // CH
N2 = 64
N1 = CH // N2
NCB = D // 128
RB = 512
NB = S // RB
H = RB // 2
EPS = 1e-5
F32, BF16, U32 = jnp.float32, jnp.bfloat16, jnp.uint32
PAD = 16

_C8 = math.cos(math.pi / 8)
_T8 = math.tan(math.pi / 8)
_R2 = math.sqrt(0.5)
_G0 = math.sqrt(2 / math.pi)
_GA = (_G0 * 0.044715) ** (1 / 3)

UN = 1
MA = 2
MS = 22
TU = (-1, 0, 3, 5, 16, 32, 35, 38)
TK = (34, 38, 41, 42, 43, 44, 45, 46)
TI = (-1, -1, -1, -1, -1, -1, -1, -1, 0, 2, 4, 6, 16, 17, 32, 33, 34, 35, 36, 37, 38, 39, 40, 41)
SU = 96
NJ = ["s0:76:105,s1:114:160,s2:168:205,m14:4:54,m18:54:108,m15:108:160,m19:144:189", "h3:0:89,h2:95:195",
      "h5:0:95:162:216,h4:216:258:324:440",
      "h7:0:108:162:216,h6:222:276:324:470,s3:54:108,s6:216:270,s7:270:372",
      "n0:0:40,s4:20:50,s5:50:80,n1:40:80,n3:80:108:162:180,s8:162:190,s9:190:216,n2:180:222,s10:200:240,s11:240:270,n4:216:250,n5:280:340,s14:200:230,s15:200:230,n7:250:270:340:370,s12:326:350,s13:350:378,n6:390:470"]
R2 = 512
FL = 256
UR = 0


def _dft_mats():
    ang = [1 / 16 + m / 4 for m in range(4)] + [1 / 8, 1 / 8 + 1 / 2, 1 / 4]
    idx = np.arange(128)
    pos = (idx // 16) * 8 + idx % 8
    part = (idx // 8) % 2
    mats = []
    for b, a in enumerate(ang):
        th = 2 * np.pi * (a + pos[:, None]) * pos[None, :] / N2
        po, pi = part[:, None], part[None, :]
        m = np.where(po == pi, np.cos(th), np.where(po == 1, np.sin(th), -np.sin(th)))
        mats.append(m * ((_C8 if b < 4 else 1.0) / 8))
    n = pos + 64 * part
    th = 2 * np.pi * pos[:, None] * n[None, :] / 128
    m = np.where(part[:, None] == 0, np.cos(th), np.sin(th))
    m[8, :] = 1.0 - 2.0 * (n % 2)
    mats.append(m / 8)
    fwd = np.stack(mats).astype(np.float32)
    n = idx // 32 * 16 + idx % 8 * 2 + idx // 16 % 2
    return np.concatenate([fwd[:, :, n // 8 * 16 + part * 8 + n % 8], fwd.transpose(0, 2, 1)])


def _outer_fwd(u):
    t0r, t0i = u[0] * (1 / _C8), u[4] * (1 / _C8)
    t2r, t2i = (u[2] - u[6]) * (_R2 / _C8), (u[2] + u[6]) * (_R2 / _C8)
    t1r, t1i = u[1] - _T8 * u[5], u[5] + _T8 * u[1]
    t3r, t3i = _T8 * u[3] - u[7], _T8 * u[7] + u[3]
    ar, ai, br, bi = t0r + t2r, t0i + t2i, t0r - t2r, t0i - t2i
    cr, ci, dr, di = t1r + t3r, t1i + t3i, t1r - t3r, t1i - t3i
    out = [(ar + cr, ai + ci), (br - di, bi + dr), (ar - cr, ai - ci), (br + di, bi - dr)]
    p = [u[j] + u[j + 4] for j in range(4)]
    q = [u[j] - u[j + 4] for j in range(4)]
    er, ei = (q[1] - q[3]) * _R2, (q[1] + q[3]) * _R2
    out += [(q[0] + er, q[2] + ei), (q[0] - er, q[2] - ei)]
    out += [(p[0] - p[2], p[1] - p[3]), (p[0] + p[2], p[1] + p[3])]
    return out


def _outer_inv(B):
    ar, ai = B[0][0] + B[2][0], B[0][1] + B[2][1]
    cr, ci = B[0][0] - B[2][0], B[0][1] - B[2][1]
    br, bi = B[1][0] + B[3][0], B[1][1] + B[3][1]
    dr, di = B[1][0] - B[3][0], B[1][1] - B[3][1]
    g0r, g0i, g2r, g2i = ar + br, ai + bi, ar - br, ai - bi
    g1r, g1i, g3r, g3i = cr + di, ci - dr, cr - di, ci + dr
    nr = [g0r * (1 / _C8), g1r + _T8 * g1i, (g2r + g2i) * (_R2 / _C8), _T8 * g3r + g3i]
    ni = [g0i * (1 / _C8), g1i - _T8 * g1r, (g2i - g2r) * (_R2 / _C8), _T8 * g3i - g3r]
    fr, fi = B[4][0] - B[5][0], B[4][1] - B[5][1]
    q = [B[4][0] + B[5][0], (fr + fi) * _R2, B[4][1] + B[5][1], (fi - fr) * _R2]
    p = [B[7][0] + B[6][0], B[7][1] + B[6][1], B[7][0] - B[6][0], B[7][1] - B[6][1]]
    return ([p[j] + q[j] + nr[j] for j in range(4)]
            + [p[j] - q[j] + ni[j] for j in range(4)])


def _gelu_scaled(x):
    t = jnp.tanh(x * (_G0 / _GA + x * x))
    return x + x * t


def _norm_stats(s1, s2, n, eps):
    m = s1 * (1.0 / n)
    return m, jnp.exp(-0.5 * jnp.log(jnp.maximum(s2 * (1.0 / n) - m * m, 0.0) + eps))


def _ln_rows(x):
    m, r = _norm_stats(jnp.sum(x, axis=-1, keepdims=True), jnp.sum(x * x, axis=-1, keepdims=True),
                       x.shape[-1], EPS)
    return (x - m) * r


def _lhs7(a11, a12, a21, a22):
    return a11 + a22, a21 + a22, a11, a22, a11 + a12, a21 - a11, a12 - a22


def _ld(ref, *idx):
    return pltpu.bitcast(ref.bitcast(jnp.uint32)[idx or ...], BF16)


def _whole(x):
    return x


def _phase(words, odd):
    return pltpu.bitcast(words & np.uint32(0xFFFF0000) if odd else words << 16, F32)


def _nn(a, b):
    return jnp.dot(a, b, preferred_element_type=F32)


def _nt(a, b):
    return lax.dot_general(a, b, (((1,), (1,)), ((), ())), preferred_element_type=F32)


def _ds(start, size, align):
    return pl.ds(start if isinstance(start, int) else pl.multiple_of(start, align), size)


def _add(xs):
    return functools.reduce(lambda x, y: x + y, xs)


def _kernel(q_h, k_h, v_h, sh_h, sk_h, sd_h, wi_h, ws_h, b_h, wo_h, c_h, wm_h, vf_h, o_h,
            q_v, k_v, v_v, sh_v, sk_v, sd_v, wi_v, ws_v, b_v, wo_v, c_v, wm_v, vf_v,
            au0_v, au1_v, fa_v, fb_v, ya_v, yb_v, bm0_v, bp0_v, bm1_v, bp1_v,
            y_v, x1_v, h0_v, z1_v, z2_v, wt_v, wr_v, bf_v, o_v, tie_v, zero_s,
            sems, osem, *lists):
    au_v, h_v = (au0_v, au1_v), (lists[32:41], lists[41:])
    copies = {}

    def start(name, src, dst):
        copies[name] = pltpu.make_async_copy(src, dst, sems.at[NCB * NA + len(copies)])
        copies[name].start()

    def wait(*names):
        for name in names:
            copies[name].wait()

    def conv_inputs(cb, a):
        rows, lanes, sem = _ds(a * CH, CH, CH), pl.ds(cb * 128, 128), sems.at[cb * NA + a]
        return (pltpu.make_async_copy(k_h.at[rows, lanes], k_v.at[cb, _ds(PAD + a * CH, CH, PAD)], sem),
                pltpu.make_async_copy(v_h.at[rows, lanes], v_v.at[cb, rows], sem),
                pltpu.make_async_copy(sk_h.at[lanes, rows], sk_v.at[cb, a], sem))

    def mixing(i):
        return pltpu.make_async_copy(ws_h.at[_ds(i * R2, R2, R2)], ws_v.at[i % 2], sems.at[NCB * NA + 16 + i])

    def fetch(stage):
        if stage < NCB:
            for a in range(NA):
                for cp in conv_inputs(stage, a):
                    cp.start()
        if stage == 0:
            start("vf", vf_h, vf_v)
        if stage == NCB:
            start("c", c_h, c_v)
            start("wm", wm_h.at[:, pl.ds(0, 5 * D)], wm_v.at[:, pl.ds(0, 5 * D)])
            start("q0", q_h.at[pl.ds(0, H)], q_v.at[pl.ds(0, H)])
            start("w2", wi_h.at[pl.ds(FH, FH)], wi_v.at[pl.ds(0, FH)])
            start("q1", q_h.at[pl.ds(H, RB - H)], q_v.at[pl.ds(H, RB - H)])
            start("w1", wi_h.at[pl.ds(0, FH)], wi_v.at[pl.ds(FH, FH)])
            start("q2", q_h.at[pl.ds(RB, S - RB)], q_v.at[pl.ds(RB, S - RB)])
        if stage == NCB + 2:
            start("wg", wm_h.at[:, pl.ds(5 * D, D)], wm_v.at[:, pl.ds(5 * D, D)])
            start("b", b_h, b_v)
            start("wo", wo_h, wo_v.at[pl.ds(0, FH)])
            mixing(0).start()

    start("sh", sh_h, sh_v)
    start("sd", sd_h, sd_v)
    fetch(0)
    fetch(1)
    for ref in (fb_v, ya_v, tie_v):
        ref[...] = jnp.zeros(ref.shape, ref.dtype)
    k_v[:, pl.ds(0, PAD), :] = jnp.zeros((NCB, PAD, 128), BF16)
    wo_v[pl.ds(FH, 256 * KO + 128 - FH), :] = jnp.zeros((256 * KO + 128 - FH, D), BF16)
    zero_s[0] = 0
    row8 = lax.broadcasted_iota(jnp.int32, (8, 128), 0)

    def tie(after, x):
        if after is None:
            return x
        never = jnp.concatenate([tie_v[...]] * (x.shape[0] // 8), axis=0) != 0
        return jnp.where(never, after, x)

    def put(cb, slot, g, res):
        for b in range(8):
            au_v[cb % 2][b, slot, pl.ds(16 * g, 16), :] = jnp.concatenate(res[b], axis=0).astype(BF16)

    def split_filter(cb, a, after):
        kt = pltpu.bitcast(sk_v[cb, a].T, U32)
        for g in range(N2 // 8):
            u = [_phase(kt[j * N2 // 2 + g // 2 * 8:j * N2 // 2 + g // 2 * 8 + 8], g % 2) for j in range(N1)]
            if g == 0:
                u[0] = u[0] + jnp.where(row8 + a == 0, sd_v[...].astype(F32)[cb:cb + 1], 0.0)
            u[:4] = [tie(after(g), x) for x in u[:4]]
            put(cb, NA + a, g, _outer_fwd(u))

    def split_signal(cb, a, after):
        keys, vals = k_v.bitcast(U32), v_v.bitcast(U32)
        taps = [jnp.broadcast_to(sh_v[j:j + 1, pl.ds(cb * 128, 128)].astype(F32), (8, 128))
                for j in range(TAPS)]
        base = a * (CH // 2) if isinstance(a, int) else pl.multiple_of(a * (CH // 2), CH // 2)
        for g in range(N2 // 8):
            w = [tie(after(g), t) for t in taps]
            u = []
            for j in range(N1):
                r = base + j * N2 // 2 + g // 2 * 8
                lag = [_phase(keys[cb, pl.ds(r + PAD // 2 + (g % 2 - t) // 2, 8), :], (g % 2 - t) % 2)
                       for t in range(TAPS)]
                u.append(_add([x * wt for x, wt in zip(lag, w)]) * _phase(vals[cb, pl.ds(r, 8), :], g % 2))
            put(cb, a, g, _outer_fwd(u))

    def spectra(cb, b, half, f_ref):
        rhs = jnp.concatenate([_ld(au_v[cb % 2], b, half * NA + a) for a in range(NA)], axis=1)
        f = _nn(_ld(vf_v, b), rhs)
        for a in range(NA):
            f_ref[half * NA + a] = f[:, 128 * a:128 * a + 128]
        return f

    def product(f_ref, y_ref, plus, real_rows=None):
        for g in range(8):
            ur, ui, kr, ki = ([f_ref[o + a, pl.ds(16 * g + 8 * c, 8), :] for a in range(NA)]
                              for o in (0, NA) for c in (0, 1))
            kr, ki = ([k[0]] + [k[a] + k[a - 1] if plus else k[a] - k[a - 1] for a in range(1, NA)]
                      for k in (kr, ki))
            for a in range(NA):
                yi = _add([kr[j] * ui[a - j] + ki[j] * ur[a - j] for j in range(a + 1)])
                if real_rows is not None and g == 0:
                    rr = _add([kr[j] * ur[a - j] for j in range(a + 1)])
                    ii = _add([ki[j] * ui[a - j] for j in range(a + 1)])
                    yr = jnp.where(real_rows, 0.5 * rr, rr - ii)
                    yi = jnp.where(real_rows, 0.5 * ii, yi)
                else:
                    yr = _add([kr[j] * ur[a - j] - ki[j] * ui[a - j] for j in range(a + 1)])
                y_ref[a, pl.ds(16 * g, 16), :] = jnp.concatenate([yr, yi], axis=0).astype(BF16)

    def residues(y_ref, b, dst):
        r = _nn(_ld(vf_v, 8 + b), jnp.concatenate([_ld(y_ref, a) for a in range(NA)], axis=1))
        for a in range(NA):
            dst[a] = r[:, 128 * a:128 * a + 128]
        return r

    def stash(t):
        return ((bm0_v.at[t], bp0_v.at[t]) if t < 16 else (bm1_v.at[t - 16], bp1_v.at[t - 16]))

    def merge(cb, a, after=lambda g: None):
        src = [stash(1 + 4 * cb + b)[s] for s in (0, 1) for b in range(4)]
        for g in range(N2 // 8):
            res = [[ref[a, pl.ds(16 * g + 8 * c, 8), :] for c in (0, 1)] for ref in src]
            res[0] = [tie(after(g), x) for x in res[0]]
            res[1] = [tie(after(g), x) for x in res[1]]
            for j, y in enumerate(_outer_inv(res)):
                y_v[cb, _ds(a * CH + j * N2 + 8 * g, 8, 8), :] = y

    def transform(cb, a, dst, active=True):
        pa = (a + 3) % 4
        res = []
        if active:
            res += [spectra(cb, a, 1, fa_v), spectra(cb, a, 0, fa_v)]
        product(fb_v, yb_v, True, row8 + (3 - pa) == 0)
        res.append(residues(ya_v, pa, dst[0]))
        if active:
            res += [spectra(cb, 4 + a, 1, fb_v), spectra(cb, 4 + a, 0, fb_v)]
            product(fa_v, ya_v, False)
        res.append(residues(yb_v, 4 + pa, dst[1]))
        return res

    def conv_step(cb, i):
        steps = [UN * i + u for u in range(UN)]
        if cb < NCB:
            for a in steps:
                for cp in conv_inputs(cb, a):
                    cp.wait()
        done = []
        for a in steps if cb else ():
            done += transform(cb - 1, a, (bm0_v.at[4 * cb - 4 + a], bp0_v.at[4 * cb - 4 + a])
                              if cb < NCB else (bm1_v.at[a], bp1_v.at[a]))
        at = lambda p: done[p // 8][16 * (p % 8):16 * (p % 8) + 8, 0:128] if done and p >= 0 else None
        for u, a in enumerate(steps):
            if cb < NCB:
                split_signal(cb, a, lambda g: at(TU[8 * u + g]))
                split_filter(cb, a, lambda g: at(TK[8 * u + g]))
            else:
                for c in range(3):
                    merge(c, a, lambda g: at(TI[24 * u + 8 * c + g]))

    wait("sh", "sd")
    for cb in range(NCB + 1):
        if cb == 1:
            wait("vf")
        fetch(cb + 2)
        pl.loop(0, NA // UN)(functools.partial(conv_step, cb))

    wait("c", "wm")
    transform(NCB, 0, stash(20), active=False)
    cc = c_v[...].astype(F32)
    sc = jnp.broadcast_to(cc / (1.0 + jnp.exp(-cc)), (16, D)).astype(BF16)
    mod = _nn(sc, wm_v[:, pl.ds(0, 5 * D)])[0:8]
    sa, ca, ga, sb, cb_ = (mod[:, i * D:(i + 1) * D] for i in range(5))
    m1, m0 = ga * (1.0 + ca), ga * sa
    n1, n0 = _GA * (1.0 + cb_), _GA * sb
    zero = zero_s[0]
    for n, (cb, a) in enumerate([(cb, a) for cb in (3, 4) for a in range(MA)]):
        merge(cb, a + zero, lambda g: mod[:, 128 * ((8 * n + g) * MS // (16 * MA)):][:, :128])

    TB = RB // 128
    PER = 2 * FH // 16

    def hidden(r0, after=(None, None)):
        out = []
        for r, a in zip((r0, r0 + 8), after):
            rows = pl.ds(r, 8)
            x = q_v[rows, :].astype(F32)
            x = jnp.concatenate([tie(a, x[:, :128]), x[:, 128:]], axis=1)
            x1 = x + (_ln_rows(x) * m1 + m0) * jnp.concatenate([y_v[j, rows, :] for j in range(NCB)], axis=1)
            x1_v[rows, :] = x1
            out.append(_ln_rows(x1) * n1 + n0)
        return jnp.concatenate(out, axis=0)

    def keep_gate(tile, z):
        lists[tile][pl.ds(zero, FH), :] = z

    def moments(tile, after):
        z, acc = lists[tile], lists[16 + tile]
        s1 = s2 = None
        for n, f in enumerate(range(0, FH, SU)):
            for r in range(f, f + SU, 8):
                d = tie(after(n)[:8] if r == f else None, z[pl.ds(r, 8), :])
                s1, s2 = (d, d * d) if s1 is None else (s1 + d, s2 + d * d)
            acc[pl.ds(16 * n + zero, 16), :] = jnp.concatenate([s1, s2], axis=0)
        s1, s2 = (jnp.sum(acc[pl.ds(16 * n + r, 8), :], axis=0, keepdims=True) for r in (0, 8))
        stats[tile] = [jnp.broadcast_to(t, (16, 128)) for t in _norm_stats(s1, s2, FH, EPS * (2 * _GA) ** 2)]

    def norm_gate(pair, after):
        for n in range(FM // 16):
            means = [tie(after(n), stats[2 * pair + c][0]) for c in (0, 1)]
            quad = [(lists[2 * pair + c][pl.ds(r + 16 * n, 16), :] - means[c]) * stats[2 * pair + c][1]
                    for r in (0, FM) for c in (0, 1)]
            for k, a in enumerate(_lhs7(*quad)):
                z2_v[k, pair, pl.ds(16 * n, 16), :] = a

    def lanes(x, j, n=1):
        return x[:, 128 * j:128 * (j + n)]

    def prepare(i, c, after):
        def put(k, n, x):
            for j in range(x.shape[1] // 128):
                h_v[i % 2][k][j, pl.ds(16 * n + zero, 16), :] = lanes(x, j).astype(BF16)

        for n in range(H // 16):
            h = hidden(i * RB + c * H + 16 * n, (after(2 * n)[:8], after(2 * n + 1)[:8]))
            top, bot = lanes(h, 0, 2), lanes(h, 2, 2)
            put(7 + c, n, lanes(h, 4))
            if c:
                half[n] = top, bot
                put(2, n, top - bot)
                put(4, n, bot)
            else:
                put(1, n, top)
                put(3, n, bot - top)
                put(0, n, top + half[n][1])
                put(5, n, top + half[n][0])
                put(6, n, bot + half[n][1])

    def side_jobs(plan, at):
        for job in plan.split(","):
            if job:
                kind, (n, *spans) = job[0], (int(x) for x in job[1:].split(":"))
                total = {"s": FH // SU, "n": FM // 16, "h": H // 8, "m": N2 // 8}[kind]
                slots = [p for lo, hi in zip(spans[::2], spans[1::2]) for p in range(lo, hi)]
                after = lambda k: at(slots[k * len(slots) // total])
                if kind == "s":
                    moments(n, after)
                elif kind == "m":
                    merge(n // NA, n % NA + zero, lambda k: after(k)[:8])
                elif kind == "n":
                    norm_gate(n, after)
                else:
                    prepare(n // 2, n % 2, after)

    def rows_of(z):
        per = z.shape[0] // 16
        return lambda p: z[16 * (p % per):16 * (p % per) + 16, 128 * (p // per):128 * (p // per) + 128]

    def project(i):
        def prod(*pairs):
            right = [_ld(h_v[i % 2][k], j) for _, k in pairs for j in range(2 if k < 7 else 1)]
            return _nt(jnp.concatenate([x for k, _ in pairs for x in left[k]], axis=1),
                       jnp.concatenate(right, axis=1))

        s5, s3, r12, s4, s1 = prod((4, 4)), prod((2, 2)), prod((7, 8)), prod((3, 3)), prod((0, 0))
        s7, s2, r21, s6 = prod((6, 6), (7, 7)), prod((1, 1)), prod((8, 7)), prod((5, 5), (8, 8))
        gate = [_gelu_scaled(((s4 - s5) + s1) + s7), _gelu_scaled((s5 + s3) + r12)]
        value = [_gelu_scaled((s4 + s2) + r21), _gelu_scaled(((s3 + s1) - s2) + s6)]
        for t in range(TB):
            keep_gate(i * TB + t, lanes(gate[t // 2], t % 2))
            z1_v[i * TB + t] = lanes(value[t // 2], t % 2).astype(BF16)
        rounds = (s5, s3, gate[1], s4, s1, gate[0], s2, value[0], lanes(value[1], 1))
        return lambda p: rounds[p // (FH // 16)][16 * (p % (FH // 16)):16 * (p % (FH // 16)) + 16, 0:128]

    def first(f0, extra=()):
        h = jnp.concatenate([_ld(h0_v, j, pl.ds(0, (RB - 16 * len(extra)) // 2)) for j in range(NCB)], axis=1)
        if extra:
            h = jnp.concatenate([h, jnp.concatenate(extra, axis=0).astype(BF16)], axis=0)
        return _gelu_scaled(_nt(wi_v[pl.ds(f0, FH), :], h))

    def keep_first(r, h):
        for j in range(NCB):
            h0_v[j, pl.ds(r, 16), :] = lanes(h, j).astype(BF16)

    stats, half = {}, {}
    wait("q0")
    for r in range(0, H, 16):
        keep_first(r, hidden(r))
    wait("w2", "q1")
    zero = pl.multiple_of(zero_s[0], 16)
    extra = [hidden(r) for r in range(H, RB, 16)]
    for n, h in enumerate(extra):
        keep_first(H + 16 * n, h)
    z = first(0, extra)
    for t in range(TB):
        keep_gate(t, lanes(z, t))
    side_jobs(NJ[0], rows_of(z))
    wait("w1", "q2")
    z = first(FH)
    for t in range(TB):
        z1_v[t] = lanes(z, t).astype(BF16)
    side_jobs(NJ[1], rows_of(z))
    sums = [_lhs7(*(wi_v[pl.ds(FH * r, FH), pl.ds(256 * c + 128 * j, 128)].astype(F32)
                    for r in (0, 1) for c in (0, 1))) for j in (0, 1)]
    left = ([[s[k].astype(BF16) for s in sums] for k in range(7)]
            + [[_whole(wi_v[pl.ds(FH * r, FH), pl.ds(512, 128)])] for r in (0, 1)])
    for i in range(1, NB):
        side_jobs(NJ[i + 1], project(i))

    wait("wg", "b", "wo")
    gb = _nn(sc, wm_v[:, pl.ds(5 * D, D)]) * (0.5 / _GA)
    bf_v[...] = b_v[...].astype(F32)
    for j in range(KO):
        a1, a2 = (wo_v[pl.ds(128 * (j + KO * c), 128), :].T.astype(F32) for c in (0, 1))
        for n, a in enumerate(_lhs7(a1[:DM], a2[:DM], a1[DM:], a2[DM:])):
            wt_v[n, j] = a.astype(BF16)
    wr_v[...] = wo_v[pl.ds(256 * KO, 128), :].T
    T2 = R2 // 128

    def mix(i):
        def w(c, r):
            return [ws_v[i % 2, pl.ds(r * H, H), pl.ds(256 * j + 128 * c, 128)].astype(F32) for j in range(S // 256)]

        def comb(x, y, sign):
            return [a + b if sign > 0 else a - b for a, b in zip(x, y)]

        def prod(n, rhs):
            def left(k):
                def part(r, c, rows):
                    return jnp.concatenate([z2_v[n, 2 * j + c, pl.ds(FT * r, rows), :] for j in range(NB)], axis=1)

                def both(c, op):
                    top = part(0, c, FT)
                    return jnp.concatenate([op(top[:FB], part(1, 1, FB)), top[FB:]], axis=0)

                return (lambda: both(0, jnp.add), lambda: part(1, 0, FB) + part(1, 1, FB),
                        lambda: part(0, 0, FT), lambda: part(1, 1, FB),
                        lambda: part(0, 0, FT) + part(0, 1, FT), lambda: part(1, 0, FB) - part(0, 0, FB),
                        lambda: both(1, jnp.subtract))[k]().astype(BF16)

            b11, b12, b21, b22 = (
                jnp.concatenate([rhs[2 * j + c][128 * r:128 * r + 128] for j in range(NB)], axis=1)
                for c in (0, 1) for r in (0, 1))
            m = lambda k, x: _nt(left(k), x.astype(BF16))
            m2, m5, m4 = m(1, b11), m(4, b22), m(3, b21 - b11)
            m1, m7, m3, m6 = m(0, b11 + b22), m(6, b21 + b22), m(2, b12 - b22), m(5, b11 + b12)
            c11 = jnp.concatenate([m4 - m5[:FB], -m5[FB:]], axis=0) + m1 + m7
            c22 = (m1[:FB] - m2) + m3[:FB] + m6
            return jnp.concatenate([jnp.concatenate([c11, m5 + m3], axis=1),
                                    jnp.concatenate([m2 + m4, c22], axis=1)], axis=0)

        def gate(r, c, g):
            tiles = [i * T2 + c * (H // 128) + t for t in range(H // 128)]
            bias = jnp.concatenate([bf_v[pl.ds(j, 1), :] for j in tiles], axis=1)
            z1 = jnp.concatenate([z1_v[j, pl.ds(FM * r, FM), :] for j in tiles], axis=1).astype(F32)
            return z1 * (g + bias)

        s2 = prod(1, w(0, 0))
        s5 = prod(4, w(1, 1))
        s4 = prod(3, comb(w(1, 0), w(0, 0), -1))
        p21 = gate(1, 0, s2 + s4)
        d11 = s4 - s5
        s1 = prod(0, comb(w(0, 0), w(1, 1), 1))
        d11, d22 = d11 + s1, s1 - s2
        p11 = gate(0, 0, d11 + prod(6, comb(w(1, 0), w(1, 1), 1)))
        s3 = prod(2, comb(w(0, 1), w(1, 1), -1))
        p12 = gate(0, 1, s3 + s5)
        p22 = gate(1, 1, (d22 + s3) + prod(5, comb(w(0, 0), w(0, 1), 1)))
        return [jnp.concatenate(p, axis=0) for p in ((p11, p21), (p12, p22))]

    def flush(k):
        rows = _ds(k * FL, FL, FL)
        return pltpu.make_async_copy(o_v.at[rows], o_h.at[rows], osem.at[k])

    def mix_step(i):
        mixing(i).wait()

        @pl.when(i + 1 < S // R2)
        def _():
            mixing(i + 1).start()

        p = mix(i)
        b11, b12, b21, b22 = (p[c][128 * KO * r:128 * KO * (r + 1)] for r in (0, 1) for c in (0, 1))

        def prod(n, rhs):
            return _nn(jnp.concatenate([_ld(wt_v, n, j) for j in range(KO)], axis=1), rhs.astype(BF16))

        def rest(c):
            tail = jnp.concatenate([p[c][256 * KO:], jnp.zeros((128 + 256 * KO - FH, H), F32)], axis=0)
            return _nn(_ld(wr_v), tail.astype(BF16))

        def finish(c, ot):
            for t in range(H // 128):
                rows = _ds(i * R2 + c * H + 128 * t, 128, 128)
                o = ot[:, 128 * t:128 * t + 128].T
                o_v[rows, :] = (x1_v[rows, :] + jnp.concatenate([gb] * 8, axis=0) * o).astype(BF16)
                done = c * H + 128 * (t + 1)
                if done % FL == 0:
                    flush(i * (R2 // FL) + done // FL - 1).start()

        r0 = rest(0)
        s2 = prod(1, b11)
        s4 = prod(3, b21 - b11)
        s5 = prod(4, b22)
        s1 = prod(0, b11 + b22)
        s7 = prod(6, b21 + b22)
        finish(0, jnp.concatenate([r0[:DM] + s4 - s5 + s1 + s7, r0[DM:] + s2 + s4], axis=0))
        r1 = rest(1)
        s3 = prod(2, b12 - b22)
        s6 = prod(5, b11 + b12)
        finish(1, jnp.concatenate([r1[:DM] + s5 + s3, (s1 - s2) + r1[DM:] + s3 + s6], axis=0))

    if UR:
        for i in range(S // R2):
            mix_step(i)
    else:
        pl.loop(0, S // R2)(mix_step)
    for k in range(S // FL):
        flush(k).wait()


@jax.jit
def pallas_adaLN_cond__ssm_conv_h3__mixer_gmlp__prompt_kernel(
    A_q, A_k, A_v, A_shift_k, A_ssm_k, A_ssm_D, B_x, B_w_in, B_w_sp, B_b_sp, B_w_out, c, w_mod,
):
    del B_x
    vf = _dft_mats().astype(BF16)
    vm = pltpu.VMEM
    tile = (128, 128)
    scratch = [
        vm((S, D), BF16), vm((NCB, PAD + S, 128), BF16), vm((NCB, S, 128), BF16), vm((TAPS, D), BF16),
        vm((NCB, NA, 128, CH), BF16), vm((NCB, 128), BF16), vm((2 * FH, D), BF16),
        vm((2, R2, S), BF16), vm((S // 128, 128), BF16), vm((256 * KO + 128, D), BF16), vm((1, D), BF16),
        vm((D, 6 * D), BF16), vm((16, *tile), BF16),
        vm((8, 2 * NA, *tile), BF16), vm((8, 2 * NA, *tile), BF16),
        vm((2 * NA, *tile), F32), vm((2 * NA, *tile), F32), vm((NA, *tile), BF16), vm((NA, *tile), BF16),
        vm((16, NA, *tile), F32), vm((16, NA, *tile), F32), vm((5, NA, *tile), F32), vm((5, NA, *tile), F32),
        vm((NCB, S, 128), F32), vm((S, D), F32), vm((NCB, RB, 128), BF16),
        vm((S // 128, FH, 128), BF16), vm((7, S // 256, FM, 128), F32),
        vm((7, KO, DM, 128), BF16), vm((D, 128), BF16), vm((S // 128, 128), F32),
        vm((S, D), BF16), vm((8, 128), jnp.int32), pltpu.SMEM((1,), jnp.int32),
        pltpu.SemaphoreType.DMA((NCB * NA + 32,)),
        pltpu.SemaphoreType.DMA((S // FL,)),
    ] + [vm((FH, 128), F32)] * 16 + [vm((FH // SU * 16, 128), F32)] * 16 + [vm((2, H, 128), BF16)] * 18
    out = pl.pallas_call(
        _kernel,
        out_shape=jax.ShapeDtypeStruct((S, D), BF16),
        in_specs=[pl.BlockSpec(memory_space=pltpu.HBM)] * 13,
        out_specs=pl.BlockSpec(memory_space=pltpu.HBM),
        scratch_shapes=scratch,
        compiler_params=pltpu.CompilerParams(vmem_limit_bytes=110 * 1024 * 1024),
    )(A_q.reshape(S, D), A_k.reshape(S, D), A_v.reshape(S, D), A_shift_k.T, A_ssm_k,
      A_ssm_D.reshape(NCB, 128), B_w_in.T, B_w_sp, B_b_sp.reshape(S // 128, 128), B_w_out, c, w_mod, vf)
    return out.reshape(1, S, D)
```

```python
import functools
import math

import numpy as np
import jax
import jax.numpy as jnp
from jax import lax
import jax.experimental.pallas as pl
import jax.experimental.pallas.tpu as pltpu

S, D, FH = 2048, 640, 864
FM, DM = FH // 2, D // 2
KO = FH // 256
FT, FB = 224, 208
TAPS = 4
CH = 512
NA = S // CH
N2 = 64
N1 = CH // N2
NCB = D // 128
RB = 512
NB = S // RB
H = RB // 2
EPS = 1e-5
F32, BF16, U32 = jnp.float32, jnp.bfloat16, jnp.uint32
PAD = 16

_C8 = math.cos(math.pi / 8)
_T8 = math.tan(math.pi / 8)
_R2 = math.sqrt(0.5)
_G0 = math.sqrt(2 / math.pi)
_GA = (_G0 * 0.044715) ** (1 / 3)

UN = 1
DG = 0
E0, ES = 0, 16
MA = 2
MS = 22
TU = (-1, 0, 3, 5, 16, 32, 35, 38)
TK = (34, 38, 41, 42, 43, 44, 45, 46)
TI = (-1, -1, -1, -1, -1, -1, -1, -1, 0, 2, 4, 6, 16, 17, 32, 33, 34, 35, 36, 37, 38, 39, 40, 41)
SU = 96
NJ = ["s0:76:105,s1:114:170,s2:168:205,m14:60:100,m18:100:140,m15:140:175,m19:165:200", "h3:0:96,h2:104:229,s3:20:80",
      "h5:0:108:132:186,h4:192:246:324:440,s4:330:402,s6:216:270",
      "h7:0:108:162:216,h6:226:280:324:440,s5:0:54,s7:54:108,s8:324:372,s10:216:270",
      "n0:0:50,n1:30:80,n2:70:108,s9:0:40,s11:40:80,n3:110:170,n4:160:216,n5:216:270,s14:170:216,s15:220:270,n7:280:340,s12:330:378,s13:380:410,n6:420:480"]
R2 = 512
FL = 256
UR = 0


def _dft_mats():
    ang = [1 / 16 + m / 4 for m in range(4)] + [1 / 8, 1 / 8 + 1 / 2, 1 / 4]
    idx = np.arange(128)
    pos = (idx // 16) * 8 + idx % 8
    part = (idx // 8) % 2
    mats = []
    for b, a in enumerate(ang):
        th = 2 * np.pi * (a + pos[:, None]) * pos[None, :] / N2
        po, pi = part[:, None], part[None, :]
        m = np.where(po == pi, np.cos(th), np.where(po == 1, np.sin(th), -np.sin(th)))
        mats.append(m * ((_C8 if b < 4 else 1.0) / 8))
    n = pos + 64 * part
    th = 2 * np.pi * pos[:, None] * n[None, :] / 128
    m = np.where(part[:, None] == 0, np.cos(th), np.sin(th))
    m[8, :] = 1.0 - 2.0 * (n % 2)
    mats.append(m / 8)
    fwd = np.stack(mats).astype(np.float32)
    n = idx // 32 * 16 + idx % 8 * 2 + idx // 16 % 2
    return fwd[:, :, n // 8 * 16 + part * 8 + n % 8]


def _outer_fwd(u):
    t0r, t0i = u[0] * (1 / _C8), u[4] * (1 / _C8)
    t2r, t2i = (u[2] - u[6]) * (_R2 / _C8), (u[2] + u[6]) * (_R2 / _C8)
    t1r, t1i = u[1] - _T8 * u[5], u[5] + _T8 * u[1]
    t3r, t3i = _T8 * u[3] - u[7], _T8 * u[7] + u[3]
    ar, ai, br, bi = t0r + t2r, t0i + t2i, t0r - t2r, t0i - t2i
    cr, ci, dr, di = t1r + t3r, t1i + t3i, t1r - t3r, t1i - t3i
    out = [(ar + cr, ai + ci), (br - di, bi + dr), (ar - cr, ai - ci), (br + di, bi - dr)]
    p = [u[j] + u[j + 4] for j in range(4)]
    q = [u[j] - u[j + 4] for j in range(4)]
    er, ei = (q[1] - q[3]) * _R2, (q[1] + q[3]) * _R2
    out += [(q[0] + er, q[2] + ei), (q[0] - er, q[2] - ei)]
    out += [(p[0] - p[2], p[1] - p[3]), (p[0] + p[2], p[1] + p[3])]
    return out


def _outer_inv(B):
    ar, ai = B[0][0] + B[2][0], B[0][1] + B[2][1]
    cr, ci = B[0][0] - B[2][0], B[0][1] - B[2][1]
    br, bi = B[1][0] + B[3][0], B[1][1] + B[3][1]
    dr, di = B[1][0] - B[3][0], B[1][1] - B[3][1]
    g0r, g0i, g2r, g2i = ar + br, ai + bi, ar - br, ai - bi
    g1r, g1i, g3r, g3i = cr + di, ci - dr, cr - di, ci + dr
    nr = [g0r * (1 / _C8), g1r + _T8 * g1i, (g2r + g2i) * (_R2 / _C8), _T8 * g3r + g3i]
    ni = [g0i * (1 / _C8), g1i - _T8 * g1r, (g2i - g2r) * (_R2 / _C8), _T8 * g3i - g3r]
    fr, fi = B[4][0] - B[5][0], B[4][1] - B[5][1]
    q = [B[4][0] + B[5][0], (fr + fi) * _R2, B[4][1] + B[5][1], (fi - fr) * _R2]
    p = [B[7][0] + B[6][0], B[7][1] + B[6][1], B[7][0] - B[6][0], B[7][1] - B[6][1]]
    return ([p[j] + q[j] + nr[j] for j in range(4)]
            + [p[j] - q[j] + ni[j] for j in range(4)])


def _gelu_scaled(x):
    t = jnp.tanh(x * (_G0 / _GA + x * x))
    return x + x * t


def _norm_stats(s1, s2, n, eps):
    m = s1 * (1.0 / n)
    return m, jnp.exp(-0.5 * jnp.log(jnp.maximum(s2 * (1.0 / n) - m * m, 0.0) + eps))


def _ln_rows(x):
    m, r = _norm_stats(jnp.sum(x, axis=-1, keepdims=True), jnp.sum(x * x, axis=-1, keepdims=True),
                       x.shape[-1], EPS)
    return (x - m) * r


def _lhs7(a11, a12, a21, a22):
    return a11 + a22, a21 + a22, a11, a22, a11 + a12, a21 - a11, a12 - a22


def _ld(ref, *idx):
    return pltpu.bitcast(ref.bitcast(jnp.uint32)[idx or ...], BF16)


def _whole(x):
    return x


def _phase(words, odd):
    return pltpu.bitcast(words & np.uint32(0xFFFF0000) if odd else words << 16, F32)


def _nn(a, b):
    return jnp.dot(a, b, preferred_element_type=F32)


def _nt(a, b):
    return lax.dot_general(a, b, (((1,), (1,)), ((), ())), preferred_element_type=F32)


def _ds(start, size, align):
    return pl.ds(start if isinstance(start, int) else pl.multiple_of(start, align), size)


def _add(xs):
    return functools.reduce(lambda x, y: x + y, xs)


def _kernel(q_h, k_h, v_h, sh_h, sk_h, sd_h, wi_h, ws_h, b_h, wo_h, c_h, wm_h, vf_h, o_h,
            q_v, k_v, v_v, sh_v, sk_v, sd_v, wi_v, ws_v, b_v, wo_v, c_v, wm_v, vf_v,
            au0_v, au1_v, fa_v, fb_v, ya_v, yb_v, bm0_v, bp0_v, bm1_v, bp1_v,
            y_v, x1_v, h0_v, z1_v, z2_v, wt_v, wr_v, bf_v, o_v, tie_v, zero_s,
            sems, osem, *lists):
    au_v, h_v = (au0_v, au1_v), (lists[32:41], lists[41:])
    copies = {}

    def start(name, src, dst):
        copies[name] = pltpu.make_async_copy(src, dst, sems.at[NCB * NA + len(copies)])
        copies[name].start()

    def wait(*names):
        for name in names:
            copies[name].wait()

    def conv_inputs(cb, a):
        rows, lanes, sem = _ds(a * CH, CH, CH), pl.ds(cb * 128, 128), sems.at[cb * NA + a]
        return (pltpu.make_async_copy(k_h.at[rows, lanes], k_v.at[cb, _ds(PAD + a * CH, CH, PAD)], sem),
                pltpu.make_async_copy(v_h.at[rows, lanes], v_v.at[cb, rows], sem),
                pltpu.make_async_copy(sk_h.at[lanes, rows], sk_v.at[cb, a], sem))

    def mixing(i):
        return pltpu.make_async_copy(ws_h.at[_ds(i * R2, R2, R2)], ws_v.at[i % 2], sems.at[NCB * NA + 16 + i])

    def fetch(stage):
        if stage < NCB:
            for a in range(NA):
                for cp in conv_inputs(stage, a):
                    cp.start()
        if stage == 0:
            start("vf", vf_h, vf_v.at[pl.ds(0, 8)])
        if stage == NCB:
            start("c", c_h, c_v)
            start("wm", wm_h.at[:, pl.ds(0, 5 * D)], wm_v.at[:, pl.ds(0, 5 * D)])
            start("q0", q_h.at[pl.ds(0, H)], q_v.at[pl.ds(0, H)])
            start("w2", wi_h.at[pl.ds(FH, FH)], wi_v.at[pl.ds(0, FH)])
            start("q1", q_h.at[pl.ds(H, RB - H)], q_v.at[pl.ds(H, RB - H)])
            start("w1", wi_h.at[pl.ds(0, FH)], wi_v.at[pl.ds(FH, FH)])
            start("q2", q_h.at[pl.ds(RB, S - RB)], q_v.at[pl.ds(RB, S - RB)])
        if stage == NCB + 2:
            start("wg", wm_h.at[:, pl.ds(5 * D, D)], wm_v.at[:, pl.ds(5 * D, D)])
            start("b", b_h, b_v)
            start("wo", wo_h, wo_v.at[pl.ds(0, FH)])
            mixing(0).start()

    start("sh", sh_h, sh_v)
    start("sd", sd_h, sd_v)
    fetch(0)
    fetch(1)
    for ref in (fb_v, ya_v, tie_v):
        ref[...] = jnp.zeros(ref.shape, ref.dtype)
    k_v[:, pl.ds(0, PAD), :] = jnp.zeros((NCB, PAD, 128), BF16)
    wo_v[pl.ds(FH, 256 * KO + 128 - FH), :] = jnp.zeros((256 * KO + 128 - FH, D), BF16)
    zero_s[0] = 0
    row8 = lax.broadcasted_iota(jnp.int32, (8, 128), 0)

    def tie(after, x):
        if after is None:
            return x
        never = jnp.concatenate([tie_v[...]] * (x.shape[0] // 8), axis=0) != 0
        return jnp.where(never, after, x)

    def put(cb, slot, g, res):
        for b in range(8):
            au_v[cb % 2][b, slot, pl.ds(16 * g, 16), :] = jnp.concatenate(res[b], axis=0).astype(BF16)

    def split_filter(cb, a, after):
        kt = pltpu.bitcast(sk_v[cb, a].T, U32)
        for g in range(N2 // 8):
            u = [_phase(kt[j * N2 // 2 + g // 2 * 8:j * N2 // 2 + g // 2 * 8 + 8], g % 2) for j in range(N1)]
            if g == 0:
                u[0] = u[0] + jnp.where(row8 + a == 0, sd_v[...].astype(F32)[cb:cb + 1], 0.0)
            u[:4] = [tie(after(g), x) for x in u[:4]]
            put(cb, NA + a, g, _outer_fwd(u))

    def split_signal(cb, a, after):
        keys, vals = k_v.bitcast(U32), v_v.bitcast(U32)
        taps = [jnp.broadcast_to(sh_v[j:j + 1, pl.ds(cb * 128, 128)].astype(F32), (8, 128))
                for j in range(TAPS)]
        base = a * (CH // 2) if isinstance(a, int) else pl.multiple_of(a * (CH // 2), CH // 2)
        for g in range(N2 // 8):
            w = [tie(after(g), t) for t in taps]
            u = []
            for j in range(N1):
                r = base + j * N2 // 2 + g // 2 * 8
                lag = [_phase(keys[cb, pl.ds(r + PAD // 2 + (g % 2 - t) // 2, 8), :], (g % 2 - t) % 2)
                       for t in range(TAPS)]
                u.append(_add([x * wt for x, wt in zip(lag, w)]) * _phase(vals[cb, pl.ds(r, 8), :], g % 2))
            put(cb, a, g, _outer_fwd(u))

    def spectra(cb, b, half, f_ref):
        rhs = jnp.concatenate([_ld(au_v[cb % 2], b, half * NA + a) for a in range(NA)], axis=1)
        f = _nn(_ld(vf_v, b), rhs)
        for a in range(NA):
            f_ref[half * NA + a] = f[:, 128 * a:128 * a + 128]
        return f

    def product(f_ref, y_ref, plus, real_rows=None):
        for g in range(8):
            ur, ui, kr, ki = ([f_ref[o + a, pl.ds(16 * g + 8 * c, 8), :] for a in range(NA)]
                              for o in (0, NA) for c in (0, 1))
            kr, ki = ([k[0]] + [k[a] + k[a - 1] if plus else k[a] - k[a - 1] for a in range(1, NA)]
                      for k in (kr, ki))
            for a in range(NA):
                yi = _add([kr[j] * ui[a - j] + ki[j] * ur[a - j] for j in range(a + 1)])
                if real_rows is not None and g == 0:
                    rr = _add([kr[j] * ur[a - j] for j in range(a + 1)])
                    ii = _add([ki[j] * ui[a - j] for j in range(a + 1)])
                    yr = jnp.where(real_rows, 0.5 * rr, rr - ii)
                    yi = jnp.where(real_rows, 0.5 * ii, yi)
                else:
                    yr = _add([kr[j] * ur[a - j] - ki[j] * ui[a - j] for j in range(a + 1)])
                y_ref[a, pl.ds(16 * g, 16), :] = jnp.concatenate([yr, yi], axis=0).astype(BF16)

    def residues(y_ref, b, dst):
        r = _nn(_ld(vf_v, 8 + b), jnp.concatenate([_ld(y_ref, a) for a in range(NA)], axis=1))
        for a in range(NA):
            dst[a] = r[:, 128 * a:128 * a + 128]
        return r

    def stash(t):
        return ((bm0_v.at[t], bp0_v.at[t]) if t < 16 else (bm1_v.at[t - 16], bp1_v.at[t - 16]))

    def merge(cb, a, after=lambda g: None):
        src = [stash(1 + 4 * cb + b)[s] for s in (0, 1) for b in range(4)]
        for g in range(N2 // 8):
            res = [[ref[a, pl.ds(16 * g + 8 * c, 8), :] for c in (0, 1)] for ref in src]
            res[0] = [tie(after(g), x) for x in res[0]]
            res[1] = [tie(after(g), x) for x in res[1]]
            for j, y in enumerate(_outer_inv(res)):
                y_v[cb, _ds(a * CH + j * N2 + 8 * g, 8, 8), :] = y

    def transform(cb, a, dst, active=True):
        pa = (a + 3) % 4
        res = []
        if active:
            res += [spectra(cb, a, 1, fa_v), spectra(cb, a, 0, fa_v)]
        product(fb_v, yb_v, True, row8 + (3 - pa) == 0)
        res.append(residues(ya_v, pa, dst[0]))
        if active:
            res += [spectra(cb, 4 + a, 1, fb_v), spectra(cb, 4 + a, 0, fb_v)]
            product(fa_v, ya_v, False)
        res.append(residues(yb_v, 4 + pa, dst[1]))
        return res

    def conv_step(cb, i):
        steps = [UN * i + u for u in range(UN)]
        if cb < NCB:
            for a in steps:
                for cp in conv_inputs(cb, a):
                    cp.wait()
        done = []
        for a in steps if cb else ():
            done += transform(cb - 1, a, (bm0_v.at[4 * cb - 4 + a], bp0_v.at[4 * cb - 4 + a])
                              if cb < NCB else (bm1_v.at[a], bp1_v.at[a]))
        at = lambda p: done[p // 8][16 * (p % 8):16 * (p % 8) + 8, 0:128] if done and p >= 0 else None
        for u, a in enumerate(steps):
            if cb < NCB:
                split_signal(cb, a, lambda g: at(TU[8 * u + g]))
                split_filter(cb, a, lambda g: at(TK[8 * u + g]))
            else:
                for c in range(3):
                    merge(c, a, lambda g: at(TI[24 * u + 8 * c + g]))

    wait("sh", "sd")
    for cb in range(NCB + 1):
        if cb == 1:
            wait("vf")
            row, col = (lax.broadcasted_iota(jnp.int32, (128, 128), d) for d in (0, 1))
            n = (col >> 5) * 16 + (col & 7) * 2 + ((col >> 4) & 1)
            order = jnp.where(row == (n >> 3) * 16 + (col & 8) + (n & 7), 1.0, 0.0).astype(BF16)
            for b in range(8):
                vf_v[8 + b] = _nt(order, vf_v[b]).astype(BF16)
        fetch(cb + 2)
        pl.loop(0, NA // UN)(functools.partial(conv_step, cb))

    wait("c", "wm")
    transform(NCB, 0, stash(20), active=False)
    cc = c_v[...].astype(F32)
    sc = jnp.broadcast_to(cc / (1.0 + jnp.exp(-cc)), (16, D)).astype(BF16)
    mod = _nn(sc, wm_v[:, pl.ds(0, 5 * D)])[0:8]
    sa, ca, ga, sb, cb_ = (mod[:, i * D:(i + 1) * D] for i in range(5))
    m1, m0 = ga * (1.0 + ca), ga * sa
    n1, n0 = _GA * (1.0 + cb_), _GA * sb
    zero = zero_s[0]
    for n, (cb, a) in enumerate([(cb, a) for cb in (3, 4) for a in range(MA)]):
        merge(cb, a + zero, lambda g: mod[:, 128 * ((8 * n + g) * MS // (16 * MA)):][:, :128])

    TB = RB // 128
    PER = 2 * FH // 16

    def hidden(r0, after=(None, None)):
        out = []
        for r, a in zip((r0, r0 + 8), after):
            rows = pl.ds(r, 8)
            x = q_v[rows, :].astype(F32)
            x = jnp.concatenate([tie(a, x[:, :128]), x[:, 128:]], axis=1)
            x1 = x + (_ln_rows(x) * m1 + m0) * jnp.concatenate([y_v[j, rows, :] for j in range(NCB)], axis=1)
            x1_v[rows, :] = x1
            out.append(_ln_rows(x1) * n1 + n0)
        return jnp.concatenate(out, axis=0)

    def keep_gate(tile, z):
        lists[tile][pl.ds(zero, FH), :] = z

    def moments(tile, after):
        z, acc = lists[tile], lists[16 + tile]
        s1 = s2 = None
        for n, f in enumerate(range(0, FH, SU)):
            for r in range(f, f + SU, 8):
                d = tie(after(n)[:8] if r == f else None, z[pl.ds(r, 8), :])
                s1, s2 = (d, d * d) if s1 is None else (s1 + d, s2 + d * d)
            acc[pl.ds(16 * n + zero, 16), :] = jnp.concatenate([s1, s2], axis=0)
        s1, s2 = (jnp.sum(acc[pl.ds(16 * n + r, 8), :], axis=0, keepdims=True) for r in (0, 8))
        stats[tile] = [jnp.broadcast_to(t, (16, 128)) for t in _norm_stats(s1, s2, FH, EPS * (2 * _GA) ** 2)]

    def norm_gate(pair, after):
        for n in range(FM // 16):
            means = [tie(after(n), stats[2 * pair + c][0]) for c in (0, 1)]
            quad = [(lists[2 * pair + c][pl.ds(r + 16 * n, 16), :] - means[c]) * stats[2 * pair + c][1]
                    for r in (0, FM) for c in (0, 1)]
            for k, a in enumerate(_lhs7(*quad)):
                z2_v[k, pair, pl.ds(16 * n, 16), :] = a

    def lanes(x, j, n=1):
        return x[:, 128 * j:128 * (j + n)]

    def prepare(i, c, after):
        def put(k, n, x):
            for j in range(x.shape[1] // 128):
                h_v[i % 2][k][j, pl.ds(16 * n + zero, 16), :] = lanes(x, j).astype(BF16)

        for n in range(H // 16):
            h = hidden(i * RB + c * H + 16 * n, (after(2 * n)[:8], after(2 * n + 1)[:8]))
            top, bot = lanes(h, 0, 2), lanes(h, 2, 2)
            put(7 + c, n, lanes(h, 4))
            if c:
                half[n] = top, bot
                put(2, n, top - bot)
                put(4, n, bot)
            else:
                put(1, n, top)
                put(3, n, bot - top)
                put(0, n, top + half[n][1])
                put(5, n, top + half[n][0])
                put(6, n, bot + half[n][1])

    def side_jobs(plan, at):
        for job in plan.split(","):
            if job:
                kind, (n, *spans) = job[0], (int(x) for x in job[1:].split(":"))
                total = {"s": FH // SU, "n": FM // 16, "h": H // 8, "m": N2 // 8}[kind]
                slots = [p for lo, hi in zip(spans[::2], spans[1::2]) for p in range(lo, hi)]
                after = lambda k: at(slots[k * len(slots) // total])
                if kind == "s":
                    moments(n, after)
                elif kind == "m":
                    merge(n // NA, n % NA + zero, lambda k: after(k)[:8])
                elif kind == "n":
                    norm_gate(n, after)
                else:
                    prepare(n // 2, n % 2, after)

    def rows_of(z):
        per = z.shape[0] // 16
        return lambda p: z[16 * (p % per):16 * (p % per) + 16, 128 * (p // per):128 * (p // per) + 128]

    def project(i):
        def prod(*pairs):
            right = [_ld(h_v[i % 2][k], j) for _, k in pairs for j in range(2 if k < 7 else 1)]
            return _nt(jnp.concatenate([x for k, _ in pairs for x in left[k]], axis=1),
                       jnp.concatenate(right, axis=1))

        s5, s3, r12, s4, s1 = prod((4, 4)), prod((2, 2)), prod((7, 8)), prod((3, 3)), prod((0, 0))
        s7, s2, r21, s6 = prod((6, 6), (7, 7)), prod((1, 1)), prod((8, 7)), prod((5, 5), (8, 8))
        gate = [((s4 - s5) + s1) + s7, (s5 + s3) + r12]
        value = [(s4 + s2) + r21, ((s3 + s1) - s2) + s6]
        for c, later in enumerate((s2, lanes(s4, 1))):
            keep_gate(i * TB + 2 * c, _gelu_scaled(lanes(gate[c], 0)))
            keep_gate(i * TB + 2 * c + 1, _gelu_scaled(tie(lanes(later, 0) if DG else None, lanes(gate[c], 1))))
        for t in range(TB):
            z1_v[i * TB + t] = lanes(value[t // 2], t % 2)
        rounds = (s5, s3, gate[1], lanes(s4, 1), lanes(s1, 1), gate[0], s2, value[0], lanes(value[1], 1))
        return lambda p: rounds[p // (FH // 16)][16 * (p % (FH // 16)):16 * (p % (FH // 16)) + 16, 0:128]

    def first(f0, r0, n, k0, k1):
        h = jnp.concatenate([_ld(h0_v, j, pl.ds(r0 // 2, n // 2)) for j in range(k0, k1)], axis=1)
        return _nt(wi_v[pl.ds(f0, FH), pl.ds(128 * k0, 128 * (k1 - k0))], h)

    def keep_first(r, h):
        for j in range(NCB):
            h0_v[j, pl.ds(r, 16), :] = lanes(h, j).astype(BF16)

    stats, half = {}, {}
    wait("q0")
    for r in range(0, H, 16):
        keep_first(r, hidden(r))
    wait("w2", "q1")
    zero = pl.multiple_of(zero_s[0], 16)
    head = first(0, 0, H, 0, 2)
    z = _gelu_scaled(head + first(0, 0, H, 2, NCB))
    at = rows_of(jnp.concatenate([lanes(head, 0), z], axis=1))
    for n in range(H // 16):
        keep_first(H + 16 * n, hidden(H + 16 * n, [at(E0 + (2 * n + k) * ES // 8)[:8] for k in (0, 1)]))
    z = jnp.concatenate([z] + [_gelu_scaled(first(0, r, 128, 0, NCB)) for r in (H, H + 128)], axis=1)
    for t in range(TB):
        keep_gate(t, lanes(z, t))
    side_jobs(NJ[0], rows_of(z))
    wait("w1", "q2")
    head = first(FH, 0, RB, NCB - 1, NCB)
    z = head + first(FH, 0, RB, 0, NCB - 1)
    for t in range(TB):
        z1_v[t] = lanes(z, t)
    side_jobs(NJ[1], rows_of(jnp.concatenate([lanes(head, 0), z], axis=1)))
    sums = [_lhs7(*(wi_v[pl.ds(FH * r, FH), pl.ds(256 * c + 128 * j, 128)].astype(F32)
                    for r in (0, 1) for c in (0, 1))) for j in (0, 1)]
    left = ([[s[k].astype(BF16) for s in sums] for k in range(7)]
            + [[_whole(wi_v[pl.ds(FH * r, FH), pl.ds(512, 128)])] for r in (0, 1)])
    for i in range(1, NB):
        side_jobs(NJ[i + 1], project(i))

    wait("wg", "b", "wo")
    gb = _nn(sc, wm_v[:, pl.ds(5 * D, D)]) * (0.5 / _GA)
    bf_v[...] = b_v[...].astype(F32)
    for j in range(KO):
        a1, a2 = (wo_v[pl.ds(128 * (j + KO * c), 128), :].T.astype(F32) for c in (0, 1))
        for n, a in enumerate(_lhs7(a1[:DM], a2[:DM], a1[DM:], a2[DM:])):
            wt_v[n, j] = a.astype(BF16)
    wr_v[...] = wo_v[pl.ds(256 * KO, 128), :].T
    T2 = R2 // 128

    def mix(i):
        def w(c, r):
            return [ws_v[i % 2, pl.ds(r * H, H), pl.ds(256 * j + 128 * c, 128)].astype(F32) for j in range(S // 256)]

        def comb(x, y, sign):
            return [a + b if sign > 0 else a - b for a, b in zip(x, y)]

        def prod(n, rhs):
            def left(k):
                def part(r, c, rows):
                    return jnp.concatenate([z2_v[n, 2 * j + c, pl.ds(FT * r, rows), :] for j in range(NB)], axis=1)

                def both(c, op):
                    top = part(0, c, FT)
                    return jnp.concatenate([op(top[:FB], part(1, 1, FB)), top[FB:]], axis=0)

                return (lambda: both(0, jnp.add), lambda: part(1, 0, FB) + part(1, 1, FB),
                        lambda: part(0, 0, FT), lambda: part(1, 1, FB),
                        lambda: part(0, 0, FT) + part(0, 1, FT), lambda: part(1, 0, FB) - part(0, 0, FB),
                        lambda: both(1, jnp.subtract))[k]().astype(BF16)

            b11, b12, b21, b22 = (
                jnp.concatenate([rhs[2 * j + c][128 * r:128 * r + 128] for j in range(NB)], axis=1)
                for c in (0, 1) for r in (0, 1))
            m = lambda k, x: _nt(left(k), x.astype(BF16))
            m2, m5, m4 = m(1, b11), m(4, b22), m(3, b21 - b11)
            m1, m7, m3, m6 = m(0, b11 + b22), m(6, b21 + b22), m(2, b12 - b22), m(5, b11 + b12)
            c11 = jnp.concatenate([m4 - m5[:FB], -m5[FB:]], axis=0) + m1 + m7
            c22 = (m1[:FB] - m2) + m3[:FB] + m6
            return jnp.concatenate([jnp.concatenate([c11, m5 + m3], axis=1),
                                    jnp.concatenate([m2 + m4, c22], axis=1)], axis=0)

        def gate(r, c, g):
            tiles = [i * T2 + c * (H // 128) + t for t in range(H // 128)]
            bias = jnp.concatenate([bf_v[pl.ds(j, 1), :] for j in tiles], axis=1)
            z1 = jnp.concatenate([z1_v[j, pl.ds(FM * r, FM), :] for j in tiles], axis=1)
            return _gelu_scaled(z1) * (g + bias)

        s2 = prod(1, w(0, 0))
        s5 = prod(4, w(1, 1))
        s4 = prod(3, comb(w(1, 0), w(0, 0), -1))
        p21 = gate(1, 0, s2 + s4)
        d11 = s4 - s5
        s1 = prod(0, comb(w(0, 0), w(1, 1), 1))
        d11, d22 = d11 + s1, s1 - s2
        p11 = gate(0, 0, d11 + prod(6, comb(w(1, 0), w(1, 1), 1)))
        s3 = prod(2, comb(w(0, 1), w(1, 1), -1))
        p12 = gate(0, 1, s3 + s5)
        p22 = gate(1, 1, (d22 + s3) + prod(5, comb(w(0, 0), w(0, 1), 1)))
        return [jnp.concatenate(p, axis=0) for p in ((p11, p21), (p12, p22))]

    def flush(k):
        rows = _ds(k * FL, FL, FL)
        return pltpu.make_async_copy(o_v.at[rows], o_h.at[rows], osem.at[k])

    def mix_step(i):
        mixing(i).wait()

        @pl.when(i + 1 < S // R2)
        def _():
            mixing(i + 1).start()

        p = mix(i)
        b11, b12, b21, b22 = (p[c][128 * KO * r:128 * KO * (r + 1)] for r in (0, 1) for c in (0, 1))

        def prod(n, rhs):
            return _nn(jnp.concatenate([_ld(wt_v, n, j) for j in range(KO)], axis=1), rhs.astype(BF16))

        def rest(c):
            tail = jnp.concatenate([p[c][256 * KO:], jnp.zeros((128 + 256 * KO - FH, H), F32)], axis=0)
            return _nn(_ld(wr_v), tail.astype(BF16))

        def finish(c, ot):
            for t in range(H // 128):
                rows = _ds(i * R2 + c * H + 128 * t, 128, 128)
                o = ot[:, 128 * t:128 * t + 128].T
                o_v[rows, :] = (x1_v[rows, :] + jnp.concatenate([gb] * 8, axis=0) * o).astype(BF16)
                done = c * H + 128 * (t + 1)
                if done % FL == 0:
                    flush(i * (R2 // FL) + done // FL - 1).start()

        r0 = rest(0)
        s2 = prod(1, b11)
        s4 = prod(3, b21 - b11)
        s5 = prod(4, b22)
        s1 = prod(0, b11 + b22)
        s7 = prod(6, b21 + b22)
        finish(0, jnp.concatenate([r0[:DM] + s4 - s5 + s1 + s7, r0[DM:] + s2 + s4], axis=0))
        r1 = rest(1)
        s3 = prod(2, b12 - b22)
        s6 = prod(5, b11 + b12)
        finish(1, jnp.concatenate([r1[:DM] + s5 + s3, (s1 - s2) + r1[DM:] + s3 + s6], axis=0))

    if UR:
        for i in range(S // R2):
            mix_step(i)
    else:
        pl.loop(0, S // R2)(mix_step)
    for k in range(S // FL):
        flush(k).wait()


@jax.jit
def pallas_adaLN_cond__ssm_conv_h3__mixer_gmlp__prompt_kernel(
    A_q, A_k, A_v, A_shift_k, A_ssm_k, A_ssm_D, B_x, B_w_in, B_w_sp, B_b_sp, B_w_out, c, w_mod,
):
    del B_x
    vf = _dft_mats().astype(BF16)
    vm = pltpu.VMEM
    tile = (128, 128)
    scratch = [
        vm((S, D), BF16), vm((NCB, PAD + S, 128), BF16), vm((NCB, S, 128), BF16), vm((TAPS, D), BF16),
        vm((NCB, NA, 128, CH), BF16), vm((NCB, 128), BF16), vm((2 * FH, D), BF16),
        vm((2, R2, S), BF16), vm((S // 128, 128), BF16), vm((256 * KO + 128, D), BF16), vm((1, D), BF16),
        vm((D, 6 * D), BF16), vm((16, *tile), BF16),
        vm((8, 2 * NA, *tile), BF16), vm((8, 2 * NA, *tile), BF16),
        vm((2 * NA, *tile), F32), vm((2 * NA, *tile), F32), vm((NA, *tile), BF16), vm((NA, *tile), BF16),
        vm((16, NA, *tile), F32), vm((16, NA, *tile), F32), vm((5, NA, *tile), F32), vm((5, NA, *tile), F32),
        vm((NCB, S, 128), F32), vm((S, D), F32), vm((NCB, RB, 128), BF16),
        vm((S // 128, FH, 128), F32), vm((7, S // 256, FM, 128), F32),
        vm((7, KO, DM, 128), BF16), vm((D, 128), BF16), vm((S // 128, 128), F32),
        vm((S, D), BF16), vm((8, 128), jnp.int32), pltpu.SMEM((1,), jnp.int32),
        pltpu.SemaphoreType.DMA((NCB * NA + 32,)),
        pltpu.SemaphoreType.DMA((S // FL,)),
    ] + [vm((FH, 128), F32)] * 16 + [vm((FH // SU * 16, 128), F32)] * 16 + [vm((2, H, 128), BF16)] * 18
    out = pl.pallas_call(
        _kernel,
        out_shape=jax.ShapeDtypeStruct((S, D), BF16),
        in_specs=[pl.BlockSpec(memory_space=pltpu.HBM)] * 13,
        out_specs=pl.BlockSpec(memory_space=pltpu.HBM),
        scratch_shapes=scratch,
        compiler_params=pltpu.CompilerParams(vmem_limit_bytes=110 * 1024 * 1024),
    )(A_q.reshape(S, D), A_k.reshape(S, D), A_v.reshape(S, D), A_shift_k.T, A_ssm_k,
      A_ssm_D.reshape(NCB, 128), B_w_in.T, B_w_sp, B_b_sp.reshape(S // 128, 128), B_w_out, c, w_mod, vf)
    return out.reshape(1, S, D)
```

```python
import functools
import math

import numpy as np
import jax
import jax.numpy as jnp
from jax import lax
import jax.experimental.pallas as pl
import jax.experimental.pallas.tpu as pltpu

S, D, FH = 2048, 640, 864
FM, DM = FH // 2, D // 2
KO = FH // 256
FT, FB = 224, 208
TAPS = 4
CH = 512
NA = S // CH
N2 = 64
N1 = CH // N2
NCB = D // 128
RB = 512
NB = S // RB
H = RB // 2
EPS = 1e-5
F32, BF16, U32 = jnp.float32, jnp.bfloat16, jnp.uint32
PAD = 16

_C8 = math.cos(math.pi / 8)
_T8 = math.tan(math.pi / 8)
_R2 = math.sqrt(0.5)
_G0 = math.sqrt(2 / math.pi)
_GA = (_G0 * 0.044715) ** (1 / 3)

UN = 1
DG = 0
E0, ES = 0, 16
MA = 2
MS = 22
TU = (-1, 0, 3, 5, 16, 32, 35, 38)
TK = (34, 38, 41, 42, 43, 44, 45, 46)
TI = (-1, -1, -1, -1, -1, -1, -1, -1, 0, 2, 4, 6, 16, 17, 32, 33, 34, 35, 36, 37, 38, 39, 40, 41)
SU = 96
NJ = ["s0:76:105,s1:114:170,s2:168:205,m14:60:100,m18:100:140,m15:140:175,m19:165:200", "h3:0:96,h2:104:229,s3:20:80",
      "h5:0:108:132:186,h4:192:246:324:440,s4:330:402,s6:216:270",
      "h7:0:108:162:216,h6:226:280:324:440,s5:0:54,s7:54:108,s8:324:372,s10:216:270",
      "n0:0:50,n1:30:80,n2:70:108,s9:0:40,s11:40:80,n3:110:170,n4:160:216,n5:216:270,s14:170:216,s15:220:270,n7:280:340,s12:330:378,s13:380:410,n6:420:480"]
R2 = 512


def _dft_mats():
    ang = [1 / 16 + m / 4 for m in range(4)] + [1 / 8, 1 / 8 + 1 / 2, 1 / 4]
    idx = np.arange(128)
    pos = (idx // 16) * 8 + idx % 8
    part = (idx // 8) % 2
    mats = []
    for b, a in enumerate(ang):
        th = 2 * np.pi * (a + pos[:, None]) * pos[None, :] / N2
        po, pi = part[:, None], part[None, :]
        m = np.where(po == pi, np.cos(th), np.where(po == 1, np.sin(th), -np.sin(th)))
        mats.append(m * ((_C8 if b < 4 else 1.0) / 8))
    n = pos + 64 * part
    th = 2 * np.pi * pos[:, None] * n[None, :] / 128
    m = np.where(part[:, None] == 0, np.cos(th), np.sin(th))
    m[8, :] = 1.0 - 2.0 * (n % 2)
    mats.append(m / 8)
    fwd = np.stack(mats).astype(np.float32)
    n = idx // 32 * 16 + idx % 8 * 2 + idx // 16 % 2
    return fwd[:, :, n // 8 * 16 + part * 8 + n % 8]


def _outer_fwd(u):
    t0r, t0i = u[0] * (1 / _C8), u[4] * (1 / _C8)
    t2r, t2i = (u[2] - u[6]) * (_R2 / _C8), (u[2] + u[6]) * (_R2 / _C8)
    t1r, t1i = u[1] - _T8 * u[5], u[5] + _T8 * u[1]
    t3r, t3i = _T8 * u[3] - u[7], _T8 * u[7] + u[3]
    ar, ai, br, bi = t0r + t2r, t0i + t2i, t0r - t2r, t0i - t2i
    cr, ci, dr, di = t1r + t3r, t1i + t3i, t1r - t3r, t1i - t3i
    out = [(ar + cr, ai + ci), (br - di, bi + dr), (ar - cr, ai - ci), (br + di, bi - dr)]
    p = [u[j] + u[j + 4] for j in range(4)]
    q = [u[j] - u[j + 4] for j in range(4)]
    er, ei = (q[1] - q[3]) * _R2, (q[1] + q[3]) * _R2
    out += [(q[0] + er, q[2] + ei), (q[0] - er, q[2] - ei)]
    out += [(p[0] - p[2], p[1] - p[3]), (p[0] + p[2], p[1] + p[3])]
    return out


def _outer_inv(B):
    ar, ai = B[0][0] + B[2][0], B[0][1] + B[2][1]
    cr, ci = B[0][0] - B[2][0], B[0][1] - B[2][1]
    br, bi = B[1][0] + B[3][0], B[1][1] + B[3][1]
    dr, di = B[1][0] - B[3][0], B[1][1] - B[3][1]
    g0r, g0i, g2r, g2i = ar + br, ai + bi, ar - br, ai - bi
    g1r, g1i, g3r, g3i = cr + di, ci - dr, cr - di, ci + dr
    nr = [g0r * (1 / _C8), g1r + _T8 * g1i, (g2r + g2i) * (_R2 / _C8), _T8 * g3r + g3i]
    ni = [g0i * (1 / _C8), g1i - _T8 * g1r, (g2i - g2r) * (_R2 / _C8), _T8 * g3i - g3r]
    fr, fi = B[4][0] - B[5][0], B[4][1] - B[5][1]
    q = [B[4][0] + B[5][0], (fr + fi) * _R2, B[4][1] + B[5][1], (fi - fr) * _R2]
    p = [B[7][0] + B[6][0], B[7][1] + B[6][1], B[7][0] - B[6][0], B[7][1] - B[6][1]]
    return ([p[j] + q[j] + nr[j] for j in range(4)]
            + [p[j] - q[j] + ni[j] for j in range(4)])


def _gelu_scaled(x):
    t = jnp.tanh(x * (_G0 / _GA + x * x))
    return x + x * t


def _norm_stats(s1, s2, n, eps):
    m = s1 * (1.0 / n)
    return m, jnp.exp(-0.5 * jnp.log(jnp.maximum(s2 * (1.0 / n) - m * m, 0.0) + eps))


def _ln_rows(x):
    m, r = _norm_stats(jnp.sum(x, axis=-1, keepdims=True), jnp.sum(x * x, axis=-1, keepdims=True),
                       x.shape[-1], EPS)
    return (x - m) * r


def _lhs7(a11, a12, a21, a22):
    return a11 + a22, a21 + a22, a11, a22, a11 + a12, a21 - a11, a12 - a22


def _ld(ref, *idx):
    return pltpu.bitcast(ref.bitcast(jnp.uint32)[idx or ...], BF16)


def _whole(x):
    return x


def _phase(words, odd):
    return pltpu.bitcast(words & np.uint32(0xFFFF0000) if odd else words << 16, F32)


def _nn(a, b):
    return jnp.dot(a, b, preferred_element_type=F32)


def _nt(a, b):
    return lax.dot_general(a, b, (((1,), (1,)), ((), ())), preferred_element_type=F32)


def _ds(start, size, align):
    return pl.ds(start if isinstance(start, int) else pl.multiple_of(start, align), size)


def _add(xs):
    return functools.reduce(lambda x, y: x + y, xs)


def _kernel(q_h, k_h, v_h, sh_h, sk_h, sd_h, wi_h, ws_h, b_h, wo_h, c_h, wm_h, vf_h, o_h,
            q_v, k_v, v_v, sh_v, sk_v, sd_v, wi_v, ws_v, b_v, wo_v, c_v, wm_v, vf_v,
            au0_v, au1_v, fa_v, fb_v, ya_v, yb_v, bm0_v, bp0_v, bm1_v, bp1_v,
            y_v, x1_v, h0_v, z1_v, z2_v, wt_v, wr_v, bf_v, o_v, tie_v, zero_s,
            sems, osem, *lists):
    au_v, h_v = (au0_v, au1_v), (lists[32:41], lists[41:])
    copies = {}

    def start(name, src, dst):
        copies[name] = pltpu.make_async_copy(src, dst, sems.at[NCB * NA + len(copies)])
        copies[name].start()

    def wait(*names):
        for name in names:
            copies[name].wait()

    def conv_inputs(cb, a):
        rows, lanes, sem = _ds(a * CH, CH, CH), pl.ds(cb * 128, 128), sems.at[cb * NA + a]
        return (pltpu.make_async_copy(k_h.at[rows, lanes], k_v.at[cb, _ds(PAD + a * CH, CH, PAD)], sem),
                pltpu.make_async_copy(v_h.at[rows, lanes], v_v.at[cb, rows], sem),
                pltpu.make_async_copy(sk_h.at[lanes, rows], sk_v.at[cb, a], sem))

    def fetch(stage):
        if stage < NCB:
            for a in range(NA):
                for cp in conv_inputs(stage, a):
                    cp.start()
        if stage == 0:
            start("vf", vf_h, vf_v.at[pl.ds(0, 8)])
        if stage == NCB:
            start("c", c_h, c_v)
            start("wm", wm_h.at[:, pl.ds(0, 5 * D)], wm_v.at[:, pl.ds(0, 5 * D)])
            start("q0", q_h.at[pl.ds(0, H)], q_v.at[pl.ds(0, H)])
            start("w2", wi_h.at[pl.ds(FH, FH)], wi_v.at[pl.ds(0, FH)])
            start("q1", q_h.at[pl.ds(H, RB - H)], q_v.at[pl.ds(H, RB - H)])
            start("w1", wi_h.at[pl.ds(0, FH)], wi_v.at[pl.ds(FH, FH)])
            start("q2", q_h.at[pl.ds(RB, S - RB)], q_v.at[pl.ds(RB, S - RB)])
        if stage == NCB + 2:
            start("wg", wm_h.at[:, pl.ds(5 * D, D)], wm_v.at[:, pl.ds(5 * D, D)])
            start("b", b_h, b_v)
            start("wo", wo_h, wo_v.at[pl.ds(0, FH)])
            start("ws", ws_h, ws_v)

    start("sh", sh_h, sh_v)
    start("sd", sd_h, sd_v)
    fetch(0)
    fetch(1)
    for ref in (fb_v, ya_v, tie_v):
        ref[...] = jnp.zeros(ref.shape, ref.dtype)
    k_v[:, pl.ds(0, PAD), :] = jnp.zeros((NCB, PAD, 128), BF16)
    wo_v[pl.ds(FH, 256 * KO + 128 - FH), :] = jnp.zeros((256 * KO + 128 - FH, D), BF16)
    zero_s[0] = 0
    row8 = lax.broadcasted_iota(jnp.int32, (8, 128), 0)

    def tie(after, x):
        if after is None:
            return x
        never = jnp.concatenate([tie_v[...]] * (x.shape[0] // 8), axis=0) != 0
        return jnp.where(never, after, x)

    def put(cb, slot, g, res):
        for b in range(8):
            au_v[cb % 2][b, slot, pl.ds(16 * g, 16), :] = jnp.concatenate(res[b], axis=0).astype(BF16)

    def split_filter(cb, a, after):
        kt = pltpu.bitcast(sk_v[cb, a].T, U32)
        for g in range(N2 // 8):
            u = [_phase(kt[j * N2 // 2 + g // 2 * 8:j * N2 // 2 + g // 2 * 8 + 8], g % 2) for j in range(N1)]
            if g == 0:
                u[0] = u[0] + jnp.where(row8 + a == 0, sd_v[...].astype(F32)[cb:cb + 1], 0.0)
            u[:4] = [tie(after(g), x) for x in u[:4]]
            put(cb, NA + a, g, _outer_fwd(u))

    def split_signal(cb, a, after):
        keys, vals = k_v.bitcast(U32), v_v.bitcast(U32)
        taps = [jnp.broadcast_to(sh_v[j:j + 1, pl.ds(cb * 128, 128)].astype(F32), (8, 128))
                for j in range(TAPS)]
        base = a * (CH // 2) if isinstance(a, int) else pl.multiple_of(a * (CH // 2), CH // 2)
        for g in range(N2 // 8):
            w = [tie(after(g), t) for t in taps]
            u = []
            for j in range(N1):
                r = base + j * N2 // 2 + g // 2 * 8
                lag = [_phase(keys[cb, pl.ds(r + PAD // 2 + (g % 2 - t) // 2, 8), :], (g % 2 - t) % 2)
                       for t in range(TAPS)]
                u.append(_add([x * wt for x, wt in zip(lag, w)]) * _phase(vals[cb, pl.ds(r, 8), :], g % 2))
            put(cb, a, g, _outer_fwd(u))

    def spectra(cb, b, half, f_ref):
        rhs = jnp.concatenate([_ld(au_v[cb % 2], b, half * NA + a) for a in range(NA)], axis=1)
        f = _nn(_ld(vf_v, b), rhs)
        for a in range(NA):
            f_ref[half * NA + a] = f[:, 128 * a:128 * a + 128]
        return f

    def product(f_ref, y_ref, plus, real_rows=None):
        for g in range(8):
            ur, ui, kr, ki = ([f_ref[o + a, pl.ds(16 * g + 8 * c, 8), :] for a in range(NA)]
                              for o in (0, NA) for c in (0, 1))
            kr, ki = ([k[0]] + [k[a] + k[a - 1] if plus else k[a] - k[a - 1] for a in range(1, NA)]
                      for k in (kr, ki))
            for a in range(NA):
                yi = _add([kr[j] * ui[a - j] + ki[j] * ur[a - j] for j in range(a + 1)])
                if real_rows is not None and g == 0:
                    rr = _add([kr[j] * ur[a - j] for j in range(a + 1)])
                    ii = _add([ki[j] * ui[a - j] for j in range(a + 1)])
                    yr = jnp.where(real_rows, 0.5 * rr, rr - ii)
                    yi = jnp.where(real_rows, 0.5 * ii, yi)
                else:
                    yr = _add([kr[j] * ur[a - j] - ki[j] * ui[a - j] for j in range(a + 1)])
                y_ref[a, pl.ds(16 * g, 16), :] = jnp.concatenate([yr, yi], axis=0).astype(BF16)

    def residues(y_ref, b, dst):
        r = _nn(_ld(vf_v, 8 + b), jnp.concatenate([_ld(y_ref, a) for a in range(NA)], axis=1))
        for a in range(NA):
            dst[a] = r[:, 128 * a:128 * a + 128]
        return r

    def stash(t):
        return ((bm0_v.at[t], bp0_v.at[t]) if t < 16 else (bm1_v.at[t - 16], bp1_v.at[t - 16]))

    def merge(cb, a, after=lambda g: None):
        src = [stash(1 + 4 * cb + b)[s] for s in (0, 1) for b in range(4)]
        for g in range(N2 // 8):
            res = [[ref[a, pl.ds(16 * g + 8 * c, 8), :] for c in (0, 1)] for ref in src]
            res[0] = [tie(after(g), x) for x in res[0]]
            res[1] = [tie(after(g), x) for x in res[1]]
            for j, y in enumerate(_outer_inv(res)):
                y_v[cb, _ds(a * CH + j * N2 + 8 * g, 8, 8), :] = y

    def transform(cb, a, dst, active=True):
        pa = (a + 3) % 4
        res = []
        if active:
            res += [spectra(cb, a, 1, fa_v), spectra(cb, a, 0, fa_v)]
        product(fb_v, yb_v, True, row8 + (3 - pa) == 0)
        res.append(residues(ya_v, pa, dst[0]))
        if active:
            res += [spectra(cb, 4 + a, 1, fb_v), spectra(cb, 4 + a, 0, fb_v)]
            product(fa_v, ya_v, False)
        res.append(residues(yb_v, 4 + pa, dst[1]))
        return res

    def conv_step(cb, i):
        steps = [UN * i + u for u in range(UN)]
        if cb < NCB:
            for a in steps:
                for cp in conv_inputs(cb, a):
                    cp.wait()
        done = []
        for a in steps if cb else ():
            done += transform(cb - 1, a, (bm0_v.at[4 * cb - 4 + a], bp0_v.at[4 * cb - 4 + a])
                              if cb < NCB else (bm1_v.at[a], bp1_v.at[a]))
        at = lambda p: done[p // 8][16 * (p % 8):16 * (p % 8) + 8, 0:128] if done and p >= 0 else None
        for u, a in enumerate(steps):
            if cb < NCB:
                split_signal(cb, a, lambda g: at(TU[8 * u + g]))
                split_filter(cb, a, lambda g: at(TK[8 * u + g]))
            else:
                for c in range(3):
                    merge(c, a, lambda g: at(TI[24 * u + 8 * c + g]))

    wait("sh", "sd")
    for cb in range(NCB + 1):
        if cb == 1:
            wait("vf")
            row, col = (lax.broadcasted_iota(jnp.int32, (128, 128), d) for d in (0, 1))
            n = (col >> 5) * 16 + (col & 7) * 2 + ((col >> 4) & 1)
            order = jnp.where(row == (n >> 3) * 16 + (col & 8) + (n & 7), 1.0, 0.0).astype(BF16)
            for b in range(8):
                vf_v[8 + b] = _nt(order, vf_v[b]).astype(BF16)
        fetch(cb + 2)
        pl.loop(0, NA // UN)(functools.partial(conv_step, cb))

    wait("c", "wm")
    transform(NCB, 0, stash(20), active=False)
    cc = c_v[...].astype(F32)
    sc = jnp.broadcast_to(cc / (1.0 + jnp.exp(-cc)), (16, D)).astype(BF16)
    mod = _nn(sc, wm_v[:, pl.ds(0, 5 * D)])[0:8]
    sa, ca, ga, sb, cb_ = (mod[:, i * D:(i + 1) * D] for i in range(5))
    m1, m0 = ga * (1.0 + ca), ga * sa
    n1, n0 = _GA * (1.0 + cb_), _GA * sb
    zero = zero_s[0]
    for n, (cb, a) in enumerate([(cb, a) for cb in (3, 4) for a in range(MA)]):
        merge(cb, a + zero, lambda g: mod[:, 128 * ((8 * n + g) * MS // (16 * MA)):][:, :128])

    TB = RB // 128
    PER = 2 * FH // 16

    def hidden(r0, after=(None, None)):
        out = []
        for r, a in zip((r0, r0 + 8), after):
            rows = pl.ds(r, 8)
            x = q_v[rows, :].astype(F32)
            x = jnp.concatenate([tie(a, x[:, :128]), x[:, 128:]], axis=1)
            x1 = x + (_ln_rows(x) * m1 + m0) * jnp.concatenate([y_v[j, rows, :] for j in range(NCB)], axis=1)
            x1_v[rows, :] = x1
            out.append(_ln_rows(x1) * n1 + n0)
        return jnp.concatenate(out, axis=0)

    def keep_gate(tile, z):
        lists[tile][pl.ds(zero, FH), :] = z

    def moments(tile, after):
        z, acc = lists[tile], lists[16 + tile]
        s1 = s2 = None
        for n, f in enumerate(range(0, FH, SU)):
            for r in range(f, f + SU, 8):
                d = tie(after(n)[:8] if r == f else None, z[pl.ds(r, 8), :])
                s1, s2 = (d, d * d) if s1 is None else (s1 + d, s2 + d * d)
            acc[pl.ds(16 * n + zero, 16), :] = jnp.concatenate([s1, s2], axis=0)
        s1, s2 = (jnp.sum(acc[pl.ds(16 * n + r, 8), :], axis=0, keepdims=True) for r in (0, 8))
        stats[tile] = [jnp.broadcast_to(t, (16, 128)) for t in _norm_stats(s1, s2, FH, EPS * (2 * _GA) ** 2)]

    def norm_gate(pair, after):
        for n in range(FM // 16):
            means = [tie(after(n), stats[2 * pair + c][0]) for c in (0, 1)]
            quad = [(lists[2 * pair + c][pl.ds(r + 16 * n, 16), :] - means[c]) * stats[2 * pair + c][1]
                    for r in (0, FM) for c in (0, 1)]
            for k, a in enumerate(_lhs7(*quad)):
                z2_v[k, pair, pl.ds(16 * n, 16), :] = a

    def lanes(x, j, n=1):
        return x[:, 128 * j:128 * (j + n)]

    def prepare(i, c, after):
        def put(k, n, x):
            for j in range(x.shape[1] // 128):
                h_v[i % 2][k][j, pl.ds(16 * n + zero, 16), :] = lanes(x, j).astype(BF16)

        for n in range(H // 16):
            h = hidden(i * RB + c * H + 16 * n, (after(2 * n)[:8], after(2 * n + 1)[:8]))
            top, bot = lanes(h, 0, 2), lanes(h, 2, 2)
            put(7 + c, n, lanes(h, 4))
            if c:
                half[n] = top, bot
                put(2, n, top - bot)
                put(4, n, bot)
            else:
                put(1, n, top)
                put(3, n, bot - top)
                put(0, n, top + half[n][1])
                put(5, n, top + half[n][0])
                put(6, n, bot + half[n][1])

    def side_jobs(plan, at):
        for job in plan.split(","):
            if job:
                kind, (n, *spans) = job[0], (int(x) for x in job[1:].split(":"))
                total = {"s": FH // SU, "n": FM // 16, "h": H // 8, "m": N2 // 8}[kind]
                slots = [p for lo, hi in zip(spans[::2], spans[1::2]) for p in range(lo, hi)]
                after = lambda k: at(slots[k * len(slots) // total])
                if kind == "s":
                    moments(n, after)
                elif kind == "m":
                    merge(n // NA, n % NA + zero, lambda k: after(k)[:8])
                elif kind == "n":
                    norm_gate(n, after)
                else:
                    prepare(n // 2, n % 2, after)

    def rows_of(z):
        per = z.shape[0] // 16
        return lambda p: z[16 * (p % per):16 * (p % per) + 16, 128 * (p // per):128 * (p // per) + 128]

    def project(i):
        def prod(*pairs):
            right = [_ld(h_v[i % 2][k], j) for _, k in pairs for j in range(2 if k < 7 else 1)]
            return _nt(jnp.concatenate([x for k, _ in pairs for x in left[k]], axis=1),
                       jnp.concatenate(right, axis=1))

        s5, s3, r12, s4, s1 = prod((4, 4)), prod((2, 2)), prod((7, 8)), prod((3, 3)), prod((0, 0))
        s7, s2, r21, s6 = prod((6, 6), (7, 7)), prod((1, 1)), prod((8, 7)), prod((5, 5), (8, 8))
        gate = [((s4 - s5) + s1) + s7, (s5 + s3) + r12]
        value = [(s4 + s2) + r21, ((s3 + s1) - s2) + s6]
        for c, later in enumerate((s2, lanes(s4, 1))):
            keep_gate(i * TB + 2 * c, _gelu_scaled(lanes(gate[c], 0)))
            keep_gate(i * TB + 2 * c + 1, _gelu_scaled(tie(lanes(later, 0) if DG else None, lanes(gate[c], 1))))
        for t in range(TB):
            z1_v[i * TB + t] = lanes(value[t // 2], t % 2)
        rounds = (s5, s3, gate[1], lanes(s4, 1), lanes(s1, 1), gate[0], s2, value[0], lanes(value[1], 1))
        return lambda p: rounds[p // (FH // 16)][16 * (p % (FH // 16)):16 * (p % (FH // 16)) + 16, 0:128]

    def first(f0, r0, n, k0, k1):
        h = jnp.concatenate([_ld(h0_v, j, pl.ds(r0 // 2, n // 2)) for j in range(k0, k1)], axis=1)
        return _nt(wi_v[pl.ds(f0, FH), pl.ds(128 * k0, 128 * (k1 - k0))], h)

    def keep_first(r, h):
        for j in range(NCB):
            h0_v[j, pl.ds(r, 16), :] = lanes(h, j).astype(BF16)

    stats, half = {}, {}
    wait("q0")
    for r in range(0, H, 16):
        keep_first(r, hidden(r))
    wait("w2", "q1")
    zero = pl.multiple_of(zero_s[0], 16)
    head = first(0, 0, H, 0, 2)
    z = _gelu_scaled(head + first(0, 0, H, 2, NCB))
    at = rows_of(jnp.concatenate([lanes(head, 0), z], axis=1))
    for n in range(H // 16):
        keep_first(H + 16 * n, hidden(H + 16 * n, [at(E0 + (2 * n + k) * ES // 8)[:8] for k in (0, 1)]))
    z = jnp.concatenate([z] + [_gelu_scaled(first(0, r, 128, 0, NCB)) for r in (H, H + 128)], axis=1)
    for t in range(TB):
        keep_gate(t, lanes(z, t))
    side_jobs(NJ[0], rows_of(z))
    wait("w1", "q2")
    head = first(FH, 0, RB, NCB - 1, NCB)
    z = head + first(FH, 0, RB, 0, NCB - 1)
    for t in range(TB):
        z1_v[t] = lanes(z, t)
    side_jobs(NJ[1], rows_of(jnp.concatenate([lanes(head, 0), z], axis=1)))
    sums = [_lhs7(*(wi_v[pl.ds(FH * r, FH), pl.ds(256 * c + 128 * j, 128)].astype(F32)
                    for r in (0, 1) for c in (0, 1))) for j in (0, 1)]
    left = ([[s[k].astype(BF16) for s in sums] for k in range(7)]
            + [[_whole(wi_v[pl.ds(FH * r, FH), pl.ds(512, 128)])] for r in (0, 1)])
    for i in range(1, NB):
        side_jobs(NJ[i + 1], project(i))

    wait("wg", "b", "wo", "ws")
    gb = _nn(sc, wm_v[:, pl.ds(5 * D, D)]) * (0.5 / _GA)
    bf_v[...] = b_v[...].astype(F32)
    for j in range(KO):
        a1, a2 = (wo_v[pl.ds(128 * (j + KO * c), 128), :].T.astype(F32) for c in (0, 1))
        for n, a in enumerate(_lhs7(a1[:DM], a2[:DM], a1[DM:], a2[DM:])):
            wt_v[n, j] = a.astype(BF16)
    wr_v[...] = wo_v[pl.ds(256 * KO, 128), :].T
    T2 = R2 // 128

    def mix(i):
        def w(c, r):
            return [ws_v[_ds(i * R2 + r * H, H, H), pl.ds(256 * j + 128 * c, 128)].astype(F32) for j in range(S // 256)]

        def comb(x, y, sign):
            return [a + b if sign > 0 else a - b for a, b in zip(x, y)]

        def prod(n, rhs):
            def left(k):
                def part(r, c, rows):
                    return jnp.concatenate([z2_v[n, 2 * j + c, pl.ds(FT * r, rows), :] for j in range(NB)], axis=1)

                def both(c, op):
                    top = part(0, c, FT)
                    return jnp.concatenate([op(top[:FB], part(1, 1, FB)), top[FB:]], axis=0)

                return (lambda: both(0, jnp.add), lambda: part(1, 0, FB) + part(1, 1, FB),
                        lambda: part(0, 0, FT), lambda: part(1, 1, FB),
                        lambda: part(0, 0, FT) + part(0, 1, FT), lambda: part(1, 0, FB) - part(0, 0, FB),
                        lambda: both(1, jnp.subtract))[k]().astype(BF16)

            b11, b12, b21, b22 = (
                jnp.concatenate([rhs[2 * j + c][128 * r:128 * r + 128] for j in range(NB)], axis=1)
                for c in (0, 1) for r in (0, 1))
            m = lambda k, x: _nt(left(k), x.astype(BF16))
            m2, m5, m4 = m(1, b11), m(4, b22), m(3, b21 - b11)
            m1, m7, m3, m6 = m(0, b11 + b22), m(6, b21 + b22), m(2, b12 - b22), m(5, b11 + b12)
            c11 = jnp.concatenate([m4 - m5[:FB], -m5[FB:]], axis=0) + m1 + m7
            c22 = (m1[:FB] - m2) + m3[:FB] + m6
            return jnp.concatenate([jnp.concatenate([c11, m5 + m3], axis=1),
                                    jnp.concatenate([m2 + m4, c22], axis=1)], axis=0)

        def gate(r, c, g):
            tiles = [i * T2 + c * (H // 128) + t for t in range(H // 128)]
            bias = jnp.concatenate([bf_v[pl.ds(j, 1), :] for j in tiles], axis=1)
            z1 = jnp.concatenate([z1_v[j, pl.ds(FM * r, FM), :] for j in tiles], axis=1)
            return _gelu_scaled(z1) * (g + bias)

        s2 = prod(1, w(0, 0))
        s5 = prod(4, w(1, 1))
        s4 = prod(3, comb(w(1, 0), w(0, 0), -1))
        p21 = gate(1, 0, s2 + s4)
        d11 = s4 - s5
        s1 = prod(0, comb(w(0, 0), w(1, 1), 1))
        d11, d22 = d11 + s1, s1 - s2
        p11 = gate(0, 0, d11 + prod(6, comb(w(1, 0), w(1, 1), 1)))
        s3 = prod(2, comb(w(0, 1), w(1, 1), -1))
        p12 = gate(0, 1, s3 + s5)
        p22 = gate(1, 1, (d22 + s3) + prod(5, comb(w(0, 0), w(0, 1), 1)))
        return [jnp.concatenate(p, axis=0) for p in ((p11, p21), (p12, p22))]

    def flush(k):
        rows = _ds(k * H, H, H)
        return pltpu.make_async_copy(o_v.at[rows], o_h.at[rows], osem.at[k])

    def finish(r0, tile):
        for t in range(H // 128):
            for j in range(NCB):
                at = _ds(r0 + 128 * t, 128, 128), pl.ds(128 * j, 128)
                o_v[at] = (x1_v[at] + jnp.concatenate([lanes(gb, j)] * 8, axis=0)
                           * tile(t, j).T.astype(F32)).astype(BF16)

    def mix_step(i):
        p = mix(i)
        b11, b12, b21, b22 = (p[c][128 * KO * r:128 * KO * (r + 1)] for r in (0, 1) for c in (0, 1))

        def prod(n, rhs):
            return _nn(jnp.concatenate([_ld(wt_v, n, j) for j in range(KO)], axis=1), rhs.astype(BF16))

        def rest(c):
            tail = jnp.concatenate([p[c][256 * KO:], jnp.zeros((128 + 256 * KO - FH, H), F32)], axis=0)
            return _nn(_ld(wr_v), tail.astype(BF16))

        r0 = rest(0)
        s2 = prod(1, b11)
        s4 = prod(3, b21 - b11)
        s5 = prod(4, b22)
        s1 = prod(0, b11 + b22)
        s7 = prod(6, b21 + b22)
        ot = jnp.concatenate([r0[:DM] + s4 - s5 + s1 + s7, r0[DM:] + s2 + s4], axis=0)
        finish(i * R2, lambda t, j: lanes(ot, t)[128 * j:128 * j + 128].astype(BF16))
        flush(2 * i).start()
        spot = _ds(i * R2 + H, 16, 16), pl.ds(0, 128)
        o_v[spot] = jnp.zeros((16, 128), BF16)
        pin = o_v[_ds(i * R2 + H + zero, 16, 16), pl.ds(0, 128)].astype(F32)
        r1 = rest(1)
        s3 = prod(2, b12 - b22)
        b = b11 + b12
        b = jnp.concatenate([b[:-16], jnp.concatenate([b[-16:, :128], tie(pin, b[-16:, 128:])], axis=1)], axis=0)
        s6 = prod(5, b)
        ot = jnp.concatenate([r1[:DM] + s5 + s3, (s1 - s2) + r1[DM:] + s3 + s6], axis=0)
        finish(i * R2 + H, lambda t, j: lanes(ot, t)[128 * j:128 * j + 128].astype(BF16))
        flush(2 * i + 1).start()

    zero = pl.multiple_of(zero_s[0], 16)
    zero = zero_s[0]
    pl.loop(0, S // R2)(mix_step)
    for k in range(S // H):
        flush(k).wait()


@jax.jit
def pallas_adaLN_cond__ssm_conv_h3__mixer_gmlp__prompt_kernel(
    A_q, A_k, A_v, A_shift_k, A_ssm_k, A_ssm_D, B_x, B_w_in, B_w_sp, B_b_sp, B_w_out, c, w_mod,
):
    del B_x
    vf = _dft_mats().astype(BF16)
    vm = pltpu.VMEM
    tile = (128, 128)
    scratch = [
        vm((S, D), BF16), vm((NCB, PAD + S, 128), BF16), vm((NCB, S, 128), BF16), vm((TAPS, D), BF16),
        vm((NCB, NA, 128, CH), BF16), vm((NCB, 128), BF16), vm((2 * FH, D), BF16),
        vm((S, S), BF16), vm((S // 128, 128), BF16), vm((256 * KO + 128, D), BF16), vm((1, D), BF16),
        vm((D, 6 * D), BF16), vm((16, *tile), BF16),
        vm((8, 2 * NA, *tile), BF16), vm((8, 2 * NA, *tile), BF16),
        vm((2 * NA, *tile), F32), vm((2 * NA, *tile), F32), vm((NA, *tile), BF16), vm((NA, *tile), BF16),
        vm((16, NA, *tile), F32), vm((16, NA, *tile), F32), vm((5, NA, *tile), F32), vm((5, NA, *tile), F32),
        vm((NCB, S, 128), F32), vm((S, D), F32), vm((NCB, RB, 128), BF16),
        vm((S // 128, FH, 128), F32), vm((7, S // 256, FM, 128), F32),
        vm((7, KO, DM, 128), BF16), vm((D, 128), BF16), vm((S // 128, 128), F32),
        vm((S, D), BF16), vm((8, 128), jnp.int32), pltpu.SMEM((1,), jnp.int32),
        pltpu.SemaphoreType.DMA((NCB * NA + 32,)),
        pltpu.SemaphoreType.DMA((S // H,)),
    ] + [vm((FH, 128), F32)] * 16 + [vm((FH // SU * 16, 128), F32)] * 16 + [vm((2, H, 128), BF16)] * 18
    out = pl.pallas_call(
        _kernel,
        out_shape=jax.ShapeDtypeStruct((S, D), BF16),
        in_specs=[pl.BlockSpec(memory_space=pltpu.HBM)] * 13,
        out_specs=pl.BlockSpec(memory_space=pltpu.HBM),
        scratch_shapes=scratch,
        compiler_params=pltpu.CompilerParams(vmem_limit_bytes=110 * 1024 * 1024),
    )(A_q.reshape(S, D), A_k.reshape(S, D), A_v.reshape(S, D), A_shift_k.T, A_ssm_k,
      A_ssm_D.reshape(NCB, 128), B_w_in.T, B_w_sp, B_b_sp.reshape(S // 128, 128), B_w_out, c, w_mod, vf)
    return out.reshape(1, S, D)
```

```python
import functools
import math

import numpy as np
import jax
import jax.numpy as jnp
from jax import lax
import jax.experimental.pallas as pl
import jax.experimental.pallas.tpu as pltpu

S, D, FH = 2048, 640, 864
FM, DM = FH // 2, D // 2
KO = FH // 256
FT, FB = 224, 208
TAPS = 4
CH = 512
NA = S // CH
N2 = 64
N1 = CH // N2
NCB = D // 128
RB = 512
NB = S // RB
H = RB // 2
EPS = 1e-5
F32, BF16, U32 = jnp.float32, jnp.bfloat16, jnp.uint32
PAD = 16

_C8 = math.cos(math.pi / 8)
_T8 = math.tan(math.pi / 8)
_R2 = math.sqrt(0.5)
_G0 = math.sqrt(2 / math.pi)
_GA = (_G0 * 0.044715) ** (1 / 3)

UN = 1
DG = 0
E0, ES = 0, 16
MA = 1
MS = 12
TU = (-1, 0, 3, 5, 16, 32, 35, 38)
TK = (34, 38, 41, 42, 43, 44, 45, 46)
TI = (-1, -1, -1, 0, 0, 2, 3, 4, 5, 5, 7, 16, 17, 17, 32, 33, 34, 36, 37, 38, 38, 39, 40, 42)
SU = 96
NJ = ["s0:70:99,s1:114:170,s2:168:205,m14:90:120,m18:120:150,m15:150:180,m19:180:210,m13:54:80,m17:70:100", "h3:0:96,h2:98:229,s3:20:80",
      "h5:0:108:132:186,h4:192:246:314:430,s4:330:402,s6:216:270",
      "h7:0:108:162:216,h6:226:280:324:440,s5:0:54,s7:54:108,s8:324:372,s10:216:270,t0:380:480",
      "n0:0:50,n1:46:80,n2:70:108,s9:0:40,s11:40:80,n3:110:170,n4:160:216,n5:216:270,s14:170:216,s15:220:270,n7:280:340,s12:330:378,s13:380:410,n6:420:480,o0:340:470"]
R2 = 512


def _dft_mats():
    ang = [1 / 16 + m / 4 for m in range(4)] + [1 / 8, 1 / 8 + 1 / 2, 1 / 4]
    idx = np.arange(128)
    pos = (idx // 16) * 8 + idx % 8
    part = (idx // 8) % 2
    mats = []
    for b, a in enumerate(ang):
        th = 2 * np.pi * (a + pos[:, None]) * pos[None, :] / N2
        po, pi = part[:, None], part[None, :]
        m = np.where(po == pi, np.cos(th), np.where(po == 1, np.sin(th), -np.sin(th)))
        mats.append(m * ((_C8 if b < 4 else 1.0) / 8))
    n = pos + 64 * part
    th = 2 * np.pi * pos[:, None] * n[None, :] / 128
    m = np.where(part[:, None] == 0, np.cos(th), np.sin(th))
    m[8, :] = 1.0 - 2.0 * (n % 2)
    mats.append(m / 8)
    fwd = np.stack(mats).astype(np.float32)
    n = idx // 32 * 16 + idx % 8 * 2 + idx // 16 % 2
    return fwd[:, :, n // 8 * 16 + part * 8 + n % 8]


def _outer_fwd(u):
    t0r, t0i = u[0] * (1 / _C8), u[4] * (1 / _C8)
    t2r, t2i = (u[2] - u[6]) * (_R2 / _C8), (u[2] + u[6]) * (_R2 / _C8)
    t1r, t1i = u[1] - _T8 * u[5], u[5] + _T8 * u[1]
    t3r, t3i = _T8 * u[3] - u[7], _T8 * u[7] + u[3]
    ar, ai, br, bi = t0r + t2r, t0i + t2i, t0r - t2r, t0i - t2i
    cr, ci, dr, di = t1r + t3r, t1i + t3i, t1r - t3r, t1i - t3i
    out = [(ar + cr, ai + ci), (br - di, bi + dr), (ar - cr, ai - ci), (br + di, bi - dr)]
    p = [u[j] + u[j + 4] for j in range(4)]
    q = [u[j] - u[j + 4] for j in range(4)]
    er, ei = (q[1] - q[3]) * _R2, (q[1] + q[3]) * _R2
    out += [(q[0] + er, q[2] + ei), (q[0] - er, q[2] - ei)]
    out += [(p[0] - p[2], p[1] - p[3]), (p[0] + p[2], p[1] + p[3])]
    return out


def _outer_inv(B):
    ar, ai = B[0][0] + B[2][0], B[0][1] + B[2][1]
    cr, ci = B[0][0] - B[2][0], B[0][1] - B[2][1]
    br, bi = B[1][0] + B[3][0], B[1][1] + B[3][1]
    dr, di = B[1][0] - B[3][0], B[1][1] - B[3][1]
    g0r, g0i, g2r, g2i = ar + br, ai + bi, ar - br, ai - bi
    g1r, g1i, g3r, g3i = cr + di, ci - dr, cr - di, ci + dr
    nr = [g0r * (1 / _C8), g1r + _T8 * g1i, (g2r + g2i) * (_R2 / _C8), _T8 * g3r + g3i]
    ni = [g0i * (1 / _C8), g1i - _T8 * g1r, (g2i - g2r) * (_R2 / _C8), _T8 * g3i - g3r]
    fr, fi = B[4][0] - B[5][0], B[4][1] - B[5][1]
    q = [B[4][0] + B[5][0], (fr + fi) * _R2, B[4][1] + B[5][1], (fi - fr) * _R2]
    p = [B[7][0] + B[6][0], B[7][1] + B[6][1], B[7][0] - B[6][0], B[7][1] - B[6][1]]
    return ([p[j] + q[j] + nr[j] for j in range(4)]
            + [p[j] - q[j] + ni[j] for j in range(4)])


def _gelu_scaled(x):
    t = jnp.tanh(x * (_G0 / _GA + x * x))
    return x + x * t


def _norm_stats(s1, s2, n, eps):
    m = s1 * (1.0 / n)
    return m, jnp.exp(-0.5 * jnp.log(jnp.maximum(s2 * (1.0 / n) - m * m, 0.0) + eps))


def _ln_rows(x):
    m, r = _norm_stats(jnp.sum(x, axis=-1, keepdims=True), jnp.sum(x * x, axis=-1, keepdims=True),
                       x.shape[-1], EPS)
    return (x - m) * r


def _lhs7(a11, a12, a21, a22):
    return a11 + a22, a21 + a22, a11, a22, a11 + a12, a21 - a11, a12 - a22


def _words(ref, *idx):
    return ref.bitcast(U32)[idx]


def _ld(ref, *idx):
    return pltpu.bitcast(_words(ref, *idx), BF16)


def _phase(words, odd):
    return pltpu.bitcast(words & np.uint32(0xFFFF0000) if odd else words << 16, F32)


def _nn(a, b):
    return jnp.dot(a, b, preferred_element_type=F32)


def _nt(a, b):
    return lax.dot_general(a, b, (((1,), (1,)), ((), ())), preferred_element_type=F32)


def _ds(start, size, align):
    return pl.ds(start if isinstance(start, int) else pl.multiple_of(start, align), size)


def _add(xs):
    return functools.reduce(lambda x, y: x + y, xs)


def _kernel(q_h, k_h, v_h, sh_h, sk_h, sd_h, wi_h, ws_h, b_h, wo_h, c_h, wm_h, vf_h, o_h,
            q_v, k_v, v_v, sh_v, sk_v, sd_v, wi_v, ws_v, b_v, wo_v, c_v, wm_v, vf_v,
            au0_v, au1_v, fa_v, fb_v, ya_v, yb_v, bm0_v, bp0_v, bm1_v, bp1_v,
            y_v, x1_v, h0_v, z1_v, z2_v, wt_v, wr_v, bf_v, o_v, tie_v, zero_s,
            sems, osem, *lists):
    au_v, h_v = (au0_v, au1_v), (lists[32:41], lists[41:])
    copies = {}

    def start(name, src, dst):
        copies[name] = pltpu.make_async_copy(src, dst, sems.at[NCB * NA + len(copies)])
        copies[name].start()

    def wait(*names):
        for name in names:
            copies[name].wait()

    def conv_inputs(cb, a):
        rows, lanes, sem = _ds(a * CH, CH, CH), pl.ds(cb * 128, 128), sems.at[cb * NA + a]
        return (pltpu.make_async_copy(k_h.at[rows, lanes], k_v.at[cb, _ds(PAD + a * CH, CH, PAD)], sem),
                pltpu.make_async_copy(v_h.at[rows, lanes], v_v.at[cb, rows], sem),
                pltpu.make_async_copy(sk_h.at[lanes, rows], sk_v.at[cb, a], sem))

    def fetch(stage):
        if stage < NCB:
            for a in range(NA):
                for cp in conv_inputs(stage, a):
                    cp.start()
        if stage == 0:
            start("vf", vf_h, vf_v.at[pl.ds(0, 8)])
        if stage == NCB:
            start("c", c_h, c_v)
            start("wm", wm_h.at[:, pl.ds(0, 5 * D)], wm_v.at[:, pl.ds(0, 5 * D)])
            start("q0", q_h.at[pl.ds(0, H)], q_v.at[pl.ds(0, H)])
            start("w2", wi_h.at[pl.ds(FH, FH)], wi_v.at[pl.ds(0, FH)])
            start("q1", q_h.at[pl.ds(H, RB - H)], q_v.at[pl.ds(H, RB - H)])
            start("w1", wi_h.at[pl.ds(0, FH)], wi_v.at[pl.ds(FH, FH)])
            start("q2", q_h.at[pl.ds(RB, 2 * RB)], q_v.at[pl.ds(RB, 2 * RB)])
            start("q3", q_h.at[pl.ds(3 * RB, RB)], q_v.at[pl.ds(3 * RB, RB)])
        if stage == NCB + 2:
            start("wg", wm_h.at[:, pl.ds(5 * D, D)], wm_v.at[:, pl.ds(5 * D, D)])
            start("b", b_h, b_v)
            start("wo", wo_h, wo_v.at[pl.ds(0, FH)])
            for j in range(S // 128):
                start(("ws", j), ws_h.at[:, pl.ds(128 * j, 128)], ws_v.at[j])

    start("sh", sh_h, sh_v)
    start("sd", sd_h, sd_v)
    fetch(0)
    fetch(1)
    for ref in (fb_v, ya_v, tie_v):
        ref[...] = jnp.zeros(ref.shape, ref.dtype)
    k_v[:, pl.ds(0, PAD), :] = jnp.zeros((NCB, PAD, 128), BF16)
    wo_v[pl.ds(FH, 256 * KO + 128 - FH), :] = jnp.zeros((256 * KO + 128 - FH, D), BF16)
    zero_s[0] = 0
    row8 = lax.broadcasted_iota(jnp.int32, (8, 128), 0)

    def tie(after, x):
        if after is None:
            return x
        never = jnp.concatenate([tie_v[...]] * (x.shape[0] // 8), axis=0) != 0
        return jnp.where(never, after, x)

    def put(cb, slot, g, res):
        for b in range(8):
            au_v[cb % 2][b, slot, pl.ds(16 * g, 16), :] = jnp.concatenate(res[b], axis=0).astype(BF16)

    def split_filter(cb, a, after):
        kt = pltpu.bitcast(sk_v[cb, a].T, U32)
        for g in range(N2 // 8):
            u = [_phase(kt[j * N2 // 2 + g // 2 * 8:j * N2 // 2 + g // 2 * 8 + 8], g % 2) for j in range(N1)]
            if g == 0:
                u[0] = u[0] + jnp.where(row8 + a == 0, sd_v[...].astype(F32)[cb:cb + 1], 0.0)
            u[:4] = [tie(after(g), x) for x in u[:4]]
            put(cb, NA + a, g, _outer_fwd(u))

    def split_signal(cb, a, after):
        taps = [jnp.broadcast_to(sh_v[j:j + 1, pl.ds(cb * 128, 128)].astype(F32), (8, 128))
                for j in range(TAPS)]
        base = a * (CH // 2) if isinstance(a, int) else pl.multiple_of(a * (CH // 2), CH // 2)
        for g in range(N2 // 8):
            w = [tie(after(g), t) for t in taps]
            u = []
            for j in range(N1):
                r = base + j * N2 // 2 + g // 2 * 8
                lag = [_phase(_words(k_v, cb, pl.ds(r + PAD // 2 + (g % 2 - t) // 2, 8)), (g % 2 - t) % 2)
                       for t in range(TAPS)]
                u.append(_add([x * wt for x, wt in zip(lag, w)]) * _phase(_words(v_v, cb, pl.ds(r, 8)), g % 2))
            put(cb, a, g, _outer_fwd(u))

    def spectra(cb, b, half, f_ref):
        rhs = jnp.concatenate([_ld(au_v[cb % 2], b, half * NA + a) for a in range(NA)], axis=1)
        f = _nn(_ld(vf_v, b), rhs)
        for a in range(NA):
            f_ref[half * NA + a] = f[:, 128 * a:128 * a + 128]
        return f

    def product(f_ref, y_ref, plus, real_rows=None):
        for g in range(8):
            ur, ui, kr, ki = ([f_ref[o + a, pl.ds(16 * g + 8 * c, 8), :] for a in range(NA)]
                              for o in (0, NA) for c in (0, 1))
            kr, ki = ([k[0]] + [k[a] + k[a - 1] if plus else k[a] - k[a - 1] for a in range(1, NA)]
                      for k in (kr, ki))
            for a in range(NA):
                yi = _add([kr[j] * ui[a - j] + ki[j] * ur[a - j] for j in range(a + 1)])
                if real_rows is not None and g == 0:
                    rr = _add([kr[j] * ur[a - j] for j in range(a + 1)])
                    ii = _add([ki[j] * ui[a - j] for j in range(a + 1)])
                    yr = jnp.where(real_rows, 0.5 * rr, rr - ii)
                    yi = jnp.where(real_rows, 0.5 * ii, yi)
                else:
                    yr = _add([kr[j] * ur[a - j] - ki[j] * ui[a - j] for j in range(a + 1)])
                y_ref[a, pl.ds(16 * g, 16), :] = jnp.concatenate([yr, yi], axis=0).astype(BF16)

    def residues(y_ref, b, dst):
        r = _nn(_ld(vf_v, 8 + b), jnp.concatenate([_ld(y_ref, a) for a in range(NA)], axis=1))
        for a in range(NA):
            dst[a] = r[:, 128 * a:128 * a + 128]
        return r

    def stash(t):
        return ((bm0_v.at[t], bp0_v.at[t]) if t < 16 else (bm1_v.at[t - 16], bp1_v.at[t - 16]))

    def merge(cb, a, after=lambda g: None):
        src = [stash(1 + 4 * cb + b)[s] for s in (0, 1) for b in range(4)]
        for g in range(N2 // 8):
            res = [[ref[a, pl.ds(16 * g + 8 * c, 8), :] for c in (0, 1)] for ref in src]
            res[0] = [tie(after(g), x) for x in res[0]]
            res[1] = [tie(after(g), x) for x in res[1]]
            for j, y in enumerate(_outer_inv(res)):
                y_v[cb, _ds(a * CH + j * N2 + 8 * g, 8, 8), :] = y

    def transform(cb, a, dst, active=True):
        pa = (a + 3) % 4
        res = []
        if active:
            res += [spectra(cb, a, 1, fa_v), spectra(cb, a, 0, fa_v)]
        product(fb_v, yb_v, True, row8 + (3 - pa) == 0)
        res.append(residues(ya_v, pa, dst[0]))
        if active:
            res += [spectra(cb, 4 + a, 1, fb_v), spectra(cb, 4 + a, 0, fb_v)]
            product(fa_v, ya_v, False)
        res.append(residues(yb_v, 4 + pa, dst[1]))
        return res

    def conv_step(cb, i):
        steps = [UN * i + u for u in range(UN)]
        if cb < NCB:
            for a in steps:
                for cp in conv_inputs(cb, a):
                    cp.wait()
        done = []
        for a in steps if cb else ():
            done += transform(cb - 1, a, (bm0_v.at[4 * cb - 4 + a], bp0_v.at[4 * cb - 4 + a])
                              if cb < NCB else (bm1_v.at[a], bp1_v.at[a]))
        at = lambda p: done[p // 8][16 * (p % 8):16 * (p % 8) + 8, 0:128] if done and p >= 0 else None
        for u, a in enumerate(steps):
            if cb < NCB:
                split_signal(cb, a, lambda g: at(TU[8 * u + g]))
                split_filter(cb, a, lambda g: at(TK[8 * u + g]))
            else:
                for c in range(3):
                    merge(c, a, lambda g: at(TI[24 * u + 8 * c + g]))

    wait("sh", "sd")
    for cb in range(NCB + 1):
        if cb == 1:
            wait("vf")
            row, col = (lax.broadcasted_iota(jnp.int32, (128, 128), d) for d in (0, 1))
            n = (col >> 5) * 16 + (col & 7) * 2 + ((col >> 4) & 1)
            order = jnp.where(row == (n >> 3) * 16 + (col & 8) + (n & 7), 1.0, 0.0).astype(BF16)
            for b in range(8):
                vf_v[8 + b] = _nt(order, vf_v[b]).astype(BF16)
        fetch(cb + 2)
        pl.loop(0, NA // UN)(functools.partial(conv_step, cb))

    wait("c", "wm", "q0")
    transform(NCB, 0, stash(20), active=False)
    cc = c_v[...].astype(F32)
    sc = jnp.broadcast_to(cc / (1.0 + jnp.exp(-cc)), (16, D)).astype(BF16)
    mod = _nn(sc, jnp.concatenate([wm_v[:, pl.ds(i * D, D)] for i in (0, 1, 2, 4, 3)], axis=1))[0:8]
    sa, ca, ga, cb_, sb = (mod[:, i * D:(i + 1) * D] for i in range(5))
    m1, m0 = ga * (1.0 + ca), ga * sa
    n1, n0 = _GA * (1.0 + cb_), _GA * sb
    zero = zero_s[0]
    for n, (cb, a) in enumerate([(cb, a) for cb in (3, 4) for a in range(MA)]):
        merge(cb, a + zero, lambda g: mod[:, 128 * ((8 * n + g) * MS // (16 * MA)):][:, :128])

    TB = RB // 128
    PER = 2 * FH // 16

    def hidden(r0, after=(None, None)):
        out = []
        for r, a in zip((r0, r0 + 8), after):
            rows = pl.ds(r, 8)
            x = q_v[rows, :].astype(F32)
            x = jnp.concatenate([tie(a, x[:, :128]), x[:, 128:]], axis=1)
            x1 = x + (_ln_rows(x) * m1 + m0) * jnp.concatenate([y_v[j, rows, :] for j in range(NCB)], axis=1)
            x1_v[rows, :] = x1
            out.append(_ln_rows(x1) * n1 + n0)
        return jnp.concatenate(out, axis=0)

    def keep_gate(tile, z):
        lists[tile][pl.ds(zero, FH), :] = z

    def moments(tile, after):
        z, acc = lists[tile], lists[16 + tile]
        s1 = s2 = None
        for n, f in enumerate(range(0, FH, SU)):
            for r in range(f, f + SU, 8):
                d = tie(after(n)[:8] if r == f else None, z[pl.ds(r, 8), :])
                s1, s2 = (d, d * d) if s1 is None else (s1 + d, s2 + d * d)
            acc[pl.ds(16 * n + zero, 16), :] = jnp.concatenate([s1, s2], axis=0)
        s1, s2 = (jnp.sum(acc[pl.ds(16 * n + r, 8), :], axis=0, keepdims=True) for r in (0, 8))
        stats[tile] = [jnp.broadcast_to(t, (16, 128)) for t in _norm_stats(s1, s2, FH, EPS * (2 * _GA) ** 2)]

    def norm_gate(pair, after):
        for n in range(FM // 16):
            means = [tie(after(n), stats[2 * pair + c][0]) for c in (0, 1)]
            quad = [(lists[2 * pair + c][pl.ds(r + 16 * n, 16), :] - means[c]) * stats[2 * pair + c][1]
                    for r in (0, FM) for c in (0, 1)]
            for k, a in enumerate(_lhs7(*quad)):
                z2_v[k, pair, pl.ds(16 * n, 16), :] = a

    def lanes(x, j, n=1):
        return x[:, 128 * j:128 * (j + n)]

    def prepare(i, c, after):
        def put(k, n, x):
            for j in range(x.shape[1] // 128):
                h_v[i % 2][k][j, pl.ds(16 * n + zero, 16), :] = lanes(x, j).astype(BF16)

        for n in range(H // 16):
            h = hidden(i * RB + c * H + 16 * n, (after(2 * n)[:8], after(2 * n + 1)[:8]))
            top, bot = lanes(h, 0, 2), lanes(h, 2, 2)
            put(7 + c, n, lanes(h, 4))
            if c:
                half[n] = top, bot
                put(2, n, top - bot)
                put(4, n, bot)
            else:
                put(1, n, top)
                put(3, n, bot - top)
                put(0, n, top + half[n][1])
                put(5, n, top + half[n][0])
                put(6, n, bot + half[n][1])

    def turn_out(after):
        for n in range((2 * KO + 1) * NCB):
            j, t = divmod(n, NCB)
            w = _words(wo_v, pl.ds(64 * j, 64), pl.ds(128 * t, 128))
            w = jnp.concatenate([tie(pltpu.bitcast(after(n)[:8], U32), w[:8]), w[8:]], axis=0)
            wr_v[j, pl.ds(128 * t + zero, 128), :] = pltpu.bitcast(w, BF16).T

    def split_out(after):
        for n in range(KO * DM // 16):
            j, r = divmod(16 * n, DM)
            quad = [wr_v[j + KO * c, pl.ds(r + DM * b, 16), :].astype(F32) for b in (0, 1) for c in (0, 1)]
            for k, a in enumerate(_lhs7(tie(after(n), quad[0]), quad[1], quad[2], tie(after(n), quad[3]))):
                wt_v[k, j, pl.ds(r, 16), :] = a.astype(BF16)

    def side_jobs(plan, at):
        for job in plan.split(","):
            if job:
                kind, (n, *spans) = job[0], (int(x) for x in job[1:].split(":"))
                total = {"s": FH // SU, "n": FM // 16, "h": H // 8, "m": N2 // 8,
                         "t": (2 * KO + 1) * NCB, "o": KO * DM // 16}[kind]
                slots = [p for lo, hi in zip(spans[::2], spans[1::2]) for p in range(lo, hi)]
                after = lambda k: at(slots[k * len(slots) // total])
                if kind == "s":
                    moments(n, after)
                elif kind == "m":
                    merge(n // NA, n % NA + zero, lambda k: after(k)[:8])
                elif kind in "to":
                    (turn_out if kind == "t" else split_out)(after)
                elif kind == "n":
                    norm_gate(n, after)
                else:
                    prepare(n // 2, n % 2, after)

    def rows_of(z):
        per = z.shape[0] // 16
        return lambda p: z[16 * (p % per):16 * (p % per) + 16, 128 * (p // per):128 * (p // per) + 128]

    def project(i):
        def prod(*pairs):
            right = [_ld(h_v[i % 2][k], j) for _, k in pairs for j in range(2 if k < 7 else 1)]
            return _nt(jnp.concatenate([x for k, _ in pairs for x in left[k]], axis=1),
                       jnp.concatenate(right, axis=1))

        s5, s3, r12, s4, s1 = prod((4, 4)), prod((2, 2)), prod((7, 8)), prod((3, 3)), prod((0, 0))
        s7, s2, r21, s6 = prod((6, 6), (7, 7)), prod((1, 1)), prod((8, 7)), prod((5, 5), (8, 8))
        gate = [((s4 - s5) + s1) + s7, (s5 + s3) + r12]
        value = [(s4 + s2) + r21, ((s3 + s1) - s2) + s6]
        for c, later in enumerate((s2, lanes(s4, 1))):
            keep_gate(i * TB + 2 * c, _gelu_scaled(lanes(gate[c], 0)))
            keep_gate(i * TB + 2 * c + 1, _gelu_scaled(tie(lanes(later, 0) if DG else None, lanes(gate[c], 1))))
        for t in range(TB):
            z1_v[i * TB + t] = lanes(value[t // 2], t % 2)
        rounds = (s5, s3, gate[1], lanes(s4, 1), lanes(s1, 1), gate[0], s2, value[0], lanes(value[1], 1))
        return lambda p: rounds[p // (FH // 16)][16 * (p % (FH // 16)):16 * (p % (FH // 16)) + 16, 0:128]

    def first(f0, r0, n, k0, k1):
        h = jnp.concatenate([_ld(h0_v, j, pl.ds(r0 // 2, n // 2)) for j in range(k0, k1)], axis=1)
        return _nt(wi_v[pl.ds(f0, FH), pl.ds(128 * k0, 128 * (k1 - k0))], h)

    def keep_first(r, h):
        for j in range(NCB):
            h0_v[j, pl.ds(r, 16), :] = lanes(h, j).astype(BF16)

    stats, half = {}, {}
    for r in range(0, H, 16):
        keep_first(r, hidden(r))
    wait("w2", "q1")
    zero = pl.multiple_of(zero_s[0], 16)
    head = first(0, 0, H, 0, 2)
    z = _gelu_scaled(head + first(0, 0, H, 2, NCB))
    at = rows_of(jnp.concatenate([lanes(head, 0), z], axis=1))
    for n in range(H // 16):
        keep_first(H + 16 * n, hidden(H + 16 * n, [at(E0 + (2 * n + k) * ES // 8)[:8] for k in (0, 1)]))
    z = jnp.concatenate([z] + [_gelu_scaled(first(0, r, 128, 0, NCB)) for r in (H, H + 128)], axis=1)
    for t in range(TB):
        keep_gate(t, lanes(z, t))
    side_jobs(NJ[0], rows_of(z))
    wait("w1", "q2")
    head = first(FH, 0, RB, NCB - 1, NCB)
    z = head + first(FH, 0, RB, 0, NCB - 1)
    for t in range(TB):
        z1_v[t] = lanes(z, t)
    side_jobs(NJ[1], rows_of(jnp.concatenate([lanes(head, 0), z], axis=1)))
    sums = [_lhs7(*(wi_v[pl.ds(FH * r, FH), pl.ds(256 * c + 128 * j, 128)].astype(F32)
                    for r in (0, 1) for c in (0, 1))) for j in (0, 1)]
    left = ([[s[k].astype(BF16) for s in sums] for k in range(7)]
            + [[wi_v[pl.ds(FH * r, FH), pl.ds(512, 128)]] for r in (0, 1)])
    for i in range(1, NB):
        if i == 2:
            wait("q3", "wg", "b", "wo")
            gb = _nn(sc, wm_v[:, pl.ds(5 * D, D)]) * (0.5 / _GA)
            bf_v[...] = b_v[...].astype(F32)
        side_jobs(NJ[i + 1], project(i))

    wait(*[("ws", j) for j in range(S // 128)])
    T2 = R2 // 128

    def mix(i):
        def w(c, r):
            return [_ld(ws_v, 2 * j + c, _ds((i * R2 + r * H) // 2, H // 2, H // 2)).astype(F32)
                    for j in range(S // 256)]

        def comb(x, y, sign):
            return [a + b if sign > 0 else a - b for a, b in zip(x, y)]

        def prod(n, rhs):
            def left(k):
                def part(r, c, rows):
                    return jnp.concatenate([z2_v[n, 2 * j + c, pl.ds(FT * r, rows), :] for j in range(NB)], axis=1)

                def both(c, op):
                    top = part(0, c, FT)
                    return jnp.concatenate([op(top[:FB], part(1, 1, FB)), top[FB:]], axis=0)

                return (lambda: both(0, jnp.add), lambda: part(1, 0, FB) + part(1, 1, FB),
                        lambda: part(0, 0, FT), lambda: part(1, 1, FB),
                        lambda: part(0, 0, FT) + part(0, 1, FT), lambda: part(1, 0, FB) - part(0, 0, FB),
                        lambda: both(1, jnp.subtract))[k]().astype(BF16)

            b11, b12, b21, b22 = (
                jnp.concatenate([rhs[2 * j + c][128 * r:128 * r + 128] for j in range(NB)], axis=1)
                for c in (0, 1) for r in (0, 1))
            m = lambda k, x: _nt(left(k), x.astype(BF16))
            m2, m5, m4 = m(1, b11), m(4, b22), m(3, b21 - b11)
            m1, m7, m3, m6 = m(0, b11 + b22), m(6, b21 + b22), m(2, b12 - b22), m(5, b11 + b12)
            c11 = jnp.concatenate([m4 - m5[:FB], -m5[FB:]], axis=0) + m1 + m7
            c22 = (m1[:FB] - m2) + m3[:FB] + m6
            return jnp.concatenate([jnp.concatenate([c11, m5 + m3], axis=1),
                                    jnp.concatenate([m2 + m4, c22], axis=1)], axis=0)

        def gate(r, c, g):
            tiles = [i * T2 + c * (H // 128) + t for t in range(H // 128)]
            bias = jnp.concatenate([bf_v[pl.ds(j, 1), :] for j in tiles], axis=1)
            z1 = jnp.concatenate([z1_v[j, pl.ds(FM * r, FM), :] for j in tiles], axis=1)
            return _gelu_scaled(z1) * (g + bias)

        s2 = prod(1, w(0, 0))
        s5 = prod(4, w(1, 1))
        s4 = prod(3, comb(w(1, 0), w(0, 0), -1))
        p21 = gate(1, 0, s2 + s4)
        d11 = s4 - s5
        s1 = prod(0, comb(w(0, 0), w(1, 1), 1))
        d11, d22 = d11 + s1, s1 - s2
        p11 = gate(0, 0, d11 + prod(6, comb(w(1, 0), w(1, 1), 1)))
        s3 = prod(2, comb(w(0, 1), w(1, 1), -1))
        p12 = gate(0, 1, s3 + s5)
        p22 = gate(1, 1, (d22 + s3) + prod(5, comb(w(0, 0), w(0, 1), 1)))
        return [jnp.concatenate(p, axis=0) for p in ((p11, p21), (p12, p22))]

    def flush(k):
        rows = _ds(k * H, H, H)
        return pltpu.make_async_copy(o_v.at[rows], o_h.at[rows], osem.at[k])

    def finish(r0, tile):
        for t in range(H // 128):
            for j in range(NCB):
                at = _ds(r0 + 128 * t, 128, 128), pl.ds(128 * j, 128)
                o_v[at] = (x1_v[at] + jnp.concatenate([lanes(gb, j)] * 8, axis=0)
                           * tile(t, j).T.astype(F32)).astype(BF16)

    def mix_step(i):
        p = mix(i)
        b11, b12, b21, b22 = (p[c][128 * KO * r:128 * KO * (r + 1)] for r in (0, 1) for c in (0, 1))

        def prod(n, rhs):
            return _nn(jnp.concatenate([_ld(wt_v, n, j) for j in range(KO)], axis=1), rhs.astype(BF16))

        def rest(c):
            tail = jnp.concatenate([p[c][256 * KO:], jnp.zeros((128 + 256 * KO - FH, H), F32)], axis=0)
            return _nn(_ld(wr_v, 2 * KO), tail.astype(BF16))

        r0 = rest(0)
        s2 = prod(1, b11)
        s4 = prod(3, b21 - b11)
        s5 = prod(4, b22)
        s1 = prod(0, b11 + b22)
        s7 = prod(6, b21 + b22)
        ot = jnp.concatenate([r0[:DM] + s4 - s5 + s1 + s7, r0[DM:] + s2 + s4], axis=0)
        finish(i * R2, lambda t, j: lanes(ot, t)[128 * j:128 * j + 128].astype(BF16))
        flush(2 * i).start()
        spot = _ds(i * R2 + H, 16, 16), pl.ds(0, 128)
        o_v[spot] = jnp.zeros((16, 128), BF16)
        pin = o_v[_ds(i * R2 + H + zero, 16, 16), pl.ds(0, 128)].astype(F32)
        r1 = rest(1)
        s3 = prod(2, b12 - b22)
        b = b11 + b12
        b = jnp.concatenate([b[:-16], jnp.concatenate([b[-16:, :128], tie(pin, b[-16:, 128:])], axis=1)], axis=0)
        s6 = prod(5, b)
        ot = jnp.concatenate([r1[:DM] + s5 + s3, (s1 - s2) + r1[DM:] + s3 + s6], axis=0)
        finish(i * R2 + H, lambda t, j: lanes(ot, t)[128 * j:128 * j + 128].astype(BF16))
        flush(2 * i + 1).start()

    zero = pl.multiple_of(zero_s[0], 16)
    zero = zero_s[0]
    pl.loop(0, S // R2)(mix_step)
    for k in range(S // H):
        flush(k).wait()


@jax.jit
def pallas_adaLN_cond__ssm_conv_h3__mixer_gmlp__prompt_kernel(
    A_q, A_k, A_v, A_shift_k, A_ssm_k, A_ssm_D, B_x, B_w_in, B_w_sp, B_b_sp, B_w_out, c, w_mod,
):
    del B_x
    vf = _dft_mats().astype(BF16)
    vm = pltpu.VMEM
    tile = (128, 128)
    scratch = [
        vm((S, D), BF16), vm((NCB, PAD + S, 128), BF16), vm((NCB, S, 128), BF16), vm((TAPS, D), BF16),
        vm((NCB, NA, 128, CH), BF16), vm((NCB, 128), BF16), vm((2 * FH, D), BF16),
        vm((S // 128, S, 128), BF16), vm((S // 128, 128), BF16), vm((256 * KO + 128, D), BF16), vm((1, D), BF16),
        vm((D, 6 * D), BF16), vm((16, *tile), BF16),
        vm((8, 2 * NA, *tile), BF16), vm((8, 2 * NA, *tile), BF16),
        vm((2 * NA, *tile), F32), vm((2 * NA, *tile), F32), vm((NA, *tile), BF16), vm((NA, *tile), BF16),
        vm((16, NA, *tile), F32), vm((16, NA, *tile), F32), vm((5, NA, *tile), F32), vm((5, NA, *tile), F32),
        vm((NCB, S, 128), F32), vm((S, D), F32), vm((NCB, RB, 128), BF16),
        vm((S // 128, FH, 128), F32), vm((7, S // 256, FM, 128), F32),
        vm((7, KO, DM, 128), BF16), vm((2 * KO + 1, D, 128), BF16), vm((S // 128, 128), F32),
        vm((S, D), BF16), vm((8, 128), jnp.int32), pltpu.SMEM((1,), jnp.int32),
        pltpu.SemaphoreType.DMA((NCB * NA + 32,)),
        pltpu.SemaphoreType.DMA((S // H,)),
    ] + [vm((FH, 128), F32)] * 16 + [vm((FH // SU * 16, 128), F32)] * 16 + ([vm((2, H, 128), BF16)] * 7 + [vm((1, H, 128), BF16)] * 2) * 2
    out = pl.pallas_call(
        _kernel,
        out_shape=jax.ShapeDtypeStruct((S, D), BF16),
        in_specs=[pl.BlockSpec(memory_space=pltpu.HBM)] * 13,
        out_specs=pl.BlockSpec(memory_space=pltpu.HBM),
        scratch_shapes=scratch,
        compiler_params=pltpu.CompilerParams(vmem_limit_bytes=110 * 1024 * 1024),
    )(A_q.reshape(S, D), A_k.reshape(S, D), A_v.reshape(S, D), A_shift_k.T, A_ssm_k,
      A_ssm_D.reshape(NCB, 128), B_w_in.T, B_w_sp, B_b_sp.reshape(S // 128, 128), B_w_out, c, w_mod, vf)
    return out.reshape(1, S, D)
```

```python
import functools
import math

import numpy as np
import jax
import jax.numpy as jnp
from jax import lax
import jax.experimental.pallas as pl
import jax.experimental.pallas.tpu as pltpu

S, D, FH = 2048, 640, 864
FM, DM = FH // 2, D // 2
KO = FH // 256
FT, FB = 224, 208
TAPS = 4
CH = 512
NA = S // CH
N2 = 64
N1 = CH // N2
NCB = D // 128
RB = 512
NB = S // RB
H = RB // 2
EPS = 1e-5
F32, BF16, U32 = jnp.float32, jnp.bfloat16, jnp.uint32
PAD = 16

_C8 = math.cos(math.pi / 8)
_T8 = math.tan(math.pi / 8)
_R2 = math.sqrt(0.5)
_G0 = math.sqrt(2 / math.pi)
_GA = (_G0 * 0.044715) ** (1 / 3)

UN = 1
DG = 0
E0, ES = 0, 16
MA = 1
MS = 12
TU = (-1, 0, 3, 5, 16, 32, 35, 38)
TK = (34, 38, 41, 42, 43, 44, 45, 46)
TI = (-1, -1, -1, 0, 0, 2, 3, 4, 5, 5, 7, 16, 17, 17, 32, 33, 34, 36, 37, 38, 38, 39, 40, 42)
SU = 96
NJ = ["s0:70:99,s1:114:170,s2:168:205,m14:90:120,m18:120:150,m15:150:180,m19:180:210,m13:54:80,m17:70:100", "h3:0:96,h2:98:229,s3:20:80",
      "h5:0:108:132:186,h4:192:246:314:430,s4:330:402,s6:216:270",
      "h7:0:108:162:216,h6:226:280:324:440,s5:0:54,s7:54:108,s8:324:372,s10:216:270,n0:380:486",
      "s9:0:40,s11:40:80,n1:0:56,n2:56:112,n3:112:168,n4:168:224,n5:224:280,s14:170:216,s15:220:270,n7:280:360,s12:330:378,s13:380:410,n6:420:480,t0:0:320,o0:370:470"]
R2 = 512


def _dft_mats():
    ang = [1 / 16 + m / 4 for m in range(4)] + [1 / 8, 1 / 8 + 1 / 2, 1 / 4]
    idx = np.arange(128)
    pos = (idx // 16) * 8 + idx % 8
    part = (idx // 8) % 2
    mats = []
    for b, a in enumerate(ang):
        th = 2 * np.pi * (a + pos[:, None]) * pos[None, :] / N2
        po, pi = part[:, None], part[None, :]
        m = np.where(po == pi, np.cos(th), np.where(po == 1, np.sin(th), -np.sin(th)))
        mats.append(m * ((_C8 if b < 4 else 1.0) / 8))
    n = pos + 64 * part
    th = 2 * np.pi * pos[:, None] * n[None, :] / 128
    m = np.where(part[:, None] == 0, np.cos(th), np.sin(th))
    m[8, :] = 1.0 - 2.0 * (n % 2)
    mats.append(m / 8)
    fwd = np.stack(mats).astype(np.float32)
    n = idx // 32 * 16 + idx % 8 * 2 + idx // 16 % 2
    return fwd[:, :, n // 8 * 16 + part * 8 + n % 8]


def _outer_fwd(u):
    t0r, t0i = u[0] * (1 / _C8), u[4] * (1 / _C8)
    t2r, t2i = (u[2] - u[6]) * (_R2 / _C8), (u[2] + u[6]) * (_R2 / _C8)
    t1r, t1i = u[1] - _T8 * u[5], u[5] + _T8 * u[1]
    t3r, t3i = _T8 * u[3] - u[7], _T8 * u[7] + u[3]
    ar, ai, br, bi = t0r + t2r, t0i + t2i, t0r - t2r, t0i - t2i
    cr, ci, dr, di = t1r + t3r, t1i + t3i, t1r - t3r, t1i - t3i
    out = [(ar + cr, ai + ci), (br - di, bi + dr), (ar - cr, ai - ci), (br + di, bi - dr)]
    p = [u[j] + u[j + 4] for j in range(4)]
    q = [u[j] - u[j + 4] for j in range(4)]
    er, ei = (q[1] - q[3]) * _R2, (q[1] + q[3]) * _R2
    out += [(q[0] + er, q[2] + ei), (q[0] - er, q[2] - ei)]
    out += [(p[0] - p[2], p[1] - p[3]), (p[0] + p[2], p[1] + p[3])]
    return out


def _outer_inv(B):
    ar, ai = B[0][0] + B[2][0], B[0][1] + B[2][1]
    cr, ci = B[0][0] - B[2][0], B[0][1] - B[2][1]
    br, bi = B[1][0] + B[3][0], B[1][1] + B[3][1]
    dr, di = B[1][0] - B[3][0], B[1][1] - B[3][1]
    g0r, g0i, g2r, g2i = ar + br, ai + bi, ar - br, ai - bi
    g1r, g1i, g3r, g3i = cr + di, ci - dr, cr - di, ci + dr
    nr = [g0r * (1 / _C8), g1r + _T8 * g1i, (g2r + g2i) * (_R2 / _C8), _T8 * g3r + g3i]
    ni = [g0i * (1 / _C8), g1i - _T8 * g1r, (g2i - g2r) * (_R2 / _C8), _T8 * g3i - g3r]
    fr, fi = B[4][0] - B[5][0], B[4][1] - B[5][1]
    q = [B[4][0] + B[5][0], (fr + fi) * _R2, B[4][1] + B[5][1], (fi - fr) * _R2]
    p = [B[7][0] + B[6][0], B[7][1] + B[6][1], B[7][0] - B[6][0], B[7][1] - B[6][1]]
    return ([p[j] + q[j] + nr[j] for j in range(4)]
            + [p[j] - q[j] + ni[j] for j in range(4)])


def _gelu_scaled(x):
    t = jnp.tanh(x * (_G0 / _GA + x * x))
    return x + x * t


def _norm_stats(s1, s2, n, eps):
    m = s1 * (1.0 / n)
    return m, jnp.exp(-0.5 * jnp.log(jnp.maximum(s2 * (1.0 / n) - m * m, 0.0) + eps))


def _ln_rows(x):
    m, r = _norm_stats(jnp.sum(x, axis=-1, keepdims=True), jnp.sum(x * x, axis=-1, keepdims=True),
                       x.shape[-1], EPS)
    return (x - m) * r


def _lhs7(a11, a12, a21, a22):
    return a11 + a22, a21 + a22, a11, a22, a11 + a12, a21 - a11, a12 - a22


def _words(ref, *idx):
    return ref.bitcast(U32)[idx]


def _ld(ref, *idx):
    return pltpu.bitcast(_words(ref, *idx), BF16)


def _phase(words, odd):
    return pltpu.bitcast(words & np.uint32(0xFFFF0000) if odd else words << 16, F32)


def _nn(a, b):
    return jnp.dot(a, b, preferred_element_type=F32)


def _nt(a, b):
    return lax.dot_general(a, b, (((1,), (1,)), ((), ())), preferred_element_type=F32)


def _ds(start, size, align):
    return pl.ds(start if isinstance(start, int) else pl.multiple_of(start, align), size)


def _add(xs):
    return functools.reduce(lambda x, y: x + y, xs)


def _kernel(q_h, k_h, v_h, sh_h, sk_h, sd_h, wi_h, ws_h, b_h, wo_h, c_h, wm_h, vf_h, o_h,
            q_v, k_v, v_v, sh_v, sk_v, sd_v, wi_v, ws_v, b_v, wo_v, c_v, wm_v, vf_v,
            au0_v, au1_v, fa_v, fb_v, ya_v, yb_v, bm0_v, bp0_v, bm1_v, bp1_v,
            y_v, x1_v, h0_v, z1_v, z2_v, wt_v, wr_v, bf_v, o_v, tie_v, zero_s,
            sems, *lists):
    au_v, h_v = (au0_v, au1_v), (lists[32:41], lists[41:])
    copies = {}

    def start(group, sem, *pairs):
        copies[group] = [pltpu.make_async_copy(src, dst, sems.at[sem]) for src, dst in pairs]
        for cp in copies[group]:
            cp.start()

    def wait(*groups):
        for group in groups:
            for cp in copies[group]:
                cp.wait()

    def conv_inputs(cb, a):
        rows, lanes, sem = _ds(a * CH, CH, CH), pl.ds(cb * 128, 128), sems.at[cb % 3 * NA + a]
        return (pltpu.make_async_copy(k_h.at[rows, lanes], k_v.at[cb, _ds(PAD + a * CH, CH, PAD)], sem),
                pltpu.make_async_copy(v_h.at[rows, lanes], v_v.at[cb, rows], sem),
                pltpu.make_async_copy(sk_h.at[lanes, rows], sk_v.at[cb, a], sem))

    def fetch(stage):
        rows = lambda r, n: (q_h.at[pl.ds(r, n)], q_v.at[pl.ds(r, n)])
        if stage == 0:
            start("taps", 12, (sh_h, sh_v), (sd_h, sd_v))
        if stage < NCB:
            for a in range(NA):
                for cp in conv_inputs(stage, a):
                    cp.start()
        if stage == 0:
            start("dft", 13, (vf_h, vf_v.at[pl.ds(0, 8)]))
        if stage == NCB:
            start("mod", 8, (c_h, c_v), (wm_h.at[:, pl.ds(0, 5 * D)], wm_v.at[:, pl.ds(0, 5 * D)]), rows(0, H))
            start("gate", 9, (wi_h.at[pl.ds(FH, FH)], wi_v.at[pl.ds(0, FH)]), rows(H, H))
            start("value", 10, (wi_h.at[pl.ds(0, FH)], wi_v.at[pl.ds(FH, FH)]), rows(RB, 2 * RB))
        if stage == NCB + 2:
            start("out", 0, rows(3 * RB, RB), (wm_h.at[:, pl.ds(5 * D, D)], wm_v.at[:, pl.ds(5 * D, D)]),
                  (b_h, b_v), (wo_h, wo_v.at[pl.ds(0, FH)]))
            start("mix", 1, *[(ws_h.at[:, pl.ds(128 * j, 128)], ws_v.at[j]) for j in range(S // 128)])

    fetch(0)
    fetch(1)
    for ref in (fb_v, ya_v, tie_v):
        ref[...] = jnp.zeros(ref.shape, ref.dtype)
    k_v[:, pl.ds(0, PAD), :] = jnp.zeros((NCB, PAD, 128), BF16)
    wo_v[pl.ds(FH, 256 * KO + 128 - FH), :] = jnp.zeros((256 * KO + 128 - FH, D), BF16)
    zero_s[0] = 0
    row8 = lax.broadcasted_iota(jnp.int32, (8, 128), 0)

    def tie(after, x):
        if after is None:
            return x
        never = jnp.concatenate([tie_v[...]] * (x.shape[0] // 8), axis=0) != 0
        return jnp.where(never, after, x)

    def put(cb, slot, g, res):
        for b in range(8):
            au_v[cb % 2][b, slot, pl.ds(16 * g, 16), :] = jnp.concatenate(res[b], axis=0).astype(BF16)

    def split_filter(cb, a, after):
        kt = pltpu.bitcast(sk_v[cb, a].T, U32)
        for g in range(N2 // 8):
            u = [_phase(kt[j * N2 // 2 + g // 2 * 8:j * N2 // 2 + g // 2 * 8 + 8], g % 2) for j in range(N1)]
            if g == 0:
                u[0] = u[0] + jnp.where(row8 + a == 0, sd_v[...].astype(F32)[cb:cb + 1], 0.0)
            u[:4] = [tie(after(g), x) for x in u[:4]]
            put(cb, NA + a, g, _outer_fwd(u))

    def split_signal(cb, a, after):
        taps = [jnp.broadcast_to(sh_v[j:j + 1, pl.ds(cb * 128, 128)].astype(F32), (8, 128))
                for j in range(TAPS)]
        base = a * (CH // 2) if isinstance(a, int) else pl.multiple_of(a * (CH // 2), CH // 2)
        for g in range(N2 // 8):
            w = [tie(after(g), t) for t in taps]
            u = []
            for j in range(N1):
                r = base + j * N2 // 2 + g // 2 * 8
                lag = [_phase(_words(k_v, cb, pl.ds(r + PAD // 2 + (g % 2 - t) // 2, 8)), (g % 2 - t) % 2)
                       for t in range(TAPS)]
                u.append(_add([x * wt for x, wt in zip(lag, w)]) * _phase(_words(v_v, cb, pl.ds(r, 8)), g % 2))
            put(cb, a, g, _outer_fwd(u))

    def spectra(cb, b, half, f_ref):
        rhs = jnp.concatenate([_ld(au_v[cb % 2], b, half * NA + a) for a in range(NA)], axis=1)
        f = _nn(_ld(vf_v, b), rhs)
        for a in range(NA):
            f_ref[half * NA + a] = f[:, 128 * a:128 * a + 128]
        return f

    def product(f_ref, y_ref, plus, real_rows=None):
        for g in range(8):
            ur, ui, kr, ki = ([f_ref[o + a, pl.ds(16 * g + 8 * c, 8), :] for a in range(NA)]
                              for o in (0, NA) for c in (0, 1))
            kr, ki = ([k[0]] + [k[a] + k[a - 1] if plus else k[a] - k[a - 1] for a in range(1, NA)]
                      for k in (kr, ki))
            for a in range(NA):
                yi = _add([kr[j] * ui[a - j] + ki[j] * ur[a - j] for j in range(a + 1)])
                if real_rows is not None and g == 0:
                    rr = _add([kr[j] * ur[a - j] for j in range(a + 1)])
                    ii = _add([ki[j] * ui[a - j] for j in range(a + 1)])
                    yr = jnp.where(real_rows, 0.5 * rr, rr - ii)
                    yi = jnp.where(real_rows, 0.5 * ii, yi)
                else:
                    yr = _add([kr[j] * ur[a - j] - ki[j] * ui[a - j] for j in range(a + 1)])
                y_ref[a, pl.ds(16 * g, 16), :] = jnp.concatenate([yr, yi], axis=0).astype(BF16)

    def residues(y_ref, b, dst):
        r = _nn(_ld(vf_v, 8 + b), jnp.concatenate([_ld(y_ref, a) for a in range(NA)], axis=1))
        for a in range(NA):
            dst[a] = r[:, 128 * a:128 * a + 128]
        return r

    def stash(t):
        return ((bm0_v.at[t], bp0_v.at[t]) if t < 16 else (bm1_v.at[t - 16], bp1_v.at[t - 16]))

    def merge(cb, a, after=lambda g: None):
        src = [stash(1 + 4 * cb + b)[s] for s in (0, 1) for b in range(4)]
        for g in range(N2 // 8):
            res = [[ref[a, pl.ds(16 * g + 8 * c, 8), :] for c in (0, 1)] for ref in src]
            res[0] = [tie(after(g), x) for x in res[0]]
            res[1] = [tie(after(g), x) for x in res[1]]
            for j, y in enumerate(_outer_inv(res)):
                y_v[cb, _ds(a * CH + j * N2 + 8 * g, 8, 8), :] = y

    def transform(cb, a, dst, active=True):
        pa = (a + 3) % 4
        res = []
        if active:
            res += [spectra(cb, a, 1, fa_v), spectra(cb, a, 0, fa_v)]
        product(fb_v, yb_v, True, row8 + (3 - pa) == 0)
        res.append(residues(ya_v, pa, dst[0]))
        if active:
            res += [spectra(cb, 4 + a, 1, fb_v), spectra(cb, 4 + a, 0, fb_v)]
            product(fa_v, ya_v, False)
        res.append(residues(yb_v, 4 + pa, dst[1]))
        return res

    def conv_step(cb, i):
        steps = [UN * i + u for u in range(UN)]
        if cb < NCB:
            for a in steps:
                for cp in conv_inputs(cb, a):
                    cp.wait()
        done = []
        for a in steps if cb else ():
            done += transform(cb - 1, a, (bm0_v.at[4 * cb - 4 + a], bp0_v.at[4 * cb - 4 + a])
                              if cb < NCB else (bm1_v.at[a], bp1_v.at[a]))
        at = lambda p: done[p // 8][16 * (p % 8):16 * (p % 8) + 8, 0:128] if done and p >= 0 else None
        for u, a in enumerate(steps):
            if cb < NCB:
                split_signal(cb, a, lambda g: at(TU[8 * u + g]))
                split_filter(cb, a, lambda g: at(TK[8 * u + g]))
            else:
                for c in range(3):
                    merge(c, a, lambda g: at(TI[24 * u + 8 * c + g]))

    wait("taps")
    for cb in range(NCB + 1):
        if cb == 1:
            wait("dft")
            row, col = (lax.broadcasted_iota(jnp.int32, (128, 128), d) for d in (0, 1))
            n = (col >> 5) * 16 + (col & 7) * 2 + ((col >> 4) & 1)
            order = jnp.where(row == (n >> 3) * 16 + (col & 8) + (n & 7), 1.0, 0.0).astype(BF16)
            back = _nt(order, jnp.concatenate([vf_v[b] for b in range(8)], axis=0))
            for b in range(8):
                vf_v[8 + b] = back[:, 128 * b:128 * b + 128].astype(BF16)
        fetch(cb + 2)
        pl.loop(0, NA // UN)(functools.partial(conv_step, cb))

    wait("mod")
    transform(NCB, 0, stash(20), active=False)
    cc = c_v[...].astype(F32)
    sc = jnp.broadcast_to(cc / (1.0 + jnp.exp(-cc)), (16, D)).astype(BF16)
    mod = _nn(sc, jnp.concatenate([wm_v[:, pl.ds(i * D, D)] for i in (0, 1, 2, 4, 3)], axis=1))[0:8]
    sa, ca, ga, cb_, sb = (mod[:, i * D:(i + 1) * D] for i in range(5))
    m1, m0 = ga * (1.0 + ca), ga * sa
    n1, n0 = _GA * (1.0 + cb_), _GA * sb
    zero = zero_s[0]
    for n, (cb, a) in enumerate([(cb, a) for cb in (3, 4) for a in range(MA)]):
        merge(cb, a + zero, lambda g: mod[:, 128 * ((8 * n + g) * MS // (16 * MA)):][:, :128])

    TB = RB // 128
    PER = 2 * FH // 16

    def hidden(r0, after=(None, None)):
        out = []
        for r, a in zip((r0, r0 + 8), after):
            rows = pl.ds(r, 8)
            x = q_v[rows, :].astype(F32)
            x = jnp.concatenate([tie(a, x[:, :128]), x[:, 128:]], axis=1)
            x1 = x + (_ln_rows(x) * m1 + m0) * jnp.concatenate([y_v[j, rows, :] for j in range(NCB)], axis=1)
            x1_v[rows, :] = x1
            out.append(_ln_rows(x1) * n1 + n0)
        return jnp.concatenate(out, axis=0)

    def keep_gate(tile, z):
        lists[tile][pl.ds(zero, FH), :] = z

    def moments(tile, after):
        z, acc = lists[tile], lists[16 + tile]
        s1 = s2 = None
        for n, f in enumerate(range(0, FH, SU)):
            for r in range(f, f + SU, 8):
                d = tie(after(n)[:8] if r == f else None, z[pl.ds(r, 8), :])
                s1, s2 = (d, d * d) if s1 is None else (s1 + d, s2 + d * d)
            acc[pl.ds(16 * n + zero, 16), :] = jnp.concatenate([s1, s2], axis=0)
        s1, s2 = (jnp.sum(acc[pl.ds(16 * n + r, 8), :], axis=0, keepdims=True) for r in (0, 8))
        stats[tile] = [jnp.broadcast_to(t, (16, 128)) for t in _norm_stats(s1, s2, FH, EPS * (2 * _GA) ** 2)]

    def norm_gate(pair, after):
        for n in range(FM // 16):
            means = [tie(after(n), stats[2 * pair + c][0]) for c in (0, 1)]
            quad = [(lists[2 * pair + c][pl.ds(r + 16 * n, 16), :] - means[c]) * stats[2 * pair + c][1]
                    for r in (0, FM) for c in (0, 1)]
            for k, a in enumerate(_lhs7(*quad)):
                z2_v[k, pair, pl.ds(16 * n, 16), :] = a

    def lanes(x, j, n=1):
        return x[:, 128 * j:128 * (j + n)]

    def prepare(i, c, after):
        def put(k, n, x):
            for j in range(x.shape[1] // 128):
                h_v[i % 2][k][j, pl.ds(16 * n + zero, 16), :] = lanes(x, j).astype(BF16)

        for n in range(H // 16):
            h = hidden(i * RB + c * H + 16 * n, (after(2 * n)[:8], after(2 * n + 1)[:8]))
            top, bot = lanes(h, 0, 2), lanes(h, 2, 2)
            put(7 + c, n, lanes(h, 4))
            if c:
                half[n] = top, bot
                put(2, n, top - bot)
                put(4, n, bot)
            else:
                put(1, n, top)
                put(3, n, bot - top)
                put(0, n, top + half[n][1])
                put(5, n, top + half[n][0])
                put(6, n, bot + half[n][1])

    def turn_out(after):
        for n in range((2 * KO + 1) * NCB):
            j, t = divmod(n, NCB)
            w = _words(wo_v, pl.ds(64 * j, 64), pl.ds(128 * t, 128))
            w = jnp.concatenate([tie(pltpu.bitcast(after(n)[:8], U32), w[:8]), w[8:]], axis=0)
            wr_v[j, pl.ds(128 * t + zero, 128), :] = pltpu.bitcast(w, BF16).T

    def split_out(after):
        for n in range(KO * DM // 16):
            j, r = divmod(16 * n, DM)
            quad = [wr_v[j + KO * c, pl.ds(r + DM * b, 16), :].astype(F32) for b in (0, 1) for c in (0, 1)]
            for k, a in enumerate(_lhs7(tie(after(n), quad[0]), quad[1], quad[2], tie(after(n), quad[3]))):
                wt_v[k, j, pl.ds(r, 16), :] = a.astype(BF16)

    def side_jobs(plan, at):
        for job in plan.split(","):
            if job:
                kind, (n, *spans) = job[0], (int(x) for x in job[1:].split(":"))
                total = {"s": FH // SU, "n": FM // 16, "h": H // 8, "m": N2 // 8,
                         "t": (2 * KO + 1) * NCB, "o": KO * DM // 16}[kind]
                slots = [p for lo, hi in zip(spans[::2], spans[1::2]) for p in range(lo, hi)]
                after = lambda k: at(slots[k * len(slots) // total])
                if kind == "s":
                    moments(n, after)
                elif kind == "m":
                    merge(n // NA, n % NA + zero, lambda k: after(k)[:8])
                elif kind in "to":
                    (turn_out if kind == "t" else split_out)(after)
                elif kind == "n":
                    norm_gate(n, after)
                else:
                    prepare(n // 2, n % 2, after)

    def rows_of(z):
        per = z.shape[0] // 16
        return lambda p: z[16 * (p % per):16 * (p % per) + 16, 128 * (p // per):128 * (p // per) + 128]

    def project(i):
        def prod(*pairs):
            right = [_ld(h_v[i % 2][k], j) for _, k in pairs for j in range(2 if k < 7 else 1)]
            return _nt(jnp.concatenate([x for k, _ in pairs for x in left[k]], axis=1),
                       jnp.concatenate(right, axis=1))

        s5, s3, r12, s4, s1 = prod((4, 4)), prod((2, 2)), prod((7, 8)), prod((3, 3)), prod((0, 0))
        s7, s2, r21, s6 = prod((6, 6), (7, 7)), prod((1, 1)), prod((8, 7)), prod((5, 5), (8, 8))
        gate = [((s4 - s5) + s1) + s7, (s5 + s3) + r12]
        value = [(s4 + s2) + r21, ((s3 + s1) - s2) + s6]
        for c, later in enumerate((s2, lanes(s4, 1))):
            keep_gate(i * TB + 2 * c, _gelu_scaled(lanes(gate[c], 0)))
            keep_gate(i * TB + 2 * c + 1, _gelu_scaled(tie(lanes(later, 0) if DG else None, lanes(gate[c], 1))))
        for t in range(TB):
            z1_v[i * TB + t] = lanes(value[t // 2], t % 2)
        rounds = (s5, s3, gate[1], lanes(s4, 1), lanes(s1, 1), gate[0], s2, value[0], lanes(value[1], 1))
        return lambda p: rounds[p // (FH // 16)][16 * (p % (FH // 16)):16 * (p % (FH // 16)) + 16, 0:128]

    def first(f0, r0, n, k0, k1):
        h = jnp.concatenate([_ld(h0_v, j, pl.ds(r0 // 2, n // 2)) for j in range(k0, k1)], axis=1)
        return _nt(wi_v[pl.ds(f0, FH), pl.ds(128 * k0, 128 * (k1 - k0))], h)

    def keep_first(r, h):
        for j in range(NCB):
            h0_v[j, pl.ds(r, 16), :] = lanes(h, j).astype(BF16)

    stats, half = {}, {}
    for r in range(0, H, 16):
        keep_first(r, hidden(r))
    wait("gate")
    zero = pl.multiple_of(zero_s[0], 16)
    head = first(0, 0, H, 0, 2)
    z = _gelu_scaled(head + first(0, 0, H, 2, NCB))
    at = rows_of(jnp.concatenate([lanes(head, 0), z], axis=1))
    for n in range(H // 16):
        keep_first(H + 16 * n, hidden(H + 16 * n, [at(E0 + (2 * n + k) * ES // 8)[:8] for k in (0, 1)]))
    z = jnp.concatenate([z] + [_gelu_scaled(first(0, r, 128, 0, NCB)) for r in (H, H + 128)], axis=1)
    for t in range(TB):
        keep_gate(t, lanes(z, t))
    side_jobs(NJ[0], rows_of(z))
    wait("value")
    head = first(FH, 0, RB, NCB - 1, NCB)
    z = head + first(FH, 0, RB, 0, NCB - 1)
    for t in range(TB):
        z1_v[t] = lanes(z, t)
    side_jobs(NJ[1], rows_of(jnp.concatenate([lanes(head, 0), z], axis=1)))
    sums = [_lhs7(*(wi_v[pl.ds(FH * r, FH), pl.ds(256 * c + 128 * j, 128)].astype(F32)
                    for r in (0, 1) for c in (0, 1))) for j in (0, 1)]
    left = ([[s[k].astype(BF16) for s in sums] for k in range(7)]
            + [[wi_v[pl.ds(FH * r, FH), pl.ds(512, 128)]] for r in (0, 1)])
    for i in range(1, NB):
        if i == 2:
            wait("out")
            gb = _nn(sc, wm_v[:, pl.ds(5 * D, D)]) * (0.5 / _GA)
            bf_v[...] = b_v[...].astype(F32)
        side_jobs(NJ[i + 1], project(i))

    wait("mix")
    T2 = R2 // 128

    def mix(i):
        def w(c, r):
            return [_ld(ws_v, 2 * j + c, _ds((i * R2 + r * H) // 2, H // 2, H // 2))
                    for j in range(S // 256)]

        def comb(x, y, sign):
            return [(jnp.add if sign > 0 else jnp.subtract)(a.astype(F32), b.astype(F32)) for a, b in zip(x, y)]

        def prod(n, rhs):
            def left(k):
                def part(r, c, rows):
                    return jnp.concatenate([z2_v[n, 2 * j + c, pl.ds(FT * r, rows), :] for j in range(NB)], axis=1)

                def both(c, op):
                    top = part(0, c, FT)
                    return jnp.concatenate([op(top[:FB], part(1, 1, FB)), top[FB:]], axis=0)

                return (lambda: both(0, jnp.add), lambda: part(1, 0, FB) + part(1, 1, FB),
                        lambda: part(0, 0, FT), lambda: part(1, 1, FB),
                        lambda: part(0, 0, FT) + part(0, 1, FT), lambda: part(1, 0, FB) - part(0, 0, FB),
                        lambda: both(1, jnp.subtract))[k]().astype(BF16)

            b11, b12, b21, b22 = (
                jnp.concatenate([rhs[2 * j + c][128 * r:128 * r + 128] for j in range(NB)], axis=1)
                for c in (0, 1) for r in (0, 1))
            m = lambda k, x: _nt(left(k), x.astype(BF16))
            m2, m5 = m(1, b11), m(4, b22)
            b11, b12, b21, b22 = (x.astype(F32) for x in (b11, b12, b21, b22))
            m4 = m(3, b21 - b11)
            m1, m7, m3, m6 = m(0, b11 + b22), m(6, b21 + b22), m(2, b12 - b22), m(5, b11 + b12)
            c11 = jnp.concatenate([m4 - m5[:FB], -m5[FB:]], axis=0) + m1 + m7
            c22 = (m1[:FB] - m2) + m3[:FB] + m6
            return jnp.concatenate([jnp.concatenate([c11, m5 + m3], axis=1),
                                    jnp.concatenate([m2 + m4, c22], axis=1)], axis=0)

        def gate(r, c, g):
            tiles = [i * T2 + c * (H // 128) + t for t in range(H // 128)]
            bias = jnp.concatenate([bf_v[pl.ds(j, 1), :] for j in tiles], axis=1)
            z1 = jnp.concatenate([z1_v[j, pl.ds(FM * r, FM), :] for j in tiles], axis=1)
            return _gelu_scaled(z1) * (g + bias)

        s2 = prod(1, w(0, 0))
        s5 = prod(4, w(1, 1))
        s4 = prod(3, comb(w(1, 0), w(0, 0), -1))
        p21 = gate(1, 0, s2 + s4)
        d11 = s4 - s5
        s1 = prod(0, comb(w(0, 0), w(1, 1), 1))
        d11, d22 = d11 + s1, s1 - s2
        p11 = gate(0, 0, d11 + prod(6, comb(w(1, 0), w(1, 1), 1)))
        s3 = prod(2, comb(w(0, 1), w(1, 1), -1))
        p12 = gate(0, 1, s3 + s5)
        p22 = gate(1, 1, (d22 + s3) + prod(5, comb(w(0, 0), w(0, 1), 1)))
        return [jnp.concatenate(p, axis=0) for p in ((p11, p21), (p12, p22))]

    def flush(k):
        rows = _ds(k * H, H, H)
        return pltpu.make_async_copy(o_v.at[rows], o_h.at[rows], sems.at[2])

    def finish(r0, tile):
        for t in range(H // 128):
            for j in range(NCB):
                at = _ds(r0 + 128 * t, 128, 128), pl.ds(128 * j, 128)
                o_v[at] = (x1_v[at] + jnp.concatenate([lanes(gb, j)] * 8, axis=0)
                           * tile(t, j).T.astype(F32)).astype(BF16)

    def mix_step(i):
        p = mix(i)
        b11, b12, b21, b22 = (p[c][128 * KO * r:128 * KO * (r + 1)] for r in (0, 1) for c in (0, 1))

        def prod(n, rhs):
            return _nn(jnp.concatenate([_ld(wt_v, n, j) for j in range(KO)], axis=1), rhs.astype(BF16))

        def rest(c):
            tail = jnp.concatenate([p[c][256 * KO:], jnp.zeros((128 + 256 * KO - FH, H), F32)], axis=0)
            return _nn(_ld(wr_v, 2 * KO), tail.astype(BF16))

        r0 = rest(0)
        s2 = prod(1, b11)
        s4 = prod(3, b21 - b11)
        s5 = prod(4, b22)
        s1 = prod(0, b11 + b22)
        s7 = prod(6, b21 + b22)
        ot = jnp.concatenate([r0[:DM] + s4 - s5 + s1 + s7, r0[DM:] + s2 + s4], axis=0)
        finish(i * R2, lambda t, j: lanes(ot, t)[128 * j:128 * j + 128].astype(BF16))
        flush(2 * i).start()
        spot = _ds(i * R2 + H, 16, 16), pl.ds(0, 128)
        o_v[spot] = jnp.zeros((16, 128), BF16)
        pin = o_v[_ds(i * R2 + H + zero, 16, 16), pl.ds(0, 128)].astype(F32)
        r1 = rest(1)
        s3 = prod(2, b12 - b22)
        b = b11 + b12
        b = jnp.concatenate([b[:-16], jnp.concatenate([b[-16:, :128], tie(pin, b[-16:, 128:])], axis=1)], axis=0)
        s6 = prod(5, b)
        ot = jnp.concatenate([r1[:DM] + s5 + s3, (s1 - s2) + r1[DM:] + s3 + s6], axis=0)
        finish(i * R2 + H, lambda t, j: lanes(ot, t)[128 * j:128 * j + 128].astype(BF16))
        flush(2 * i + 1).start()

    zero = pl.multiple_of(zero_s[0], 16)
    zero = zero_s[0]
    pl.loop(0, S // R2)(mix_step)
    for k in range(S // H):
        flush(k).wait()


@jax.jit
def pallas_adaLN_cond__ssm_conv_h3__mixer_gmlp__prompt_kernel(
    A_q, A_k, A_v, A_shift_k, A_ssm_k, A_ssm_D, B_x, B_w_in, B_w_sp, B_b_sp, B_w_out, c, w_mod,
):
    del B_x
    vf = _dft_mats().astype(BF16)
    vm = pltpu.VMEM
    tile = (128, 128)
    scratch = [
        vm((S, D), BF16), vm((NCB, PAD + S, 128), BF16), vm((NCB, S, 128), BF16), vm((TAPS, D), BF16),
        vm((NCB, NA, 128, CH), BF16), vm((NCB, 128), BF16), vm((2 * FH, D), BF16),
        vm((S // 128, S, 128), BF16), vm((S // 128, 128), BF16), vm((256 * KO + 128, D), BF16), vm((1, D), BF16),
        vm((D, 6 * D), BF16), vm((16, *tile), BF16),
        vm((8, 2 * NA, *tile), BF16), vm((8, 2 * NA, *tile), BF16),
        vm((2 * NA, *tile), F32), vm((2 * NA, *tile), F32), vm((NA, *tile), BF16), vm((NA, *tile), BF16),
        vm((16, NA, *tile), F32), vm((16, NA, *tile), F32), vm((5, NA, *tile), F32), vm((5, NA, *tile), F32),
        vm((NCB, S, 128), F32), vm((S, D), F32), vm((NCB, RB, 128), BF16),
        vm((S // 128, FH, 128), F32), vm((7, S // 256, FM, 128), F32),
        vm((7, KO, DM, 128), BF16), vm((2 * KO + 1, D, 128), BF16), vm((S // 128, 128), F32),
        vm((S, D), BF16), vm((8, 128), jnp.int32), pltpu.SMEM((1,), jnp.int32),
        pltpu.SemaphoreType.DMA((14,)),
    ] + [vm((FH, 128), F32)] * 16 + [vm((FH // SU * 16, 128), F32)] * 16 + ([vm((2, H, 128), BF16)] * 7 + [vm((1, H, 128), BF16)] * 2) * 2
    out = pl.pallas_call(
        _kernel,
        out_shape=jax.ShapeDtypeStruct((S, D), BF16),
        in_specs=[pl.BlockSpec(memory_space=pltpu.HBM)] * 13,
        out_specs=pl.BlockSpec(memory_space=pltpu.HBM),
        scratch_shapes=scratch,
        compiler_params=pltpu.CompilerParams(vmem_limit_bytes=110 * 1024 * 1024),
    )(A_q.reshape(S, D), A_k.reshape(S, D), A_v.reshape(S, D), A_shift_k.T, A_ssm_k,
      A_ssm_D.reshape(NCB, 128), B_w_in.T, B_w_sp, B_b_sp.reshape(S // 128, 128), B_w_out, c, w_mod, vf)
    return out.reshape(1, S, D)
```

```python
import functools
import math

import numpy as np
import jax
import jax.numpy as jnp
from jax import lax
import jax.experimental.pallas as pl
import jax.experimental.pallas.tpu as pltpu

S, D, FH = 2048, 640, 864
FM, DM = FH // 2, D // 2
KO = FH // 256
FT, FB = 224, 208
TAPS = 4
CH = 512
NA = S // CH
N2 = 64
N1 = CH // N2
NCB = D // 128
RB = 512
NB = S // RB
H = RB // 2
EPS = 1e-5
F32, BF16, U32 = jnp.float32, jnp.bfloat16, jnp.uint32
PAD = 16

_C8 = math.cos(math.pi / 8)
_T8 = math.tan(math.pi / 8)
_R2 = math.sqrt(0.5)
_G0 = math.sqrt(2 / math.pi)
_GA = (_G0 * 0.044715) ** (1 / 3)

E0, ES = 0, 16
TU = (-1, 0, 3, 5, 16, 32, 35, 38)
TK = (34, 38, 41, 42, 43, 44, 45, 46)
TI = (-1, -1, -1, 0, 0, 2, 3, 4, 5, 5, 7, 16, 17, 17, 32, 33, 34, 36, 37, 38, 38, 39, 40, 42)
SU = 96
NJ = ["s0:70:89,s1:124:180,s2:168:205,m14:90:120,m18:120:150,m15:150:180,m19:180:210,m13:54:80,m17:70:100", "h3:0:96,h2:108:229,s3:20:80",
      "h5:0:108:132:186,h4:182:246:314:430,s4:314:402,s6:222:276",
      "h7:22:114:162:200,h6:226:280:324:440,s5:0:70,s7:54:108,s8:324:372,s10:216:246,n0:380:486",
      "s9:0:40,s11:40:80,n1:0:56,n2:56:112,n3:112:168,n4:168:224,n5:224:280,s14:160:206,s15:236:270,n7:280:344,s12:330:378,s13:380:410,n6:414:474,t0:0:320,o0:370:470"]


def _dft_mats():
    ang = [1 / 16 + m / 4 for m in range(4)] + [1 / 8, 1 / 8 + 1 / 2, 1 / 4]
    idx = np.arange(128)
    pos = (idx // 16) * 8 + idx % 8
    part = (idx // 8) % 2
    mats = []
    for b, a in enumerate(ang):
        th = 2 * np.pi * (a + pos[:, None]) * pos[None, :] / N2
        po, pi = part[:, None], part[None, :]
        m = np.where(po == pi, np.cos(th), np.where(po == 1, np.sin(th), -np.sin(th)))
        mats.append(m * ((_C8 if b < 4 else 1.0) / 8))
    n = pos + 64 * part
    th = 2 * np.pi * pos[:, None] * n[None, :] / 128
    m = np.where(part[:, None] == 0, np.cos(th), np.sin(th))
    m[8, :] = 1.0 - 2.0 * (n % 2)
    mats.append(m / 8)
    fwd = np.stack(mats).astype(np.float32)
    n = idx // 32 * 16 + idx % 8 * 2 + idx // 16 % 2
    return fwd[:, :, n // 8 * 16 + part * 8 + n % 8]


def _outer_fwd(u):
    t0r, t0i = u[0] * (1 / _C8), u[4] * (1 / _C8)
    t2r, t2i = (u[2] - u[6]) * (_R2 / _C8), (u[2] + u[6]) * (_R2 / _C8)
    t1r, t1i = u[1] - _T8 * u[5], u[5] + _T8 * u[1]
    t3r, t3i = _T8 * u[3] - u[7], _T8 * u[7] + u[3]
    ar, ai, br, bi = t0r + t2r, t0i + t2i, t0r - t2r, t0i - t2i
    cr, ci, dr, di = t1r + t3r, t1i + t3i, t1r - t3r, t1i - t3i
    out = [(ar + cr, ai + ci), (br - di, bi + dr), (ar - cr, ai - ci), (br + di, bi - dr)]
    p = [u[j] + u[j + 4] for j in range(4)]
    q = [u[j] - u[j + 4] for j in range(4)]
    er, ei = (q[1] - q[3]) * _R2, (q[1] + q[3]) * _R2
    out += [(q[0] + er, q[2] + ei), (q[0] - er, q[2] - ei)]
    out += [(p[0] - p[2], p[1] - p[3]), (p[0] + p[2], p[1] + p[3])]
    return out


def _outer_inv(B):
    ar, ai = B[0][0] + B[2][0], B[0][1] + B[2][1]
    cr, ci = B[0][0] - B[2][0], B[0][1] - B[2][1]
    br, bi = B[1][0] + B[3][0], B[1][1] + B[3][1]
    dr, di = B[1][0] - B[3][0], B[1][1] - B[3][1]
    g0r, g0i, g2r, g2i = ar + br, ai + bi, ar - br, ai - bi
    g1r, g1i, g3r, g3i = cr + di, ci - dr, cr - di, ci + dr
    nr = [g0r * (1 / _C8), g1r + _T8 * g1i, (g2r + g2i) * (_R2 / _C8), _T8 * g3r + g3i]
    ni = [g0i * (1 / _C8), g1i - _T8 * g1r, (g2i - g2r) * (_R2 / _C8), _T8 * g3i - g3r]
    fr, fi = B[4][0] - B[5][0], B[4][1] - B[5][1]
    q = [B[4][0] + B[5][0], (fr + fi) * _R2, B[4][1] + B[5][1], (fi - fr) * _R2]
    p = [B[7][0] + B[6][0], B[7][1] + B[6][1], B[7][0] - B[6][0], B[7][1] - B[6][1]]
    return ([p[j] + q[j] + nr[j] for j in range(4)]
            + [p[j] - q[j] + ni[j] for j in range(4)])


def _gelu_scaled(x):
    t = jnp.tanh(x * (_G0 / _GA + x * x))
    return x + x * t


def _norm_stats(s1, s2, n, eps):
    m = s1 * (1.0 / n)
    return m, jnp.exp(-0.5 * jnp.log(jnp.maximum(s2 * (1.0 / n) - m * m, 0.0) + eps))


def _ln_rows(x):
    m, r = _norm_stats(jnp.sum(x, axis=-1, keepdims=True), jnp.sum(x * x, axis=-1, keepdims=True),
                       x.shape[-1], EPS)
    return (x - m) * r


def _lhs7(a11, a12, a21, a22):
    return a11 + a22, a21 + a22, a11, a22, a11 + a12, a21 - a11, a12 - a22


def _words(ref, *idx):
    return ref.bitcast(U32)[idx]


def _ld(ref, *idx):
    return pltpu.bitcast(_words(ref, *idx), BF16)


def _phase(words, odd):
    return pltpu.bitcast(words & np.uint32(0xFFFF0000) if odd else words << 16, F32)


def _nn(a, b):
    return jnp.dot(a, b, preferred_element_type=F32)


def _nt(a, b):
    return lax.dot_general(a, b, (((1,), (1,)), ((), ())), preferred_element_type=F32)


def _ds(start, size, align):
    return pl.ds(start if isinstance(start, int) else pl.multiple_of(start, align), size)


def _tile(x, j, n=1):
    return x[:, 128 * j:128 * (j + n)]


def _add(xs):
    return functools.reduce(lambda x, y: x + y, xs)


def _kernel(q_h, k_h, v_h, sh_h, sk_h, sd_h, wi_h, ws_h, b_h, wo_h, c_h, wm_h, vf_h, o_h,
            q_v, k_v, v_v, sh_v, sk_v, sd_v, wi_v, ws_v, b_v, wo_v, c_v, wm_v, vf_v,
            au0_v, au1_v, fa_v, fb_v, ya_v, yb_v, bm0_v, bp0_v, bm1_v, bp1_v,
            y_v, x1_v, h0_v, z1_v, z2_v, wt_v, wr_v, bf_v, o_v, tie_v, zero_s,
            sems, *lists):
    au_v, zf_v, sum_v, h_v = (au0_v, au1_v), lists[:16], lists[16:32], (lists[32:41], lists[41:])
    copies = {}

    def start(group, sem, *pairs):
        copies[group] = [pltpu.make_async_copy(src, dst, sems.at[sem]) for src, dst in pairs]
        for cp in copies[group]:
            cp.start()

    def wait(*groups):
        for group in groups:
            for cp in copies[group]:
                cp.wait()

    def conv_inputs(cb, a):
        rows, lanes, sem = _ds(a * CH, CH, CH), pl.ds(cb * 128, 128), sems.at[cb % 3 * NA + a]
        return (pltpu.make_async_copy(k_h.at[rows, lanes], k_v.at[cb, _ds(PAD + a * CH, CH, PAD)], sem),
                pltpu.make_async_copy(v_h.at[rows, lanes], v_v.at[cb, rows], sem),
                pltpu.make_async_copy(sk_h.at[lanes, rows], sk_v.at[cb, a], sem))

    def fetch(stage):
        rows = lambda r, n: (q_h.at[pl.ds(r, n)], q_v.at[pl.ds(r, n)])
        if stage == 0:
            start("taps", 12, (sh_h, sh_v), (sd_h, sd_v))
        if stage < 3:
            for a in range(NA):
                for cp in conv_inputs(stage, a):
                    cp.start()
        if stage == 4:
            for a in range(NA):
                (k3, v3, f3), (k4, v4, _) = conv_inputs(3, a), conv_inputs(4, a)
                for cp in (k3, k4, v3, v4, f3):
                    cp.start()
            for a in range(NA):
                conv_inputs(4, a)[2].start()
        if stage == 0:
            start("dft", 13, (vf_h, vf_v.at[pl.ds(0, 8)]))
        if stage == NCB:
            start("mod", 8, (c_h, c_v), (wm_h.at[:, pl.ds(0, 5 * D)], wm_v.at[:, pl.ds(0, 5 * D)]), rows(0, H))
            start("gate", 9, (wi_h.at[pl.ds(FH, FH)], wi_v.at[pl.ds(0, FH)]), rows(H, H))
            start("value", 10, (wi_h.at[pl.ds(0, FH)], wi_v.at[pl.ds(FH, FH)]), rows(RB, 2 * RB))
        if stage == NCB + 2:
            start("out", 0, rows(3 * RB, RB), (wm_h.at[:, pl.ds(5 * D, D)], wm_v.at[:, pl.ds(5 * D, D)]),
                  (b_h, b_v), (wo_h, wo_v.at[pl.ds(0, FH)]))
            start("mix", 1, *[(ws_h.at[:, pl.ds(128 * j, 128)], ws_v.at[j]) for j in range(S // 128)])

    fetch(0)
    fetch(1)
    for ref in (fb_v, ya_v, tie_v):
        ref[...] = jnp.zeros(ref.shape, ref.dtype)
    k_v[:, pl.ds(0, PAD), :] = jnp.zeros((NCB, PAD, 128), BF16)
    wo_v[pl.ds(FH, 256 * KO + 128 - FH), :] = jnp.zeros((256 * KO + 128 - FH, D), BF16)
    zero_s[0] = 0
    row8 = lax.broadcasted_iota(jnp.int32, (8, 128), 0)

    def tie(after, x):
        if after is None:
            return x
        never = jnp.concatenate([tie_v[...]] * (x.shape[0] // 8), axis=0) != 0
        return jnp.where(never, after, x)

    def put(cb, slot, g, res):
        for b in range(8):
            au_v[cb % 2][b, slot, pl.ds(16 * g, 16), :] = jnp.concatenate(res[b], axis=0).astype(BF16)

    def split_filter(cb, a, after):
        kt = pltpu.bitcast(sk_v[cb, a].T, U32)
        for g in range(N2 // 8):
            u = [_phase(kt[j * N2 // 2 + g // 2 * 8:j * N2 // 2 + g // 2 * 8 + 8], g % 2) for j in range(N1)]
            if g == 0:
                u[0] = u[0] + jnp.where(row8 + a == 0, sd_v[...].astype(F32)[cb:cb + 1], 0.0)
            u[:4] = [tie(after(g), x) for x in u[:4]]
            put(cb, NA + a, g, _outer_fwd(u))

    def split_signal(cb, a, after):
        taps = [jnp.broadcast_to(sh_v[j:j + 1, pl.ds(cb * 128, 128)].astype(F32), (8, 128))
                for j in range(TAPS)]
        base = a * (CH // 2) if isinstance(a, int) else pl.multiple_of(a * (CH // 2), CH // 2)
        for g in range(N2 // 8):
            w = [tie(after(g), t) for t in taps]
            u = []
            for j in range(N1):
                r = base + j * N2 // 2 + g // 2 * 8
                lag = [_phase(_words(k_v, cb, pl.ds(r + PAD // 2 + (g % 2 - t) // 2, 8)), (g % 2 - t) % 2)
                       for t in range(TAPS)]
                u.append(_add([x * wt for x, wt in zip(lag, w)]) * _phase(_words(v_v, cb, pl.ds(r, 8)), g % 2))
            put(cb, a, g, _outer_fwd(u))

    def spectra(cb, b, half, f_ref):
        rhs = jnp.concatenate([_ld(au_v[cb % 2], b, half * NA + a) for a in range(NA)], axis=1)
        f = _nn(_ld(vf_v, b), rhs)
        for a in range(NA):
            f_ref[half * NA + a] = f[:, 128 * a:128 * a + 128]
        return f

    def product(f_ref, y_ref, plus, real_rows=None):
        for g in range(8):
            ur, ui, kr, ki = ([f_ref[o + a, pl.ds(16 * g + 8 * c, 8), :] for a in range(NA)]
                              for o in (0, NA) for c in (0, 1))
            kr, ki = ([k[0]] + [k[a] + k[a - 1] if plus else k[a] - k[a - 1] for a in range(1, NA)]
                      for k in (kr, ki))
            for a in range(NA):
                yi = _add([kr[j] * ui[a - j] + ki[j] * ur[a - j] for j in range(a + 1)])
                if real_rows is not None and g == 0:
                    rr = _add([kr[j] * ur[a - j] for j in range(a + 1)])
                    ii = _add([ki[j] * ui[a - j] for j in range(a + 1)])
                    yr = jnp.where(real_rows, 0.5 * rr, rr - ii)
                    yi = jnp.where(real_rows, 0.5 * ii, yi)
                else:
                    yr = _add([kr[j] * ur[a - j] - ki[j] * ui[a - j] for j in range(a + 1)])
                y_ref[a, pl.ds(16 * g, 16), :] = jnp.concatenate([yr, yi], axis=0).astype(BF16)

    def residues(y_ref, b, dst):
        r = _nn(_ld(vf_v, 8 + b), jnp.concatenate([_ld(y_ref, a) for a in range(NA)], axis=1))
        for a in range(NA):
            dst[a] = r[:, 128 * a:128 * a + 128]
        return r

    def stash(t):
        return ((bm0_v.at[t], bp0_v.at[t]) if t < 16 else (bm1_v.at[t - 16], bp1_v.at[t - 16]))

    def merge(cb, a, after=lambda g: None):
        src = [stash(1 + 4 * cb + b)[s] for s in (0, 1) for b in range(4)]
        for g in range(N2 // 8):
            res = [[ref[a, pl.ds(16 * g + 8 * c, 8), :] for c in (0, 1)] for ref in src]
            res[0] = [tie(after(g), x) for x in res[0]]
            res[1] = [tie(after(g), x) for x in res[1]]
            for j, y in enumerate(_outer_inv(res)):
                y_v[cb, _ds(a * CH + j * N2 + 8 * g, 8, 8), :] = y

    def transform(cb, a, dst, active=True):
        pa = (a + 3) % 4
        res = []
        if active:
            res += [spectra(cb, a, 1, fa_v), spectra(cb, a, 0, fa_v)]
        product(fb_v, yb_v, True, row8 + (3 - pa) == 0)
        res.append(residues(ya_v, pa, dst[0]))
        if active:
            res += [spectra(cb, 4 + a, 1, fb_v), spectra(cb, 4 + a, 0, fb_v)]
            product(fa_v, ya_v, False)
        res.append(residues(yb_v, 4 + pa, dst[1]))
        return res

    def conv_step(cb, a):
        if cb < NCB:
            for cp in conv_inputs(cb, a):
                cp.wait()
        if cb:
            done = transform(cb - 1, a, (bm0_v.at[4 * cb - 4 + a], bp0_v.at[4 * cb - 4 + a])
                             if cb < NCB else (bm1_v.at[a], bp1_v.at[a]))
        at = lambda p: done[p // 8][16 * (p % 8):16 * (p % 8) + 8, 0:128] if cb and p >= 0 else None
        if cb < NCB:
            split_signal(cb, a, lambda g: at(TU[g]))
            split_filter(cb, a, lambda g: at(TK[g]))
        else:
            for c in range(3):
                merge(c, a, lambda g: at(TI[8 * c + g]))

    wait("taps")
    for cb in range(NCB + 1):
        if cb == 1:
            wait("dft")
            row, col = (lax.broadcasted_iota(jnp.int32, (128, 128), d) for d in (0, 1))
            n = (col >> 5) * 16 + (col & 7) * 2 + ((col >> 4) & 1)
            order = jnp.where(row == (n >> 3) * 16 + (col & 8) + (n & 7), 1.0, 0.0).astype(BF16)
            back = _nt(order, jnp.concatenate([vf_v[b] for b in range(8)], axis=0))
            for b in range(8):
                vf_v[8 + b] = back[:, 128 * b:128 * b + 128].astype(BF16)
        fetch(cb + 2)
        pl.loop(0, NA)(functools.partial(conv_step, cb))

    wait("mod")
    transform(NCB, 0, stash(20), active=False)
    cc = c_v[...].astype(F32)
    sc = jnp.broadcast_to(cc / (1.0 + jnp.exp(-cc)), (16, D)).astype(BF16)
    mod = _nn(sc, jnp.concatenate([wm_v[:, pl.ds(i * D, D)] for i in (0, 1, 2, 4, 3)], axis=1))[0:8]
    sa, ca, ga, cb_, sb = (mod[:, i * D:(i + 1) * D] for i in range(5))
    m1, m0 = ga * (1.0 + ca), ga * sa
    n1, n0 = _GA * (1.0 + cb_), _GA * sb
    zero = zero_s[0]
    for n, cb in enumerate((3, 4)):
        merge(cb, zero, lambda g: _tile(mod, (8 * n + g) * 3 // 4))

    TB = RB // 128

    def hidden(r0, after=(None, None)):
        out = []
        for r, a in zip((r0, r0 + 8), after):
            rows = pl.ds(r, 8)
            x = q_v[rows, :].astype(F32)
            x = jnp.concatenate([tie(a, x[:, :128]), x[:, 128:]], axis=1)
            x1 = x + (_ln_rows(x) * m1 + m0) * jnp.concatenate([y_v[j, rows, :] for j in range(NCB)], axis=1)
            x1_v[rows, :] = x1
            out.append(_ln_rows(x1) * n1 + n0)
        return jnp.concatenate(out, axis=0)

    def keep_gate(tile, z):
        zf_v[tile][pl.ds(zero, FH), :] = z

    def moments(tile, after):
        z, acc = zf_v[tile], sum_v[tile]
        s1 = s2 = None
        for n, f in enumerate(range(0, FH, SU)):
            for r in range(f, f + SU, 8):
                d = tie(after(n)[:8] if r == f else None, z[pl.ds(r, 8), :])
                s1, s2 = (d, d * d) if s1 is None else (s1 + d, s2 + d * d)
            acc[pl.ds(16 * n + zero, 16), :] = jnp.concatenate([s1, s2], axis=0)
        s1, s2 = (jnp.sum(acc[pl.ds(16 * n + r, 8), :], axis=0, keepdims=True) for r in (0, 8))
        stats[tile] = [jnp.broadcast_to(t, (16, 128)) for t in _norm_stats(s1, s2, FH, EPS * (2 * _GA) ** 2)]

    def norm_gate(pair, after):
        for n in range(FM // 16):
            means = [tie(after(n), stats[2 * pair + c][0]) for c in (0, 1)]
            quad = [(zf_v[2 * pair + c][pl.ds(r + 16 * n, 16), :] - means[c]) * stats[2 * pair + c][1]
                    for r in (0, FM) for c in (0, 1)]
            for k, a in enumerate(_lhs7(*quad)):
                z2_v[k, pair, pl.ds(16 * n, 16), :] = a

    def prepare(i, c, after):
        def put(k, n, x):
            for j in range(x.shape[1] // 128):
                h_v[i % 2][k][j, pl.ds(16 * n + zero, 16), :] = _tile(x, j).astype(BF16)

        for n in range(H // 16):
            h = hidden(i * RB + c * H + 16 * n, (after(2 * n)[:8], after(2 * n + 1)[:8]))
            top, bot = _tile(h, 0, 2), _tile(h, 2, 2)
            put(7 + c, n, _tile(h, 4))
            if c:
                half[n] = top, bot
                put(2, n, top - bot)
                put(4, n, bot)
            else:
                put(1, n, top)
                put(3, n, bot - top)
                put(0, n, top + half[n][1])
                put(5, n, top + half[n][0])
                put(6, n, bot + half[n][1])

    def turn_out(after):
        for n in range((2 * KO + 1) * NCB):
            j, t = divmod(n, NCB)
            w = _words(wo_v, pl.ds(64 * j, 64), pl.ds(128 * t, 128))
            w = jnp.concatenate([tie(pltpu.bitcast(after(n)[:8], U32), w[:8]), w[8:]], axis=0)
            wr_v[j, pl.ds(128 * t + zero, 128), :] = pltpu.bitcast(w, BF16).T

    def split_out(after):
        for n in range(KO * DM // 16):
            j, r = divmod(16 * n, DM)
            quad = [wr_v[j + KO * c, pl.ds(r + DM * b, 16), :].astype(F32) for b in (0, 1) for c in (0, 1)]
            for k, a in enumerate(_lhs7(tie(after(n), quad[0]), quad[1], quad[2], tie(after(n), quad[3]))):
                wt_v[k, j, pl.ds(r, 16), :] = a.astype(BF16)

    def side_jobs(plan, at):
        for job in plan.split(","):
            if job:
                kind, (n, *spans) = job[0], (int(x) for x in job[1:].split(":"))
                total = {"s": FH // SU, "n": FM // 16, "h": H // 8, "m": N2 // 8,
                         "t": (2 * KO + 1) * NCB, "o": KO * DM // 16}[kind]
                slots = [p for lo, hi in zip(spans[::2], spans[1::2]) for p in range(lo, hi)]
                after = lambda k: at(slots[k * len(slots) // total])
                if kind == "s":
                    moments(n, after)
                elif kind == "m":
                    merge(n // NA, n % NA + zero, lambda k: after(k)[:8])
                elif kind in "to":
                    (turn_out if kind == "t" else split_out)(after)
                elif kind == "n":
                    norm_gate(n, after)
                else:
                    prepare(n // 2, n % 2, after)

    def rows_of(z):
        per = z.shape[0] // 16
        return lambda p: z[16 * (p % per):16 * (p % per) + 16, 128 * (p // per):128 * (p // per) + 128]

    def project(i):
        def prod(*pairs):
            right = [_ld(h_v[i % 2][k], j) for _, k in pairs for j in range(2 if k < 7 else 1)]
            return _nt(jnp.concatenate([x for k, _ in pairs for x in left[k]], axis=1),
                       jnp.concatenate(right, axis=1))

        s5, s3, r12, s4, s1 = prod((4, 4)), prod((2, 2)), prod((7, 8)), prod((3, 3)), prod((0, 0))
        s7, s2, r21, s6 = prod((6, 6), (7, 7)), prod((1, 1)), prod((8, 7)), prod((5, 5), (8, 8))
        gate = [((s4 - s5) + s1) + s7, (s5 + s3) + r12]
        value = [(s4 + s2) + r21, ((s3 + s1) - s2) + s6]
        for t in range(TB):
            keep_gate(i * TB + t, _gelu_scaled(_tile(gate[t // 2], t % 2)))
            z1_v[i * TB + t] = _tile(value[t // 2], t % 2)
        rounds = (s5, s3, gate[1], _tile(s4, 1), _tile(s1, 1), gate[0], s2, value[0], _tile(value[1], 1))
        return lambda p: rounds[p // (FH // 16)][16 * (p % (FH // 16)):16 * (p % (FH // 16)) + 16, 0:128]

    def first(f0, r0, n, k0, k1):
        h = jnp.concatenate([_ld(h0_v, j, pl.ds(r0 // 2, n // 2)) for j in range(k0, k1)], axis=1)
        return _nt(wi_v[pl.ds(f0, FH), pl.ds(128 * k0, 128 * (k1 - k0))], h)

    def keep_first(r, h):
        for j in range(NCB):
            h0_v[j, pl.ds(r, 16), :] = _tile(h, j).astype(BF16)

    stats, half = {}, {}
    for r in range(0, H, 16):
        keep_first(r, hidden(r))
    wait("gate")
    zero = pl.multiple_of(zero_s[0], 16)
    head = first(0, 0, H, 0, 2)
    z = _gelu_scaled(head + first(0, 0, H, 2, NCB))
    at = rows_of(jnp.concatenate([_tile(head, 0), z], axis=1))
    for n in range(H // 16):
        keep_first(H + 16 * n, hidden(H + 16 * n, [at(E0 + (2 * n + k) * ES // 8)[:8] for k in (0, 1)]))
    z = jnp.concatenate([z] + [_gelu_scaled(first(0, r, 128, 0, NCB)) for r in (H, H + 128)], axis=1)
    for t in range(TB):
        keep_gate(t, _tile(z, t))
    side_jobs(NJ[0], rows_of(z))
    wait("value")
    head = first(FH, 0, RB, NCB - 1, NCB)
    z = head + first(FH, 0, RB, 0, NCB - 1)
    for t in range(TB):
        z1_v[t] = _tile(z, t)
    side_jobs(NJ[1], rows_of(jnp.concatenate([_tile(head, 0), z], axis=1)))
    sums = [_lhs7(*(wi_v[pl.ds(FH * r, FH), pl.ds(256 * c + 128 * j, 128)].astype(F32)
                    for r in (0, 1) for c in (0, 1))) for j in (0, 1)]
    left = ([[s[k].astype(BF16) for s in sums] for k in range(7)]
            + [[wi_v[pl.ds(FH * r, FH), pl.ds(512, 128)]] for r in (0, 1)])
    for i in range(1, NB):
        if i == 2:
            wait("out")
            gb = _nn(sc, wm_v[:, pl.ds(5 * D, D)]) * (0.5 / _GA)
            bf_v[...] = b_v[...].astype(F32)
        side_jobs(NJ[i + 1], project(i))

    wait("mix")

    def mix(i):
        def w(c, r):
            return [_ld(ws_v, 2 * j + c, _ds((i * RB + r * H) // 2, H // 2, H // 2))
                    for j in range(S // 256)]

        def comb(x, y, sign):
            return [(jnp.add if sign > 0 else jnp.subtract)(a.astype(F32), b.astype(F32)) for a, b in zip(x, y)]

        def prod(n, rhs):
            def left(k):
                def part(r, c, rows):
                    return jnp.concatenate([z2_v[n, 2 * j + c, pl.ds(FT * r, rows), :] for j in range(NB)], axis=1)

                def both(c, op):
                    top = part(0, c, FT)
                    return jnp.concatenate([op(top[:FB], part(1, 1, FB)), top[FB:]], axis=0)

                return (lambda: both(0, jnp.add), lambda: part(1, 0, FB) + part(1, 1, FB),
                        lambda: part(0, 0, FT), lambda: part(1, 1, FB),
                        lambda: part(0, 0, FT) + part(0, 1, FT), lambda: part(1, 0, FB) - part(0, 0, FB),
                        lambda: both(1, jnp.subtract))[k]().astype(BF16)

            b11, b12, b21, b22 = (
                jnp.concatenate([rhs[2 * j + c][128 * r:128 * r + 128] for j in range(NB)], axis=1)
                for c in (0, 1) for r in (0, 1))
            m = lambda k, x: _nt(left(k), x.astype(BF16))
            m2, m5 = m(1, b11), m(4, b22)
            b11, b12, b21, b22 = (x.astype(F32) for x in (b11, b12, b21, b22))
            m4 = m(3, b21 - b11)
            m1, m7, m3, m6 = m(0, b11 + b22), m(6, b21 + b22), m(2, b12 - b22), m(5, b11 + b12)
            c11 = jnp.concatenate([m4 - m5[:FB], -m5[FB:]], axis=0) + m1 + m7
            c22 = (m1[:FB] - m2) + m3[:FB] + m6
            return jnp.concatenate([jnp.concatenate([c11, m5 + m3], axis=1),
                                    jnp.concatenate([m2 + m4, c22], axis=1)], axis=0)

        def gate(r, c, g):
            tiles = [i * TB + c * (H // 128) + t for t in range(H // 128)]
            bias = jnp.concatenate([bf_v[pl.ds(j, 1), :] for j in tiles], axis=1)
            z1 = jnp.concatenate([z1_v[j, pl.ds(FM * r, FM), :] for j in tiles], axis=1)
            return _gelu_scaled(z1) * (g + bias)

        s2 = prod(1, w(0, 0))
        s5 = prod(4, w(1, 1))
        s4 = prod(3, comb(w(1, 0), w(0, 0), -1))
        p21 = gate(1, 0, s2 + s4)
        d11 = s4 - s5
        s1 = prod(0, comb(w(0, 0), w(1, 1), 1))
        d11, d22 = d11 + s1, s1 - s2
        p11 = gate(0, 0, d11 + prod(6, comb(w(1, 0), w(1, 1), 1)))
        s3 = prod(2, comb(w(0, 1), w(1, 1), -1))
        p12 = gate(0, 1, s3 + s5)
        p22 = gate(1, 1, (d22 + s3) + prod(5, comb(w(0, 0), w(0, 1), 1)))
        return [jnp.concatenate(p, axis=0) for p in ((p11, p21), (p12, p22))]

    def flush(k):
        rows = _ds(k * H, H, H)
        return pltpu.make_async_copy(o_v.at[rows], o_h.at[rows], sems.at[2])

    def finish(r0, tile):
        for t in range(H // 128):
            for j in range(NCB):
                at = _ds(r0 + 128 * t, 128, 128), pl.ds(128 * j, 128)
                o_v[at] = (x1_v[at] + jnp.concatenate([_tile(gb, j)] * 8, axis=0)
                           * tile(t, j).T.astype(F32)).astype(BF16)

    def mix_step(i):
        p = mix(i)
        b11, b12, b21, b22 = (p[c][128 * KO * r:128 * KO * (r + 1)] for r in (0, 1) for c in (0, 1))

        def prod(n, rhs):
            return _nn(jnp.concatenate([_ld(wt_v, n, j) for j in range(KO)], axis=1), rhs.astype(BF16))

        def rest(c):
            tail = jnp.concatenate([p[c][256 * KO:], jnp.zeros((128 + 256 * KO - FH, H), F32)], axis=0)
            return _nn(_ld(wr_v, 2 * KO), tail.astype(BF16))

        r0 = rest(0)
        s2 = prod(1, b11)
        s4 = prod(3, b21 - b11)
        s5 = prod(4, b22)
        s1 = prod(0, b11 + b22)
        s7 = prod(6, b21 + b22)
        ot = jnp.concatenate([r0[:DM] + s4 - s5 + s1 + s7, r0[DM:] + s2 + s4], axis=0)
        finish(i * RB, lambda t, j: _tile(ot, t)[128 * j:128 * j + 128].astype(BF16))
        flush(2 * i).start()
        spot = _ds(i * RB + H, 16, 16), pl.ds(0, 128)
        o_v[spot] = jnp.zeros((16, 128), BF16)
        pin = o_v[_ds(i * RB + H + zero, 16, 16), pl.ds(0, 128)].astype(F32)
        r1 = rest(1)
        s3 = prod(2, b12 - b22)
        b = b11 + b12
        b = jnp.concatenate([b[:-16], jnp.concatenate([b[-16:, :128], tie(pin, b[-16:, 128:])], axis=1)], axis=0)
        s6 = prod(5, b)
        ot = jnp.concatenate([r1[:DM] + s5 + s3, (s1 - s2) + r1[DM:] + s3 + s6], axis=0)
        finish(i * RB + H, lambda t, j: _tile(ot, t)[128 * j:128 * j + 128].astype(BF16))
        flush(2 * i + 1).start()

    zero = pl.multiple_of(zero_s[0], 16)
    zero = zero_s[0]
    pl.loop(0, NB)(mix_step)
    for k in range(S // H):
        flush(k).wait()


@jax.jit
def pallas_adaLN_cond__ssm_conv_h3__mixer_gmlp__prompt_kernel(
    A_q, A_k, A_v, A_shift_k, A_ssm_k, A_ssm_D, B_x, B_w_in, B_w_sp, B_b_sp, B_w_out, c, w_mod,
):
    del B_x
    vf = _dft_mats().astype(BF16)
    vm = pltpu.VMEM
    tile = (128, 128)
    scratch = [
        vm((S, D), BF16), vm((NCB, PAD + S, 128), BF16), vm((NCB, S, 128), BF16), vm((TAPS, D), BF16),
        vm((NCB, NA, 128, CH), BF16), vm((NCB, 128), BF16), vm((2 * FH, D), BF16),
        vm((S // 128, S, 128), BF16), vm((S // 128, 128), BF16), vm((256 * KO + 128, D), BF16), vm((1, D), BF16),
        vm((D, 6 * D), BF16), vm((16, *tile), BF16),
        vm((8, 2 * NA, *tile), BF16), vm((8, 2 * NA, *tile), BF16),
        vm((2 * NA, *tile), F32), vm((2 * NA, *tile), F32), vm((NA, *tile), BF16), vm((NA, *tile), BF16),
        vm((16, NA, *tile), F32), vm((16, NA, *tile), F32), vm((5, NA, *tile), F32), vm((5, NA, *tile), F32),
        vm((NCB, S, 128), F32), vm((S, D), F32), vm((NCB, RB, 128), BF16),
        vm((S // 128, FH, 128), F32), vm((7, S // 256, FM, 128), F32),
        vm((7, KO, DM, 128), BF16), vm((2 * KO + 1, D, 128), BF16), vm((S // 128, 128), F32),
        vm((S, D), BF16), vm((8, 128), jnp.int32), pltpu.SMEM((1,), jnp.int32),
        pltpu.SemaphoreType.DMA((14,)),
    ] + [vm((FH, 128), F32)] * 16 + [vm((FH // SU * 16, 128), F32)] * 16 + ([vm((2, H, 128), BF16)] * 7 + [vm((1, H, 128), BF16)] * 2) * 2
    out = pl.pallas_call(
        _kernel,
        out_shape=jax.ShapeDtypeStruct((S, D), BF16),
        in_specs=[pl.BlockSpec(memory_space=pltpu.HBM)] * 13,
        out_specs=pl.BlockSpec(memory_space=pltpu.HBM),
        scratch_shapes=scratch,
        compiler_params=pltpu.CompilerParams(vmem_limit_bytes=110 * 1024 * 1024),
    )(A_q.reshape(S, D), A_k.reshape(S, D), A_v.reshape(S, D), A_shift_k.T, A_ssm_k,
      A_ssm_D.reshape(NCB, 128), B_w_in.T, B_w_sp, B_b_sp.reshape(S // 128, 128), B_w_out, c, w_mod, vf)
    return out.reshape(1, S, D)
```

```python
import functools
import math

import numpy as np
import jax
import jax.numpy as jnp
from jax import lax
import jax.experimental.pallas as pl
import jax.experimental.pallas.tpu as pltpu

S, D, FH = 2048, 640, 864
FM, DM = FH // 2, D // 2
KO = FH // 256
FT, FB = 224, 208
TAPS = 4
CH = 512
NA = S // CH
N2 = 64
N1 = CH // N2
NCB = D // 128
RB = 512
NB = S // RB
H = RB // 2
EPS = 1e-5
F32, BF16, U32 = jnp.float32, jnp.bfloat16, jnp.uint32
PAD = 16

_C8 = math.cos(math.pi / 8)
_T8 = math.tan(math.pi / 8)
_R2 = math.sqrt(0.5)
_G0 = math.sqrt(2 / math.pi)
_GA = (_G0 * 0.044715) ** (1 / 3)

E0, ES = 0, 16
TU = (-1, 0, 3, 5, 16, 32, 35, 38)
TK = (34, 38, 41, 42, 43, 44, 45, 46)
TI = (-1, -1, -1, 0, 0, 2, 3, 4, 5, 5, 7, 16, 17, 17, 32, 33, 34, 36, 37, 38, 38, 39, 40, 42)
SU = 24
NJ = ["s0:70:89,s1:124:180,s2:168:205,m14:90:120,m18:120:150,m15:150:180,m19:180:210,m13:54:80,m17:70:100", "h3:0:96,h2:108:229,s3:20:80",
      "h5:0:108:132:186,h4:182:246:314:430,s4:314:402,s6:222:276",
      "h7:22:114:162:200,h6:226:280:324:440,s5:0:70,s7:54:108,s8:324:372,s10:216:246,n0:380:486",
      "s9:0:40,s11:40:80,n1:0:56,n2:56:112,n3:112:168,n4:168:224,n5:224:280,s14:160:206,s15:236:270,n7:280:344,s12:330:378,s13:380:410,n6:414:474,t0:0:320,o0:370:470"]


def _dft_mats():
    def turn(k):
        return [jnp.cos(((k - s) & 1023).astype(F32) * (2 * math.pi / 1024)) for s in (0, 256)]

    def times(x, y, i):
        return [x[0] * y[0][i:i + 1] - x[1] * y[1][i:i + 1], x[0] * y[1][i:i + 1] + x[1] * y[0][i:i + 1]]

    row, col = (lax.broadcasted_iota(jnp.int32, (8, 128), d) for d in (0, 1))
    n, imag = (col >> 5) * 16 + (col & 7) * 2 + ((col >> 4) & 1), (col >> 3) & 1
    root = jnp.where(row < 4, 1 + 4 * row, jnp.where(row < 6, 8 * row - 30, 4))
    root = [t * jnp.where(row < 4, _C8 / 8, 1 / 8) for t in turn(root * n + 256 * imag)]
    fine, coarse = turn(16 * row * n), turn(128 * row * n)
    rows = [[t for g in range(8) for t in times(base, coarse, g)]
            for base in (times(fine, root, b) for b in range(7))]
    n = n + 64 * imag
    fine, coarse = [t * (1 / 8) for t in turn(8 * row * n)], turn(64 * row * n)
    last = [t for g in range(8) for t in times(fine, coarse, g)]
    last[1] = jnp.where(row == 0, (1 - 2 * (n & 1)).astype(F32) * (1 / 8), last[1])
    return [jnp.concatenate(r, axis=0).astype(BF16) for r in rows + [last]]


def _outer_fwd(u):
    t0r, t0i = u[0] * (1 / _C8), u[4] * (1 / _C8)
    t2r, t2i = (u[2] - u[6]) * (_R2 / _C8), (u[2] + u[6]) * (_R2 / _C8)
    t1r, t1i = u[1] - _T8 * u[5], u[5] + _T8 * u[1]
    t3r, t3i = _T8 * u[3] - u[7], _T8 * u[7] + u[3]
    ar, ai, br, bi = t0r + t2r, t0i + t2i, t0r - t2r, t0i - t2i
    cr, ci, dr, di = t1r + t3r, t1i + t3i, t1r - t3r, t1i - t3i
    out = [(ar + cr, ai + ci), (br - di, bi + dr), (ar - cr, ai - ci), (br + di, bi - dr)]
    p = [u[j] + u[j + 4] for j in range(4)]
    q = [u[j] - u[j + 4] for j in range(4)]
    er, ei = (q[1] - q[3]) * _R2, (q[1] + q[3]) * _R2
    out += [(q[0] + er, q[2] + ei), (q[0] - er, q[2] - ei)]
    out += [(p[0] - p[2], p[1] - p[3]), (p[0] + p[2], p[1] + p[3])]
    return out


def _outer_inv(B):
    ar, ai = B[0][0] + B[2][0], B[0][1] + B[2][1]
    cr, ci = B[0][0] - B[2][0], B[0][1] - B[2][1]
    br, bi = B[1][0] + B[3][0], B[1][1] + B[3][1]
    dr, di = B[1][0] - B[3][0], B[1][1] - B[3][1]
    g0r, g0i, g2r, g2i = ar + br, ai + bi, ar - br, ai - bi
    g1r, g1i, g3r, g3i = cr + di, ci - dr, cr - di, ci + dr
    nr = [g0r * (1 / _C8), g1r + _T8 * g1i, (g2r + g2i) * (_R2 / _C8), _T8 * g3r + g3i]
    ni = [g0i * (1 / _C8), g1i - _T8 * g1r, (g2i - g2r) * (_R2 / _C8), _T8 * g3i - g3r]
    fr, fi = B[4][0] - B[5][0], B[4][1] - B[5][1]
    q = [B[4][0] + B[5][0], (fr + fi) * _R2, B[4][1] + B[5][1], (fi - fr) * _R2]
    p = [B[7][0] + B[6][0], B[7][1] + B[6][1], B[7][0] - B[6][0], B[7][1] - B[6][1]]
    return ([p[j] + q[j] + nr[j] for j in range(4)]
            + [p[j] - q[j] + ni[j] for j in range(4)])


def _gelu_scaled(x):
    t = jnp.tanh(x * (_G0 / _GA + x * x))
    return x + x * t


def _norm_stats(s1, s2, n, eps):
    m = s1 * (1.0 / n)
    return m, jnp.exp(-0.5 * jnp.log(jnp.maximum(s2 * (1.0 / n) - m * m, 0.0) + eps))


def _ln_rows(x):
    m, r = _norm_stats(jnp.sum(x, axis=-1, keepdims=True), jnp.sum(x * x, axis=-1, keepdims=True),
                       x.shape[-1], EPS)
    return (x - m) * r


def _lhs7(a11, a12, a21, a22):
    return a11 + a22, a21 + a22, a11, a22, a11 + a12, a21 - a11, a12 - a22


def _words(ref, *idx):
    return ref.bitcast(U32)[idx]


def _ld(ref, *idx):
    return pltpu.bitcast(_words(ref, *idx), BF16)


def _phase(words, odd):
    return pltpu.bitcast(words & np.uint32(0xFFFF0000) if odd else words << 16, F32)


def _nn(a, b):
    return jnp.dot(a, b, preferred_element_type=F32)


def _nt(a, b):
    return lax.dot_general(a, b, (((1,), (1,)), ((), ())), preferred_element_type=F32)


def _ds(start, size, align):
    return pl.ds(start if isinstance(start, int) else pl.multiple_of(start, align), size)


def _tile(x, j, n=1):
    return x[:, 128 * j:128 * (j + n)]


def _add(xs):
    return functools.reduce(lambda x, y: x + y, xs)


def _kernel(q_h, k_h, v_h, sh_h, sk_h, sd_h, wi_h, ws_h, b_h, wo_h, c_h, wm_h, o_h,
            q_v, k_v, v_v, sh_v, sk_v, sd_v, wi_v, ws_v, b_v, wo_v, c_v, wm_v, vf_v,
            au0_v, au1_v, fa_v, fb_v, ya_v, yb_v, bm0_v, bp0_v, bm1_v, bp1_v,
            y_v, x1_v, h0_v, z1_v, z2_v, wt_v, wr_v, bf_v, o_v, tie_v, zero_s,
            sems, *lists):
    au_v, zf_v, sum_v, h_v = (au0_v, au1_v), lists[:16], lists[16:32], (lists[32:41], lists[41:])
    copies = {}

    def start(group, sem, *pairs):
        copies[group] = [pltpu.make_async_copy(src, dst, sems.at[sem]) for src, dst in pairs]
        for cp in copies[group]:
            cp.start()

    def wait(*groups):
        for group in groups:
            for cp in copies[group]:
                cp.wait()

    def conv_inputs(cb, a):
        rows, lanes, sem = _ds(a * CH, CH, CH), pl.ds(cb * 128, 128), sems.at[cb % 3 * NA + a]
        return (pltpu.make_async_copy(k_h.at[rows, lanes], k_v.at[cb, _ds(PAD + a * CH, CH, PAD)], sem),
                pltpu.make_async_copy(v_h.at[rows, lanes], v_v.at[cb, rows], sem),
                pltpu.make_async_copy(sk_h.at[lanes, rows], sk_v.at[cb, a], sem))

    def fetch(stage):
        rows = lambda r, n: (q_h.at[pl.ds(r, n)], q_v.at[pl.ds(r, n)])
        if stage == 0:
            start("taps", 12, (sh_h, sh_v), (sd_h, sd_v))
        if stage < 3:
            for a in range(NA):
                for cp in conv_inputs(stage, a):
                    cp.start()
        if stage == 4:
            for a in range(NA):
                (k3, v3, f3), (k4, v4, _) = conv_inputs(3, a), conv_inputs(4, a)
                for cp in (k3, k4, v3, v4, f3):
                    cp.start()
            for a in range(NA):
                conv_inputs(4, a)[2].start()
        if stage == NCB:
            start("mod", 8, (c_h, c_v), (wm_h.at[:, pl.ds(0, 5 * D)], wm_v.at[:, pl.ds(0, 5 * D)]), rows(0, H))
            start("gate", 9, (wi_h.at[pl.ds(FH, FH)], wi_v.at[pl.ds(0, FH)]), rows(H, H))
            start("value", 10, (wi_h.at[pl.ds(0, FH)], wi_v.at[pl.ds(FH, FH)]), rows(RB, 2 * RB))
        if stage == NCB + 2:
            start("out", 0, rows(3 * RB, RB), (wm_h.at[:, pl.ds(5 * D, D)], wm_v.at[:, pl.ds(5 * D, D)]),
                  (b_h, b_v), (wo_h, wo_v.at[pl.ds(0, FH)]))
            start("mix", 1, *[(ws_h.at[:, pl.ds(128 * j, 128)], ws_v.at[j]) for j in range(S // 128)])

    fetch(0)
    fetch(1)
    for ref in (fb_v, ya_v, tie_v):
        ref[...] = jnp.zeros(ref.shape, ref.dtype)
    k_v[:, pl.ds(0, PAD), :] = jnp.zeros((NCB, PAD, 128), BF16)
    wo_v[pl.ds(FH, 256 * KO + 128 - FH), :] = jnp.zeros((256 * KO + 128 - FH, D), BF16)
    row, col = (lax.broadcasted_iota(jnp.int32, (128, 128), d) for d in (0, 1))
    n = (col >> 5) * 16 + (col & 7) * 2 + ((col >> 4) & 1)
    order = jnp.where(row == (n >> 3) * 16 + (col & 8) + (n & 7), 1.0, 0.0).astype(BF16)
    mats = _dft_mats()
    back = _nt(order, jnp.concatenate(mats, axis=0))
    for b in range(8):
        vf_v[b] = mats[b]
        vf_v[8 + b] = _tile(back, b).astype(BF16)
    zero_s[0] = 0
    row8 = lax.broadcasted_iota(jnp.int32, (8, 128), 0)

    def tie(after, x):
        if after is None:
            return x
        never = jnp.concatenate([tie_v[...]] * (x.shape[0] // 8), axis=0) != 0
        return jnp.where(never, after, x)

    def put(cb, slot, g, res):
        for b in range(8):
            au_v[cb % 2][b, slot, pl.ds(16 * g, 16), :] = jnp.concatenate(res[b], axis=0).astype(BF16)

    def split_filter(cb, a, after):
        kt = pltpu.bitcast(sk_v[cb, a].T, U32)
        for g in range(N2 // 8):
            u = [_phase(kt[j * N2 // 2 + g // 2 * 8:j * N2 // 2 + g // 2 * 8 + 8], g % 2) for j in range(N1)]
            if g == 0:
                u[0] = u[0] + jnp.where(row8 + a == 0, sd_v[...].astype(F32)[cb:cb + 1], 0.0)
            u[:4] = [tie(after(g), x) for x in u[:4]]
            put(cb, NA + a, g, _outer_fwd(u))

    def split_signal(cb, a, after):
        taps = [jnp.broadcast_to(sh_v[j:j + 1, pl.ds(cb * 128, 128)].astype(F32), (8, 128))
                for j in range(TAPS)]
        base = a * (CH // 2) if isinstance(a, int) else pl.multiple_of(a * (CH // 2), CH // 2)
        for g in range(N2 // 8):
            w = [tie(after(g), t) for t in taps]
            u = []
            for j in range(N1):
                r = base + j * N2 // 2 + g // 2 * 8
                lag = [_phase(_words(k_v, cb, pl.ds(r + PAD // 2 + (g % 2 - t) // 2, 8)), (g % 2 - t) % 2)
                       for t in range(TAPS)]
                u.append(_add([x * wt for x, wt in zip(lag, w)]) * _phase(_words(v_v, cb, pl.ds(r, 8)), g % 2))
            put(cb, a, g, _outer_fwd(u))

    def spectra(cb, b, half, f_ref):
        rhs = jnp.concatenate([_ld(au_v[cb % 2], b, half * NA + a) for a in range(NA)], axis=1)
        f = _nn(_ld(vf_v, b), rhs)
        for a in range(NA):
            f_ref[half * NA + a] = f[:, 128 * a:128 * a + 128]
        return f

    def product(f_ref, y_ref, plus, real_rows=None):
        for g in range(8):
            ur, ui, kr, ki = ([f_ref[o + a, pl.ds(16 * g + 8 * c, 8), :] for a in range(NA)]
                              for o in (0, NA) for c in (0, 1))
            kr, ki = ([k[0]] + [k[a] + k[a - 1] if plus else k[a] - k[a - 1] for a in range(1, NA)]
                      for k in (kr, ki))
            for a in range(NA):
                yi = _add([kr[j] * ui[a - j] + ki[j] * ur[a - j] for j in range(a + 1)])
                if real_rows is not None and g == 0:
                    rr = _add([kr[j] * ur[a - j] for j in range(a + 1)])
                    ii = _add([ki[j] * ui[a - j] for j in range(a + 1)])
                    yr = jnp.where(real_rows, 0.5 * rr, rr - ii)
                    yi = jnp.where(real_rows, 0.5 * ii, yi)
                else:
                    yr = _add([kr[j] * ur[a - j] - ki[j] * ui[a - j] for j in range(a + 1)])
                y_ref[a, pl.ds(16 * g, 16), :] = jnp.concatenate([yr, yi], axis=0).astype(BF16)

    def residues(y_ref, b, dst):
        r = _nn(_ld(vf_v, 8 + b), jnp.concatenate([_ld(y_ref, a) for a in range(NA)], axis=1))
        for a in range(NA):
            dst[a] = r[:, 128 * a:128 * a + 128]
        return r

    def stash(t):
        return ((bm0_v.at[t], bp0_v.at[t]) if t < 16 else (bm1_v.at[t - 16], bp1_v.at[t - 16]))

    def merge(cb, a, after=lambda g: None):
        src = [stash(1 + 4 * cb + b)[s] for s in (0, 1) for b in range(4)]
        for g in range(N2 // 8):
            res = [[ref[a, pl.ds(16 * g + 8 * c, 8), :] for c in (0, 1)] for ref in src]
            res[0] = [tie(after(g), x) for x in res[0]]
            res[1] = [tie(after(g), x) for x in res[1]]
            for j, y in enumerate(_outer_inv(res)):
                y_v[cb, _ds(a * CH + j * N2 + 8 * g, 8, 8), :] = y

    def transform(cb, a, dst, active=True):
        pa = (a + 3) % 4
        res = []
        if active:
            res += [spectra(cb, a, 1, fa_v), spectra(cb, a, 0, fa_v)]
        product(fb_v, yb_v, True, row8 + (3 - pa) == 0)
        res.append(residues(ya_v, pa, dst[0]))
        if active:
            res += [spectra(cb, 4 + a, 1, fb_v), spectra(cb, 4 + a, 0, fb_v)]
            product(fa_v, ya_v, False)
        res.append(residues(yb_v, 4 + pa, dst[1]))
        return res

    def conv_step(cb, a):
        if cb < NCB:
            for cp in conv_inputs(cb, a):
                cp.wait()
        if cb:
            done = transform(cb - 1, a, (bm0_v.at[4 * cb - 4 + a], bp0_v.at[4 * cb - 4 + a])
                             if cb < NCB else (bm1_v.at[a], bp1_v.at[a]))
        at = lambda p: done[p // 8][16 * (p % 8):16 * (p % 8) + 8, 0:128] if cb and p >= 0 else None
        if cb < NCB:
            split_signal(cb, a, lambda g: at(TU[g]))
            split_filter(cb, a, lambda g: at(TK[g]))
        else:
            for c in range(3):
                merge(c, a, lambda g: at(TI[8 * c + g]))

    wait("taps")
    for cb in range(NCB + 1):
        fetch(cb + 2)
        pl.loop(0, NA)(functools.partial(conv_step, cb))

    wait("mod")
    transform(NCB, 0, stash(20), active=False)
    cc = c_v[...].astype(F32)
    sc = jnp.broadcast_to(cc / (1.0 + jnp.exp(-cc)), (16, D)).astype(BF16)
    mod = _nn(sc, jnp.concatenate([wm_v[:, pl.ds(i * D, D)] for i in (0, 1, 2, 4, 3)], axis=1))[0:8]
    sa, ca, ga, cb_, sb = (mod[:, i * D:(i + 1) * D] for i in range(5))
    m1, m0 = ga * (1.0 + ca), ga * sa
    n1, n0 = _GA * (1.0 + cb_), _GA * sb
    zero = zero_s[0]
    for n, cb in enumerate((3, 4)):
        merge(cb, zero, lambda g: _tile(mod, (8 * n + g) * 3 // 4))

    TB = RB // 128

    def hidden(r0, after=(None, None)):
        out = []
        for r, a in zip((r0, r0 + 8), after):
            rows = pl.ds(r, 8)
            x = q_v[rows, :].astype(F32)
            x = jnp.concatenate([tie(a, x[:, :128]), x[:, 128:]], axis=1)
            x1 = x + (_ln_rows(x) * m1 + m0) * jnp.concatenate([y_v[j, rows, :] for j in range(NCB)], axis=1)
            x1_v[rows, :] = x1
            out.append(_ln_rows(x1) * n1 + n0)
        return jnp.concatenate(out, axis=0)

    def keep_gate(tile, z):
        zf_v[tile][pl.ds(zero, FH), :] = z

    def moments(tile, after):
        z, acc = zf_v[tile], sum_v[tile]
        s1 = s2 = None
        for n, f in enumerate(range(0, FH, SU)):
            for r in range(f, f + SU, 8):
                d = tie(after(n)[:8] if r == f else None, z[pl.ds(r, 8), :])
                s1, s2 = (d, d * d) if s1 is None else (s1 + d, s2 + d * d)
            acc[pl.ds(16 * n + zero, 16), :] = jnp.concatenate([s1, s2], axis=0)
        s1, s2 = (jnp.sum(acc[pl.ds(16 * n + r, 8), :], axis=0, keepdims=True) for r in (0, 8))
        stats[tile] = [jnp.broadcast_to(t, (8, 128)) for t in _norm_stats(s1, s2, FH, EPS * (2 * _GA) ** 2)]

    def norm_gate(pair, after):
        for n in range(FM // 8):
            means = [tie(after(n)[:8], stats[2 * pair + c][0]) for c in (0, 1)]
            quad = [(zf_v[2 * pair + c][pl.ds(r + 8 * n, 8), :] - means[c]) * stats[2 * pair + c][1]
                    for r in (0, FM) for c in (0, 1)]
            for k, a in enumerate(_lhs7(*quad)):
                z2_v[k, pair, pl.ds(8 * n, 8), :] = a

    def prepare(i, c, after):
        def put(k, n, x):
            for j in range(x.shape[1] // 128):
                h_v[i % 2][k][j, pl.ds(16 * n + zero, 16), :] = _tile(x, j).astype(BF16)

        for n in range(H // 16):
            h = hidden(i * RB + c * H + 16 * n, (after(2 * n)[:8], after(2 * n + 1)[:8]))
            top, bot = _tile(h, 0, 2), _tile(h, 2, 2)
            put(7 + c, n, _tile(h, 4))
            if c:
                half[n] = top, bot
                put(2, n, top - bot)
                put(4, n, bot)
            else:
                put(1, n, top)
                put(3, n, bot - top)
                put(0, n, top + half[n][1])
                put(5, n, top + half[n][0])
                put(6, n, bot + half[n][1])

    def turn_out(after):
        for n in range((2 * KO + 1) * NCB):
            j, t = divmod(n, NCB)
            w = _words(wo_v, pl.ds(64 * j, 64), pl.ds(128 * t, 128))
            w = jnp.concatenate([tie(pltpu.bitcast(after(n)[:8], U32), w[:8]), w[8:]], axis=0)
            wr_v[j, pl.ds(128 * t + zero, 128), :] = pltpu.bitcast(w, BF16).T

    def split_out(after):
        for n in range(KO * DM // 16):
            j, r = divmod(16 * n, DM)
            quad = [wr_v[j + KO * c, pl.ds(r + DM * b, 16), :].astype(F32) for b in (0, 1) for c in (0, 1)]
            for k, a in enumerate(_lhs7(tie(after(n), quad[0]), quad[1], quad[2], tie(after(n), quad[3]))):
                wt_v[k, j, pl.ds(r, 16), :] = a.astype(BF16)

    def side_jobs(plan, at):
        for job in plan.split(","):
            if job:
                kind, (n, *spans) = job[0], (int(x) for x in job[1:].split(":"))
                total = {"s": FH // SU, "n": FM // 8, "h": H // 8, "m": N2 // 8,
                         "t": (2 * KO + 1) * NCB, "o": KO * DM // 16}[kind]
                slots = [p for lo, hi in zip(spans[::2], spans[1::2]) for p in range(lo, hi)]
                after = lambda k: at(slots[k * len(slots) // total])
                if kind == "s":
                    moments(n, after)
                elif kind == "m":
                    merge(n // NA, n % NA + zero, lambda k: after(k)[:8])
                elif kind in "to":
                    (turn_out if kind == "t" else split_out)(after)
                elif kind == "n":
                    norm_gate(n, after)
                else:
                    prepare(n // 2, n % 2, after)

    def rows_of(z):
        per = z.shape[0] // 16
        return lambda p: z[16 * (p % per):16 * (p % per) + 16, 128 * (p // per):128 * (p // per) + 128]

    def project(i):
        def prod(*pairs):
            right = [_ld(h_v[i % 2][k], j) for _, k in pairs for j in range(2 if k < 7 else 1)]
            return _nt(jnp.concatenate([x for k, _ in pairs for x in left[k]], axis=1),
                       jnp.concatenate(right, axis=1))

        s5, s3, r12, s4, s1 = prod((4, 4)), prod((2, 2)), prod((7, 8)), prod((3, 3)), prod((0, 0))
        s7, s2, r21, s6 = prod((6, 6), (7, 7)), prod((1, 1)), prod((8, 7)), prod((5, 5), (8, 8))
        gate = [((s4 - s5) + s1) + s7, (s5 + s3) + r12]
        value = [(s4 + s2) + r21, ((s3 + s1) - s2) + s6]
        for t in range(TB):
            keep_gate(i * TB + t, _gelu_scaled(_tile(gate[t // 2], t % 2)))
            z1_v[i * TB + t] = _tile(value[t // 2], t % 2)
        rounds = (s5, s3, gate[1], _tile(s4, 1), _tile(s1, 1), gate[0], s2, value[0], _tile(value[1], 1))
        return lambda p: rounds[p // (FH // 16)][16 * (p % (FH // 16)):16 * (p % (FH // 16)) + 16, 0:128]

    def first(f0, r0, n, k0, k1):
        h = jnp.concatenate([_ld(h0_v, j, pl.ds(r0 // 2, n // 2)) for j in range(k0, k1)], axis=1)
        return _nt(wi_v[pl.ds(f0, FH), pl.ds(128 * k0, 128 * (k1 - k0))], h)

    def keep_first(r, h):
        for j in range(NCB):
            h0_v[j, pl.ds(r, 16), :] = _tile(h, j).astype(BF16)

    stats, half = {}, {}
    for r in range(0, H, 16):
        keep_first(r, hidden(r))
    wait("gate")
    zero = pl.multiple_of(zero_s[0], 16)
    head = first(0, 0, H, 0, 2)
    z = _gelu_scaled(head + first(0, 0, H, 2, NCB))
    at = rows_of(jnp.concatenate([_tile(head, 0), z], axis=1))
    for n in range(H // 16):
        keep_first(H + 16 * n, hidden(H + 16 * n, [at(E0 + (2 * n + k) * ES // 8)[:8] for k in (0, 1)]))
    z = jnp.concatenate([z] + [_gelu_scaled(first(0, r, 128, 0, NCB)) for r in (H, H + 128)], axis=1)
    for t in range(TB):
        keep_gate(t, _tile(z, t))
    side_jobs(NJ[0], rows_of(z))
    wait("value")
    head = first(FH, 0, RB, NCB - 1, NCB)
    z = head + first(FH, 0, RB, 0, NCB - 1)
    for t in range(TB):
        z1_v[t] = _tile(z, t)
    side_jobs(NJ[1], rows_of(jnp.concatenate([_tile(head, 0), z], axis=1)))
    sums = [_lhs7(*(wi_v[pl.ds(FH * r, FH), pl.ds(256 * c + 128 * j, 128)].astype(F32)
                    for r in (0, 1) for c in (0, 1))) for j in (0, 1)]
    left = ([[s[k].astype(BF16) for s in sums] for k in range(7)]
            + [[wi_v[pl.ds(FH * r, FH), pl.ds(512, 128)]] for r in (0, 1)])
    for i in range(1, NB):
        if i == 2:
            wait("out")
        side_jobs(NJ[i + 1], project(i))
    gb = _nn(sc, wm_v[:, pl.ds(5 * D, D)]) * (0.5 / _GA)
    bf_v[...] = b_v[...].astype(F32)

    wait("mix")

    def mix(i):
        def w(c, r):
            return [_ld(ws_v, 2 * j + c, _ds((i * RB + r * H) // 2, H // 2, H // 2))
                    for j in range(S // 256)]

        def comb(x, y, sign):
            return [(jnp.add if sign > 0 else jnp.subtract)(a.astype(F32), b.astype(F32)) for a, b in zip(x, y)]

        def prod(n, rhs):
            def left(k):
                def part(r, c, rows):
                    return jnp.concatenate([z2_v[n, 2 * j + c, pl.ds(FT * r, rows), :] for j in range(NB)], axis=1)

                def both(c, op):
                    top = part(0, c, FT)
                    return jnp.concatenate([op(top[:FB], part(1, 1, FB)), top[FB:]], axis=0)

                return (lambda: both(0, jnp.add), lambda: part(1, 0, FB) + part(1, 1, FB),
                        lambda: part(0, 0, FT), lambda: part(1, 1, FB),
                        lambda: part(0, 0, FT) + part(0, 1, FT), lambda: part(1, 0, FB) - part(0, 0, FB),
                        lambda: both(1, jnp.subtract))[k]().astype(BF16)

            b11, b12, b21, b22 = (
                jnp.concatenate([rhs[2 * j + c][128 * r:128 * r + 128] for j in range(NB)], axis=1)
                for c in (0, 1) for r in (0, 1))
            m = lambda k, x: _nt(left(k), x.astype(BF16))
            m2, m5 = m(1, b11), m(4, b22)
            b11, b12, b21, b22 = (x.astype(F32) for x in (b11, b12, b21, b22))
            m4 = m(3, b21 - b11)
            m1, m7, m3, m6 = m(0, b11 + b22), m(6, b21 + b22), m(2, b12 - b22), m(5, b11 + b12)
            c11 = jnp.concatenate([m4 - m5[:FB], -m5[FB:]], axis=0) + m1 + m7
            c22 = (m1[:FB] - m2) + m3[:FB] + m6
            return jnp.concatenate([jnp.concatenate([c11, m5 + m3], axis=1),
                                    jnp.concatenate([m2 + m4, c22], axis=1)], axis=0)

        def gate(r, c, g):
            tiles = [i * TB + c * (H // 128) + t for t in range(H // 128)]
            bias = jnp.concatenate([bf_v[pl.ds(j, 1), :] for j in tiles], axis=1)
            z1 = jnp.concatenate([z1_v[j, pl.ds(FM * r, FM), :] for j in tiles], axis=1)
            return _gelu_scaled(z1) * (g + bias)

        s2 = prod(1, w(0, 0))
        s5 = prod(4, w(1, 1))
        s4 = prod(3, comb(w(1, 0), w(0, 0), -1))
        p21 = gate(1, 0, s2 + s4)
        d11 = s4 - s5
        s1 = prod(0, comb(w(0, 0), w(1, 1), 1))
        d11, d22 = d11 + s1, s1 - s2
        p11 = gate(0, 0, d11 + prod(6, comb(w(1, 0), w(1, 1), 1)))
        s3 = prod(2, comb(w(0, 1), w(1, 1), -1))
        p12 = gate(0, 1, s3 + s5)
        p22 = gate(1, 1, (d22 + s3) + prod(5, comb(w(0, 0), w(0, 1), 1)))
        return [jnp.concatenate(p, axis=0) for p in ((p11, p21), (p12, p22))]

    def flush(k):
        rows = _ds(k * H, H, H)
        return [pltpu.make_async_copy(o_v.at[j, rows], o_h.at[rows, pl.ds(128 * j, 128)], sems.at[2])
                for j in range(NCB)]

    def finish(r0, tile):
        for t in range(H // 128):
            for j in range(NCB):
                at = _ds(r0 + 128 * t, 128, 128), pl.ds(128 * j, 128)
                o_v[j, at[0], :] = (x1_v[at] + jnp.concatenate([_tile(gb, j)] * 8, axis=0)
                           * tile(t, j).T.astype(F32)).astype(BF16)

    def mix_step(i):
        p = mix(i)
        b11, b12, b21, b22 = (p[c][128 * KO * r:128 * KO * (r + 1)] for r in (0, 1) for c in (0, 1))

        def prod(n, rhs):
            return _nn(jnp.concatenate([_ld(wt_v, n, j) for j in range(KO)], axis=1), rhs.astype(BF16))

        def rest(c):
            tail = jnp.concatenate([p[c][256 * KO:], jnp.zeros((128 + 256 * KO - FH, H), F32)], axis=0)
            return _nn(_ld(wr_v, 2 * KO), tail.astype(BF16))

        r0 = rest(0)
        s2 = prod(1, b11)
        s4 = prod(3, b21 - b11)
        s5 = prod(4, b22)
        s1 = prod(0, b11 + b22)
        s7 = prod(6, b21 + b22)
        ot = jnp.concatenate([r0[:DM] + s4 - s5 + s1 + s7, r0[DM:] + s2 + s4], axis=0)
        finish(i * RB, lambda t, j: _tile(ot, t)[128 * j:128 * j + 128].astype(BF16))
        for cp in flush(2 * i):
            cp.start()
        spot = 0, _ds(i * RB + H, 16, 16)
        o_v[spot] = jnp.zeros((16, 128), BF16)
        pin = o_v[0, _ds(i * RB + H + zero, 16, 16)].astype(F32)
        r1 = rest(1)
        s3 = prod(2, b12 - b22)
        b = b11 + b12
        b = jnp.concatenate([b[:-16], jnp.concatenate([b[-16:, :128], tie(pin, b[-16:, 128:])], axis=1)], axis=0)
        s6 = prod(5, b)
        ot = jnp.concatenate([r1[:DM] + s5 + s3, (s1 - s2) + r1[DM:] + s3 + s6], axis=0)
        finish(i * RB + H, lambda t, j: _tile(ot, t)[128 * j:128 * j + 128].astype(BF16))
        for cp in flush(2 * i + 1):
            cp.start()

    zero = pl.multiple_of(zero_s[0], 16)
    zero = zero_s[0]
    pl.loop(0, NB)(mix_step)
    for k in range(S // H):
        for cp in flush(k):
            cp.wait()


@jax.jit
def pallas_adaLN_cond__ssm_conv_h3__mixer_gmlp__prompt_kernel(
    A_q, A_k, A_v, A_shift_k, A_ssm_k, A_ssm_D, B_x, B_w_in, B_w_sp, B_b_sp, B_w_out, c, w_mod,
):
    del B_x
    vm = pltpu.VMEM
    tile = (128, 128)
    scratch = [
        vm((S, D), BF16), vm((NCB, PAD + S, 128), BF16), vm((NCB, S, 128), BF16), vm((TAPS, D), BF16),
        vm((NCB, NA, 128, CH), BF16), vm((NCB, 128), BF16), vm((2 * FH, D), BF16),
        vm((S // 128, S, 128), BF16), vm((S // 128, 128), BF16), vm((256 * KO + 128, D), BF16), vm((1, D), BF16),
        vm((D, 6 * D), BF16), vm((16, *tile), BF16),
        vm((8, 2 * NA, *tile), BF16), vm((8, 2 * NA, *tile), BF16),
        vm((2 * NA, *tile), F32), vm((2 * NA, *tile), F32), vm((NA, *tile), BF16), vm((NA, *tile), BF16),
        vm((16, NA, *tile), F32), vm((16, NA, *tile), F32), vm((5, NA, *tile), F32), vm((5, NA, *tile), F32),
        vm((NCB, S, 128), F32), vm((S, D), F32), vm((NCB, RB, 128), BF16),
        vm((S // 128, FH, 128), F32), vm((7, S // 256, FM, 128), F32),
        vm((7, KO, DM, 128), BF16), vm((2 * KO + 1, D, 128), BF16), vm((S // 128, 128), F32),
        vm((NCB, S, 128), BF16), vm((8, 128), jnp.int32), pltpu.SMEM((1,), jnp.int32),
        pltpu.SemaphoreType.DMA((13,)),
    ] + [vm((FH, 128), F32)] * 16 + [vm((FH // SU * 16, 128), F32)] * 16 + ([vm((2, H, 128), BF16)] * 7 + [vm((1, H, 128), BF16)] * 2) * 2
    out = pl.pallas_call(
        _kernel,
        out_shape=jax.ShapeDtypeStruct((S, D), BF16),
        in_specs=[pl.BlockSpec(memory_space=pltpu.HBM)] * 12,
        out_specs=pl.BlockSpec(memory_space=pltpu.HBM),
        scratch_shapes=scratch,
        compiler_params=pltpu.CompilerParams(vmem_limit_bytes=110 * 1024 * 1024),
    )(A_q.reshape(S, D), A_k.reshape(S, D), A_v.reshape(S, D), A_shift_k.T, A_ssm_k,
      A_ssm_D.reshape(NCB, 128), B_w_in.T, B_w_sp, B_b_sp.reshape(S // 128, 128), B_w_out, c, w_mod)
    return out.reshape(1, S, D)
```

```python
import functools
import math

import numpy as np
import jax
import jax.numpy as jnp
from jax import lax
import jax.experimental.pallas as pl
import jax.experimental.pallas.tpu as pltpu

S, D, FH = 2048, 640, 864
FM, DM = FH // 2, D // 2
KO = FH // 256
FT, FB = 224, 208
TAPS = 4
CH = 512
NA = S // CH
N2 = 64
N1 = CH // N2
NCB = D // 128
RB = 512
NB = S // RB
H = RB // 2
EPS = 1e-5
F32, BF16, U32 = jnp.float32, jnp.bfloat16, jnp.uint32
PAD = 16

_C8 = math.cos(math.pi / 8)
_T8 = math.tan(math.pi / 8)
_R2 = math.sqrt(0.5)
_G0 = math.sqrt(2 / math.pi)
_GA = (_G0 * 0.044715) ** (1 / 3)

E0, ES = 0, 16
TU = (-1, 0, 3, 5, 16, 32, 35, 38)
TK = (34, 38, 41, 42, 43, 44, 45, 46)
TI = (-1, -1, -1, 0, 0, 2, 3, 4, 5, 5, 7, 16, 17, 17, 32, 33, 34, 36, 37, 38, 38, 39, 40, 42)
SU = 24
NJ = [
    "s0:70:89,s1:118:190,s2:168:205,m14:100:120,m18:120:150,m15:150:180,m19:180:210,m13:54:80,m17:70:100",
    "h3:0:96,h2:118:219,s3:20:80",
    "h5:0:108:142:196,h4:182:246:314:430,s4:330:418,s6:222:276",
    "h7:22:114:162:216,h6:226:280:330:446,s5:0:70,s7:44:98,s8:324:372,s10:240:270,n0:370:486",
    "s9:0:40,s11:40:80,n1:0:56,n2:56:112,n3:112:168,n4:168:224,n5:218:280,s14:160:206,s15:220:270,n7:280:344,s12:330:378,s13:380:410,n6:414:474,t0:10:330,o0:370:470",
]


def _dft_mats():
    def turn(k):
        return [jnp.cos(((k - s) & 1023).astype(F32) * (2 * math.pi / 1024)) for s in (0, 256)]

    def times(x, y, i):
        return [x[0] * y[0][i:i + 1] - x[1] * y[1][i:i + 1], x[0] * y[1][i:i + 1] + x[1] * y[0][i:i + 1]]

    row, col = (lax.broadcasted_iota(jnp.int32, (8, 128), d) for d in (0, 1))
    n, imag = (col >> 5) * 16 + (col & 7) * 2 + ((col >> 4) & 1), (col >> 3) & 1
    root = jnp.where(row < 4, 1 + 4 * row, jnp.where(row < 6, 8 * row - 30, 4))
    root = [t * jnp.where(row < 4, _C8 / 8, 1 / 8) for t in turn(root * n + 256 * imag)]
    fine, coarse = turn(16 * row * n), turn(128 * row * n)
    rows = [[t for g in range(8) for t in times(base, coarse, g)]
            for base in (times(fine, root, b) for b in range(7))]
    n = n + 64 * imag
    fine, coarse = [t * (1 / 8) for t in turn(8 * row * n)], turn(64 * row * n)
    last = [t for g in range(8) for t in times(fine, coarse, g)]
    last[1] = jnp.where(row == 0, (1 - 2 * (n & 1)).astype(F32) * (1 / 8), last[1])
    return [jnp.concatenate(r, axis=0).astype(BF16) for r in rows + [last]]


def _outer_fwd(u):
    t0r, t0i = u[0] * (1 / _C8), u[4] * (1 / _C8)
    t2r, t2i = (u[2] - u[6]) * (_R2 / _C8), (u[2] + u[6]) * (_R2 / _C8)
    t1r, t1i = u[1] - _T8 * u[5], u[5] + _T8 * u[1]
    t3r, t3i = _T8 * u[3] - u[7], _T8 * u[7] + u[3]
    ar, ai, br, bi = t0r + t2r, t0i + t2i, t0r - t2r, t0i - t2i
    cr, ci, dr, di = t1r + t3r, t1i + t3i, t1r - t3r, t1i - t3i
    out = [(ar + cr, ai + ci), (br - di, bi + dr), (ar - cr, ai - ci), (br + di, bi - dr)]
    p = [u[j] + u[j + 4] for j in range(4)]
    q = [u[j] - u[j + 4] for j in range(4)]
    er, ei = (q[1] - q[3]) * _R2, (q[1] + q[3]) * _R2
    out += [(q[0] + er, q[2] + ei), (q[0] - er, q[2] - ei)]
    out += [(p[0] - p[2], p[1] - p[3]), (p[0] + p[2], p[1] + p[3])]
    return out


def _outer_inv(B):
    ar, ai = B[0][0] + B[2][0], B[0][1] + B[2][1]
    cr, ci = B[0][0] - B[2][0], B[0][1] - B[2][1]
    br, bi = B[1][0] + B[3][0], B[1][1] + B[3][1]
    dr, di = B[1][0] - B[3][0], B[1][1] - B[3][1]
    g0r, g0i, g2r, g2i = ar + br, ai + bi, ar - br, ai - bi
    g1r, g1i, g3r, g3i = cr + di, ci - dr, cr - di, ci + dr
    nr = [g0r * (1 / _C8), g1r + _T8 * g1i, (g2r + g2i) * (_R2 / _C8), _T8 * g3r + g3i]
    ni = [g0i * (1 / _C8), g1i - _T8 * g1r, (g2i - g2r) * (_R2 / _C8), _T8 * g3i - g3r]
    fr, fi = B[4][0] - B[5][0], B[4][1] - B[5][1]
    q = [B[4][0] + B[5][0], (fr + fi) * _R2, B[4][1] + B[5][1], (fi - fr) * _R2]
    p = [B[7][0] + B[6][0], B[7][1] + B[6][1], B[7][0] - B[6][0], B[7][1] - B[6][1]]
    return ([p[j] + q[j] + nr[j] for j in range(4)]
            + [p[j] - q[j] + ni[j] for j in range(4)])


def _gelu_scaled(x):
    t = jnp.tanh(x * (_G0 / _GA + x * x))
    return x + x * t


def _norm_stats(s1, s2, n, eps):
    m = s1 * (1.0 / n)
    return m, jnp.exp(-0.5 * jnp.log(jnp.maximum(s2 * (1.0 / n) - m * m, 0.0) + eps))


def _ln_rows(x):
    m, r = _norm_stats(jnp.sum(x, axis=-1, keepdims=True), jnp.sum(x * x, axis=-1, keepdims=True),
                       x.shape[-1], EPS)
    return (x - m) * r


def _lhs7(a11, a12, a21, a22):
    return a11 + a22, a21 + a22, a11, a22, a11 + a12, a21 - a11, a12 - a22


def _words(ref, *idx):
    return ref.bitcast(U32)[idx]


def _ld(ref, *idx):
    return pltpu.bitcast(_words(ref, *idx), BF16)


def _phase(words, odd):
    return pltpu.bitcast(words & np.uint32(0xFFFF0000) if odd else words << 16, F32)


def _nn(a, b):
    return jnp.dot(a, b, preferred_element_type=F32)


def _nt(a, b):
    return lax.dot_general(a, b, (((1,), (1,)), ((), ())), preferred_element_type=F32)


def _ds(start, size, align):
    return pl.ds(start if isinstance(start, int) else pl.multiple_of(start, align), size)


def _tile(x, j, n=1):
    return x[:, 128 * j:128 * (j + n)]


def _add(xs):
    return functools.reduce(lambda x, y: x + y, xs)


def _kernel(q_h, k_h, v_h, sh_h, sk_h, sd_h, wi_h, ws_h, b_h, wo_h, c_h, wm_h, o_h,
            q_v, k_v, v_v, sh_v, sk_v, sd_v, wi_v, ws_v, b_v, wo_v, c_v, wm_v, vf_v,
            au0_v, au1_v, fa_v, fb_v, ya_v, yb_v, bm0_v, bp0_v, bm1_v, bp1_v,
            y_v, x1_v, h0_v, z1_v, z2_v, wt_v, wr_v, bf_v, o_v, tie_v, zero_s,
            sems, *lists):
    au_v, zf_v, sum_v, h_v = (au0_v, au1_v), lists[:16], lists[16:32], (lists[32:41], lists[41:])
    copies = {}

    def start(group, sem, *pairs):
        copies[group] = [pltpu.make_async_copy(src, dst, sems.at[sem]) for src, dst in pairs]
        for cp in copies[group]:
            cp.start()

    def wait(*groups):
        for group in groups:
            for cp in copies[group]:
                cp.wait()

    def conv_inputs(cb, a):
        rows, lanes, sem = _ds(a * CH, CH, CH), pl.ds(cb * 128, 128), sems.at[cb % 3 * NA + a]
        return (pltpu.make_async_copy(k_h.at[rows, lanes], k_v.at[cb, _ds(PAD + a * CH, CH, PAD)], sem),
                pltpu.make_async_copy(v_h.at[rows, lanes], v_v.at[cb, rows], sem),
                pltpu.make_async_copy(sk_h.at[lanes, rows], sk_v.at[cb, a], sem))

    def fetch(stage):
        rows = lambda r, n: (q_h.at[pl.ds(r, n)], q_v.at[pl.ds(r, n)])
        if stage == 0:
            start("taps", 12, (sh_h, sh_v), (sd_h, sd_v))
        if stage < 3:
            for a in range(NA):
                for cp in conv_inputs(stage, a):
                    cp.start()
        if stage == 4:
            later = []
            for a in range(NA):
                (k3, v3, f3), (k4, v4, f4) = conv_inputs(3, a), conv_inputs(4, a)
                later.append(f4)
                for cp in (k3, k4, v3, v4, f3):
                    cp.start()
            for cp in later:
                cp.start()
        if stage == NCB:
            start("mod", 8, (c_h, c_v), (wm_h.at[:, pl.ds(0, 5 * D)], wm_v.at[:, pl.ds(0, 5 * D)]), rows(0, H))
            start("gate", 9, (wi_h.at[pl.ds(FH, FH)], wi_v.at[pl.ds(0, FH)]), rows(H, H))
            start("value", 10, (wi_h.at[pl.ds(0, FH)], wi_v.at[pl.ds(FH, FH)]), rows(RB, 2 * RB))
        if stage == NCB + 2:
            start("out", 0, rows(3 * RB, RB), (wm_h.at[:, pl.ds(5 * D, D)], wm_v.at[:, pl.ds(5 * D, D)]),
                  (b_h, b_v), (wo_h, wo_v.at[pl.ds(0, FH)]))
            start("mix", 1, *[(ws_h.at[:, pl.ds(128 * j, 128)], ws_v.at[j]) for j in range(S // 128)])

    fetch(0)
    fetch(1)
    for ref in (fb_v, ya_v, tie_v):
        ref[...] = jnp.zeros(ref.shape, ref.dtype)
    k_v[:, pl.ds(0, PAD), :] = jnp.zeros((NCB, PAD, 128), BF16)
    wo_v[pl.ds(FH, 256 * KO + 128 - FH), :] = jnp.zeros((256 * KO + 128 - FH, D), BF16)
    row, col = (lax.broadcasted_iota(jnp.int32, (128, 128), d) for d in (0, 1))
    n = (col >> 5) * 16 + (col & 7) * 2 + ((col >> 4) & 1)
    order = jnp.where(row == (n >> 3) * 16 + (col & 8) + (n & 7), 1.0, 0.0).astype(BF16)
    mats = _dft_mats()
    back = _nt(order, jnp.concatenate(mats, axis=0))
    for b in range(8):
        vf_v[b] = mats[b]
        vf_v[8 + b] = _tile(back, b).astype(BF16)
    zero_s[0] = 0
    row8 = lax.broadcasted_iota(jnp.int32, (8, 128), 0)

    def tie(after, x):
        if after is None:
            return x
        never = jnp.concatenate([tie_v[...]] * (x.shape[0] // 8), axis=0) != 0
        return jnp.where(never, after, x)

    def put(cb, slot, g, res):
        for b in range(8):
            au_v[cb % 2][b, slot, pl.ds(16 * g, 16), :] = jnp.concatenate(res[b], axis=0).astype(BF16)

    def split_filter(cb, a, after):
        kt = pltpu.bitcast(sk_v[cb, a].T, U32)
        for g in range(N2 // 8):
            u = [_phase(kt[j * N2 // 2 + g // 2 * 8:j * N2 // 2 + g // 2 * 8 + 8], g % 2) for j in range(N1)]
            if g == 0:
                u[0] = u[0] + jnp.where(row8 + a == 0, sd_v[...].astype(F32)[cb:cb + 1], 0.0)
            u[:4] = [tie(after(g), x) for x in u[:4]]
            put(cb, NA + a, g, _outer_fwd(u))

    def split_signal(cb, a, after):
        taps = [jnp.broadcast_to(sh_v[j:j + 1, pl.ds(cb * 128, 128)].astype(F32), (8, 128))
                for j in range(TAPS)]
        base = a * (CH // 2) if isinstance(a, int) else pl.multiple_of(a * (CH // 2), CH // 2)
        for g in range(N2 // 8):
            w = [tie(after(g), t) for t in taps]
            u = []
            for j in range(N1):
                r = base + j * N2 // 2 + g // 2 * 8
                lag = [_phase(_words(k_v, cb, pl.ds(r + PAD // 2 + (g % 2 - t) // 2, 8)), (g % 2 - t) % 2)
                       for t in range(TAPS)]
                u.append(_add([x * wt for x, wt in zip(lag, w)]) * _phase(_words(v_v, cb, pl.ds(r, 8)), g % 2))
            put(cb, a, g, _outer_fwd(u))

    def spectra(cb, b, half, f_ref):
        rhs = jnp.concatenate([_ld(au_v[cb % 2], b, half * NA + a) for a in range(NA)], axis=1)
        f = _nn(_ld(vf_v, b), rhs)
        for a in range(NA):
            f_ref[half * NA + a] = f[:, 128 * a:128 * a + 128]
        return f

    def product(f_ref, y_ref, plus, real_rows=None):
        for g in range(8):
            ur, ui, kr, ki = ([f_ref[o + a, pl.ds(16 * g + 8 * c, 8), :] for a in range(NA)]
                              for o in (0, NA) for c in (0, 1))
            kr, ki = ([k[0]] + [k[a] + k[a - 1] if plus else k[a] - k[a - 1] for a in range(1, NA)]
                      for k in (kr, ki))
            for a in range(NA):
                yi = _add([kr[j] * ui[a - j] + ki[j] * ur[a - j] for j in range(a + 1)])
                if real_rows is not None and g == 0:
                    rr = _add([kr[j] * ur[a - j] for j in range(a + 1)])
                    ii = _add([ki[j] * ui[a - j] for j in range(a + 1)])
                    yr = jnp.where(real_rows, 0.5 * rr, rr - ii)
                    yi = jnp.where(real_rows, 0.5 * ii, yi)
                else:
                    yr = _add([kr[j] * ur[a - j] - ki[j] * ui[a - j] for j in range(a + 1)])
                y_ref[a, pl.ds(16 * g, 16), :] = jnp.concatenate([yr, yi], axis=0).astype(BF16)

    def residues(y_ref, b, dst):
        r = _nn(_ld(vf_v, 8 + b), jnp.concatenate([_ld(y_ref, a) for a in range(NA)], axis=1))
        for a in range(NA):
            dst[a] = r[:, 128 * a:128 * a + 128]
        return r

    def stash(t):
        return ((bm0_v.at[t], bp0_v.at[t]) if t < 16 else (bm1_v.at[t - 16], bp1_v.at[t - 16]))

    def merge(cb, a, after=lambda g: None):
        src = [stash(1 + 4 * cb + b)[s] for s in (0, 1) for b in range(4)]
        for g in range(N2 // 8):
            res = [[ref[a, pl.ds(16 * g + 8 * c, 8), :] for c in (0, 1)] for ref in src]
            res[0] = [tie(after(g), x) for x in res[0]]
            res[1] = [tie(after(g), x) for x in res[1]]
            for j, y in enumerate(_outer_inv(res)):
                y_v[cb, _ds(a * CH + j * N2 + 8 * g, 8, 8), :] = y

    def transform(cb, a, dst, active=True):
        pa = (a + 3) % 4
        res = []
        if active:
            res += [spectra(cb, a, 1, fa_v), spectra(cb, a, 0, fa_v)]
        product(fb_v, yb_v, True, row8 + (3 - pa) == 0)
        res.append(residues(ya_v, pa, dst[0]))
        if active:
            res += [spectra(cb, 4 + a, 1, fb_v), spectra(cb, 4 + a, 0, fb_v)]
            product(fa_v, ya_v, False)
        res.append(residues(yb_v, 4 + pa, dst[1]))
        return res

    def conv_step(cb, a):
        if cb < NCB:
            for cp in conv_inputs(cb, a):
                cp.wait()
        if cb:
            done = transform(cb - 1, a, (bm0_v.at[4 * cb - 4 + a], bp0_v.at[4 * cb - 4 + a])
                             if cb < NCB else (bm1_v.at[a], bp1_v.at[a]))
        at = lambda p: done[p // 8][16 * (p % 8):16 * (p % 8) + 8, 0:128] if cb and p >= 0 else None
        if cb < NCB:
            split_signal(cb, a, lambda g: at(TU[g]))
            split_filter(cb, a, lambda g: at(TK[g]))
        else:
            for c in range(3):
                merge(c, a, lambda g: at(TI[8 * c + g]))

    wait("taps")
    for cb in range(NCB + 1):
        fetch(cb + 2)
        pl.loop(0, NA)(functools.partial(conv_step, cb))

    wait("mod")
    transform(NCB, 0, stash(20), active=False)
    cc = c_v[...].astype(F32)
    sc = jnp.broadcast_to(cc / (1.0 + jnp.exp(-cc)), (16, D)).astype(BF16)
    mod = _nn(sc, jnp.concatenate([wm_v[:, pl.ds(i * D, D)] for i in (0, 1, 2, 4, 3)], axis=1))[0:8]
    sa, ca, ga, cb_, sb = (mod[:, i * D:(i + 1) * D] for i in range(5))
    m1, m0 = ga * (1.0 + ca), ga * sa
    n1, n0 = _GA * (1.0 + cb_), _GA * sb
    zero = zero_s[0]
    for n, cb in enumerate((3, 4)):
        merge(cb, zero, lambda g: _tile(mod, (8 * n + g) * 3 // 4))

    TB = RB // 128

    def hidden(r0, after=(None, None)):
        out = []
        for r, a in zip((r0, r0 + 8), after):
            rows = pl.ds(r, 8)
            x = q_v[rows, :].astype(F32)
            x = jnp.concatenate([tie(a, x[:, :128]), x[:, 128:]], axis=1)
            x1 = x + (_ln_rows(x) * m1 + m0) * jnp.concatenate([y_v[j, rows, :] for j in range(NCB)], axis=1)
            x1_v[rows, :] = x1
            out.append(_ln_rows(x1) * n1 + n0)
        return jnp.concatenate(out, axis=0)

    def keep_gate(tile, z):
        zf_v[tile][pl.ds(zero, FH), :] = z

    def moments(tile, after):
        z, acc = zf_v[tile], sum_v[tile]
        s1 = s2 = None
        for n, f in enumerate(range(0, FH, SU)):
            for r in range(f, f + SU, 8):
                d = tie(after(n)[:8] if r == f else None, z[pl.ds(r, 8), :])
                s1, s2 = (d, d * d) if s1 is None else (s1 + d, s2 + d * d)
            acc[pl.ds(16 * n + zero, 16), :] = jnp.concatenate([s1, s2], axis=0)
        s1, s2 = (jnp.sum(acc[pl.ds(16 * n + r, 8), :], axis=0, keepdims=True) for r in (0, 8))
        stats[tile] = [jnp.broadcast_to(t, (8, 128)) for t in _norm_stats(s1, s2, FH, EPS * (2 * _GA) ** 2)]

    def norm_gate(pair, after):
        for n in range(FM // 8):
            means = [tie(after(n)[:8], stats[2 * pair + c][0]) for c in (0, 1)]
            quad = [(zf_v[2 * pair + c][pl.ds(r + 8 * n, 8), :] - means[c]) * stats[2 * pair + c][1]
                    for r in (0, FM) for c in (0, 1)]
            for k, a in enumerate(_lhs7(*quad)):
                z2_v[k, pair, pl.ds(8 * n, 8), :] = a

    def prepare(i, c, after):
        def put(k, n, x):
            for j in range(x.shape[1] // 128):
                h_v[i % 2][k][j, pl.ds(16 * n + zero, 16), :] = _tile(x, j).astype(BF16)

        for n in range(H // 16):
            h = hidden(i * RB + c * H + 16 * n, (after(2 * n)[:8], after(2 * n + 1)[:8]))
            top, bot = _tile(h, 0, 2), _tile(h, 2, 2)
            put(7 + c, n, _tile(h, 4))
            if c:
                half[n] = top, bot
                put(2, n, top - bot)
                put(4, n, bot)
            else:
                put(1, n, top)
                put(3, n, bot - top)
                put(0, n, top + half[n][1])
                put(5, n, top + half[n][0])
                put(6, n, bot + half[n][1])

    def turn_out(after):
        for n in range((2 * KO + 1) * NCB):
            j, t = divmod(n, NCB)
            w = _words(wo_v, pl.ds(64 * j, 64), pl.ds(128 * t, 128))
            w = jnp.concatenate([tie(pltpu.bitcast(after(n)[:8], U32), w[:8]), w[8:]], axis=0)
            wr_v[j, pl.ds(128 * t + zero, 128), :] = pltpu.bitcast(w, BF16).T

    def split_out(after):
        for n in range(KO * DM // 16):
            j, r = divmod(16 * n, DM)
            quad = [wr_v[j + KO * c, pl.ds(r + DM * b, 16), :].astype(F32) for b in (0, 1) for c in (0, 1)]
            for k, a in enumerate(_lhs7(tie(after(n), quad[0]), quad[1], quad[2], tie(after(n), quad[3]))):
                wt_v[k, j, pl.ds(r, 16), :] = a.astype(BF16)

    def side_jobs(plan, at):
        for job in plan.split(","):
            if job:
                kind, (n, *spans) = job[0], (int(x) for x in job[1:].split(":"))
                total = {"s": FH // SU, "n": FM // 8, "h": H // 8, "m": N2 // 8,
                         "t": (2 * KO + 1) * NCB, "o": KO * DM // 16}[kind]
                slots = [p for lo, hi in zip(spans[::2], spans[1::2]) for p in range(lo, hi)]
                after = lambda k: at(slots[k * len(slots) // total])
                if kind == "s":
                    moments(n, after)
                elif kind == "m":
                    merge(n // NA, n % NA + zero, lambda k: after(k)[:8])
                elif kind in "to":
                    (turn_out if kind == "t" else split_out)(after)
                elif kind == "n":
                    norm_gate(n, after)
                else:
                    prepare(n // 2, n % 2, after)

    def rows_of(z):
        per = z.shape[0] // 16
        return lambda p: z[16 * (p % per):16 * (p % per) + 16, 128 * (p // per):128 * (p // per) + 128]

    def project(i):
        def prod(*pairs):
            right = [_ld(h_v[i % 2][k], j) for _, k in pairs for j in range(2 if k < 7 else 1)]
            return _nt(jnp.concatenate([x for k, _ in pairs for x in left[k]], axis=1),
                       jnp.concatenate(right, axis=1))

        s5, s3, r12, s4, s1 = prod((4, 4)), prod((2, 2)), prod((7, 8)), prod((3, 3)), prod((0, 0))
        s7, s2, r21, s6 = prod((6, 6), (7, 7)), prod((1, 1)), prod((8, 7)), prod((5, 5), (8, 8))
        gate = [((s4 - s5) + s1) + s7, (s5 + s3) + r12]
        value = [(s4 + s2) + r21, ((s3 + s1) - s2) + s6]
        for t in range(TB):
            keep_gate(i * TB + t, _gelu_scaled(_tile(gate[t // 2], t % 2)))
            z1_v[i * TB + t] = _tile(value[t // 2], t % 2)
        rounds = (s5, s3, gate[1], _tile(s4, 1), _tile(s1, 1), gate[0], s2, value[0], _tile(value[1], 1))
        return lambda p: rounds[p // (FH // 16)][16 * (p % (FH // 16)):16 * (p % (FH // 16)) + 16, 0:128]

    def first(f0, r0, n, k0, k1):
        h = jnp.concatenate([_ld(h0_v, j, pl.ds(r0 // 2, n // 2)) for j in range(k0, k1)], axis=1)
        return _nt(wi_v[pl.ds(f0, FH), pl.ds(128 * k0, 128 * (k1 - k0))], h)

    def keep_first(r, h):
        for j in range(NCB):
            h0_v[j, pl.ds(r, 16), :] = _tile(h, j).astype(BF16)

    stats, half = {}, {}
    for r in range(0, H, 16):
        keep_first(r, hidden(r))
    wait("gate")
    zero = pl.multiple_of(zero_s[0], 16)
    head = first(0, 0, H, 0, 2)
    z = _gelu_scaled(head + first(0, 0, H, 2, NCB))
    at = rows_of(jnp.concatenate([_tile(head, 0), z], axis=1))
    for n in range(H // 16):
        keep_first(H + 16 * n, hidden(H + 16 * n, [at(E0 + (2 * n + k) * ES // 8)[:8] for k in (0, 1)]))
    z = jnp.concatenate([z] + [_gelu_scaled(first(0, r, 128, 0, NCB)) for r in (H, H + 128)], axis=1)
    for t in range(TB):
        keep_gate(t, _tile(z, t))
    side_jobs(NJ[0], rows_of(z))
    wait("value")
    head = first(FH, 0, RB, NCB - 1, NCB)
    z = head + first(FH, 0, RB, 0, NCB - 1)
    for t in range(TB):
        z1_v[t] = _tile(z, t)
    side_jobs(NJ[1], rows_of(jnp.concatenate([_tile(head, 0), z], axis=1)))
    sums = [_lhs7(*(wi_v[pl.ds(FH * r, FH), pl.ds(256 * c + 128 * j, 128)].astype(F32)
                    for r in (0, 1) for c in (0, 1))) for j in (0, 1)]
    left = ([[s[k].astype(BF16) for s in sums] for k in range(7)]
            + [[wi_v[pl.ds(FH * r, FH), pl.ds(512, 128)]] for r in (0, 1)])
    for i in range(1, NB):
        if i == 2:
            wait("out")
        side_jobs(NJ[i + 1], project(i))
    gb = _nn(sc, wm_v[:, pl.ds(5 * D, D)]) * (0.5 / _GA)
    bf_v[...] = b_v[...].astype(F32)

    wait("mix")

    def mix(i):
        def w(c, r):
            return [_ld(ws_v, 2 * j + c, _ds((i * RB + r * H) // 2, H // 2, H // 2))
                    for j in range(S // 256)]

        def comb(x, y, sign):
            return [(jnp.add if sign > 0 else jnp.subtract)(a.astype(F32), b.astype(F32)) for a, b in zip(x, y)]

        def prod(n, rhs):
            def left(k):
                def part(r, c, rows):
                    return jnp.concatenate([z2_v[n, 2 * j + c, pl.ds(FT * r, rows), :] for j in range(NB)], axis=1)

                def both(c, op):
                    top = part(0, c, FT)
                    return jnp.concatenate([op(top[:FB], part(1, 1, FB)), top[FB:]], axis=0)

                return (lambda: both(0, jnp.add), lambda: part(1, 0, FB) + part(1, 1, FB),
                        lambda: part(0, 0, FT), lambda: part(1, 1, FB),
                        lambda: part(0, 0, FT) + part(0, 1, FT), lambda: part(1, 0, FB) - part(0, 0, FB),
                        lambda: both(1, jnp.subtract))[k]().astype(BF16)

            b11, b12, b21, b22 = (
                jnp.concatenate([rhs[2 * j + c][128 * r:128 * r + 128] for j in range(NB)], axis=1)
                for c in (0, 1) for r in (0, 1))
            m = lambda k, x: _nt(left(k), x.astype(BF16))
            m2, m5 = m(1, b11), m(4, b22)
            b11, b12, b21, b22 = (x.astype(F32) for x in (b11, b12, b21, b22))
            m4 = m(3, b21 - b11)
            m1, m7, m3, m6 = m(0, b11 + b22), m(6, b21 + b22), m(2, b12 - b22), m(5, b11 + b12)
            c11 = jnp.concatenate([m4 - m5[:FB], -m5[FB:]], axis=0) + m1 + m7
            c22 = (m1[:FB] - m2) + m3[:FB] + m6
            return jnp.concatenate([jnp.concatenate([c11, m5 + m3], axis=1),
                                    jnp.concatenate([m2 + m4, c22], axis=1)], axis=0)

        def gate(r, c, g):
            tiles = [i * TB + c * (H // 128) + t for t in range(H // 128)]
            bias = jnp.concatenate([bf_v[pl.ds(j, 1), :] for j in tiles], axis=1)
            z1 = jnp.concatenate([z1_v[j, pl.ds(FM * r, FM), :] for j in tiles], axis=1)
            return _gelu_scaled(z1) * (g + bias)

        s2 = prod(1, w(0, 0))
        s5 = prod(4, w(1, 1))
        s4 = prod(3, comb(w(1, 0), w(0, 0), -1))
        p21 = gate(1, 0, s2 + s4)
        d11 = s4 - s5
        s1 = prod(0, comb(w(0, 0), w(1, 1), 1))
        d11, d22 = d11 + s1, s1 - s2
        p11 = gate(0, 0, d11 + prod(6, comb(w(1, 0), w(1, 1), 1)))
        s3 = prod(2, comb(w(0, 1), w(1, 1), -1))
        p12 = gate(0, 1, s3 + s5)
        p22 = gate(1, 1, (d22 + s3) + prod(5, comb(w(0, 0), w(0, 1), 1)))
        return [jnp.concatenate(p, axis=0) for p in ((p11, p21), (p12, p22))]

    def flush(k):
        rows = _ds(k * H, H, H)
        return [pltpu.make_async_copy(o_v.at[j, rows], o_h.at[rows, pl.ds(128 * j, 128)], sems.at[2])
                for j in range(NCB)]

    def finish(r0, tile):
        for t in range(H // 128):
            for j in range(NCB):
                at = _ds(r0 + 128 * t, 128, 128), pl.ds(128 * j, 128)
                o_v[j, at[0], :] = (x1_v[at] + jnp.concatenate([_tile(gb, j)] * 8, axis=0)
                           * tile(t, j).T.astype(F32)).astype(BF16)

    def mix_step(i):
        p = mix(i)
        b11, b12, b21, b22 = (p[c][128 * KO * r:128 * KO * (r + 1)] for r in (0, 1) for c in (0, 1))

        def prod(n, rhs):
            return _nn(jnp.concatenate([_ld(wt_v, n, j) for j in range(KO)], axis=1), rhs.astype(BF16))

        def rest(c):
            tail = jnp.concatenate([p[c][256 * KO:], jnp.zeros((128 + 256 * KO - FH, H), F32)], axis=0)
            return _nn(_ld(wr_v, 2 * KO), tail.astype(BF16))

        r0 = rest(0)
        s2 = prod(1, b11)
        s4 = prod(3, b21 - b11)
        s5 = prod(4, b22)
        s1 = prod(0, b11 + b22)
        s7 = prod(6, b21 + b22)
        ot = jnp.concatenate([r0[:DM] + s4 - s5 + s1 + s7, r0[DM:] + s2 + s4], axis=0)
        finish(i * RB, lambda t, j: _tile(ot, t)[128 * j:128 * j + 128].astype(BF16))
        for cp in flush(2 * i):
            cp.start()
        spot = 0, _ds(i * RB + H, 16, 16)
        o_v[spot] = jnp.zeros((16, 128), BF16)
        pin = o_v[0, _ds(i * RB + H + zero, 16, 16)].astype(F32)
        r1 = rest(1)
        s3 = prod(2, b12 - b22)
        b = b11 + b12
        b = jnp.concatenate([b[:-16], jnp.concatenate([b[-16:, :128], tie(pin, b[-16:, 128:])], axis=1)], axis=0)
        s6 = prod(5, b)
        ot = jnp.concatenate([r1[:DM] + s5 + s3, (s1 - s2) + r1[DM:] + s3 + s6], axis=0)
        finish(i * RB + H, lambda t, j: _tile(ot, t)[128 * j:128 * j + 128].astype(BF16))
        for cp in flush(2 * i + 1):
            cp.start()

    zero = pl.multiple_of(zero_s[0], 16)
    zero = zero_s[0]
    pl.loop(0, NB)(mix_step)
    for k in range(S // H):
        for cp in flush(k):
            cp.wait()


@jax.jit
def pallas_adaLN_cond__ssm_conv_h3__mixer_gmlp__prompt_kernel(
    A_q, A_k, A_v, A_shift_k, A_ssm_k, A_ssm_D, B_x, B_w_in, B_w_sp, B_b_sp, B_w_out, c, w_mod,
):
    del B_x
    vm = pltpu.VMEM
    tile = (128, 128)
    scratch = [
        vm((S, D), BF16), vm((NCB, PAD + S, 128), BF16), vm((NCB, S, 128), BF16), vm((TAPS, D), BF16),
        vm((NCB, NA, 128, CH), BF16), vm((NCB, 128), BF16), vm((2 * FH, D), BF16),
        vm((S // 128, S, 128), BF16), vm((S // 128, 128), BF16), vm((256 * KO + 128, D), BF16), vm((1, D), BF16),
        vm((D, 6 * D), BF16), vm((16, *tile), BF16),
        vm((8, 2 * NA, *tile), BF16), vm((8, 2 * NA, *tile), BF16),
        vm((2 * NA, *tile), F32), vm((2 * NA, *tile), F32), vm((NA, *tile), BF16), vm((NA, *tile), BF16),
        vm((16, NA, *tile), F32), vm((16, NA, *tile), F32), vm((5, NA, *tile), F32), vm((5, NA, *tile), F32),
        vm((NCB, S, 128), F32), vm((S, D), F32), vm((NCB, RB, 128), BF16),
        vm((S // 128, FH, 128), F32), vm((7, S // 256, FM, 128), F32),
        vm((7, KO, DM, 128), BF16), vm((2 * KO + 1, D, 128), BF16), vm((S // 128, 128), F32),
        vm((NCB, S, 128), BF16), vm((8, 128), jnp.int32), pltpu.SMEM((1,), jnp.int32),
        pltpu.SemaphoreType.DMA((13,)),
    ]
    scratch += [vm((FH, 128), F32)] * 16 + [vm((FH // SU * 16, 128), F32)] * 16
    scratch += ([vm((2, H, 128), BF16)] * 7 + [vm((1, H, 128), BF16)] * 2) * 2
    out = pl.pallas_call(
        _kernel,
        out_shape=jax.ShapeDtypeStruct((S, D), BF16),
        in_specs=[pl.BlockSpec(memory_space=pltpu.HBM)] * 12,
        out_specs=pl.BlockSpec(memory_space=pltpu.HBM),
        scratch_shapes=scratch,
        compiler_params=pltpu.CompilerParams(vmem_limit_bytes=110 * 1024 * 1024),
    )(A_q.reshape(S, D), A_k.reshape(S, D), A_v.reshape(S, D), A_shift_k.T, A_ssm_k,
      A_ssm_D.reshape(NCB, 128), B_w_in.T, B_w_sp, B_b_sp.reshape(S // 128, 128), B_w_out, c, w_mod)
    return out.reshape(1, S, D)
```

```python
import functools
import math

import numpy as np
import jax
import jax.numpy as jnp
from jax import lax
import jax.experimental.pallas as pl
import jax.experimental.pallas.tpu as pltpu

S, D, FH = 2048, 640, 864
FM, DM = FH // 2, D // 2
KO = FH // 256
FT, FB = 224, 208
TAPS = 4
CH = 512
NA = S // CH
N2 = 64
N1 = CH // N2
NCB = D // 128
RB = 512
NB = S // RB
H = RB // 2
EPS = 1e-5
F32, BF16, U32 = jnp.float32, jnp.bfloat16, jnp.uint32
PAD = 16

_C8 = math.cos(math.pi / 8)
_T8 = math.tan(math.pi / 8)
_R2 = math.sqrt(0.5)
_G0 = math.sqrt(2 / math.pi)
_GA = (_G0 * 0.044715) ** (1 / 3)

E0, ES = 0, 16
TU = (-1, 0, 3, 5, 16, 32, 35, 38)
TK = (34, 38, 41, 42, 43, 44, 45, 46)
TI = (-1, -1, -1, 0, 0, 2, 3, 4, 5, 5, 7, 16, 17, 17, 32, 33, 34, 36, 37, 38, 38, 39, 40, 42)
SU = 24
NJ = [
    "s0:70:89,s1:118:190,s2:168:205,m14:100:120,m18:120:150,m15:150:180,m19:180:210,m13:54:80,m17:70:100",
    "h3:0:96,h2:118:219,s3:20:80",
    "h5:0:108:142:196,h4:182:246:314:430,s4:330:418,s6:222:276",
    "h7:22:114:162:216,h6:226:280:330:446,s5:0:70,s7:44:98,s8:324:372,s10:240:270,n0:370:486",
    "s9:0:40,s11:40:80,n1:0:56,n2:56:112,n3:112:168,n4:168:224,n5:218:280,s14:160:206,s15:220:270,n7:280:344,s12:330:378,s13:380:410,n6:414:474,t0:10:330,o0:370:470",
]


def _dft_mats():
    def turn(k):
        return [jnp.cos(((k - s) & 1023).astype(F32) * (2 * math.pi / 1024)) for s in (0, 256)]

    def times(x, y, i):
        return [x[0] * y[0][i:i + 1] - x[1] * y[1][i:i + 1], x[0] * y[1][i:i + 1] + x[1] * y[0][i:i + 1]]

    row, col = (lax.broadcasted_iota(jnp.int32, (8, 128), d) for d in (0, 1))
    n, imag = (col >> 5) * 16 + (col & 7) * 2 + ((col >> 4) & 1), (col >> 3) & 1
    root = jnp.where(row < 4, 1 + 4 * row, jnp.where(row < 6, 8 * row - 30, 4))
    root = [t * jnp.where(row < 4, _C8 / 8, 1 / 8) for t in turn(root * n + 256 * imag)]
    fine, coarse = turn(16 * row * n), turn(128 * row * n)
    rows = [[t for g in range(8) for t in times(base, coarse, g)]
            for base in (times(fine, root, b) for b in range(7))]
    n = n + 64 * imag
    fine, coarse = [t * (1 / 8) for t in turn(8 * row * n)], turn(64 * row * n)
    last = [t for g in range(8) for t in times(fine, coarse, g)]
    last[1] = jnp.where(row == 0, (1 - 2 * (n & 1)).astype(F32) * (1 / 8), last[1])
    return [jnp.concatenate(r, axis=0).astype(BF16) for r in rows + [last]]


def _outer_fwd(u):
    t0r, t0i = u[0] * (1 / _C8), u[4] * (1 / _C8)
    t2r, t2i = (u[2] - u[6]) * (_R2 / _C8), (u[2] + u[6]) * (_R2 / _C8)
    t1r, t1i = u[1] - _T8 * u[5], u[5] + _T8 * u[1]
    t3r, t3i = _T8 * u[3] - u[7], _T8 * u[7] + u[3]
    ar, ai, br, bi = t0r + t2r, t0i + t2i, t0r - t2r, t0i - t2i
    cr, ci, dr, di = t1r + t3r, t1i + t3i, t1r - t3r, t1i - t3i
    out = [(ar + cr, ai + ci), (br - di, bi + dr), (ar - cr, ai - ci), (br + di, bi - dr)]
    p = [u[j] + u[j + 4] for j in range(4)]
    q = [u[j] - u[j + 4] for j in range(4)]
    er, ei = (q[1] - q[3]) * _R2, (q[1] + q[3]) * _R2
    out += [(q[0] + er, q[2] + ei), (q[0] - er, q[2] - ei)]
    out += [(p[0] - p[2], p[1] - p[3]), (p[0] + p[2], p[1] + p[3])]
    return out


def _outer_inv(B):
    ar, ai = B[0][0] + B[2][0], B[0][1] + B[2][1]
    cr, ci = B[0][0] - B[2][0], B[0][1] - B[2][1]
    br, bi = B[1][0] + B[3][0], B[1][1] + B[3][1]
    dr, di = B[1][0] - B[3][0], B[1][1] - B[3][1]
    g0r, g0i, g2r, g2i = ar + br, ai + bi, ar - br, ai - bi
    g1r, g1i, g3r, g3i = cr + di, ci - dr, cr - di, ci + dr
    nr = [g0r * (1 / _C8), g1r + _T8 * g1i, (g2r + g2i) * (_R2 / _C8), _T8 * g3r + g3i]
    ni = [g0i * (1 / _C8), g1i - _T8 * g1r, (g2i - g2r) * (_R2 / _C8), _T8 * g3i - g3r]
    fr, fi = B[4][0] - B[5][0], B[4][1] - B[5][1]
    q = [B[4][0] + B[5][0], (fr + fi) * _R2, B[4][1] + B[5][1], (fi - fr) * _R2]
    p = [B[7][0] + B[6][0], B[7][1] + B[6][1], B[7][0] - B[6][0], B[7][1] - B[6][1]]
    return ([p[j] + q[j] + nr[j] for j in range(4)]
            + [p[j] - q[j] + ni[j] for j in range(4)])


def _gelu_scaled(x):
    t = jnp.tanh(x * (_G0 / _GA + x * x))
    return x + x * t


def _norm_stats(s1, s2, n, eps):
    m = s1 * (1.0 / n)
    return m, jnp.exp(-0.5 * jnp.log(jnp.maximum(s2 * (1.0 / n) - m * m, 0.0) + eps))


def _ln_rows(x):
    m, r = _norm_stats(jnp.sum(x, axis=-1, keepdims=True), jnp.sum(x * x, axis=-1, keepdims=True),
                       x.shape[-1], EPS)
    return (x - m) * r


def _lhs7(a11, a12, a21, a22):
    return a11 + a22, a21 + a22, a11, a22, a11 + a12, a21 - a11, a12 - a22


def _words(ref, *idx):
    return ref.bitcast(U32)[idx]


def _ld(ref, *idx):
    return pltpu.bitcast(_words(ref, *idx), BF16)


def _phase(words, odd):
    return pltpu.bitcast(words & np.uint32(0xFFFF0000) if odd else words << 16, F32)


def _nn(a, b):
    return jnp.dot(a, b, preferred_element_type=F32)


def _nt(a, b):
    return lax.dot_general(a, b, (((1,), (1,)), ((), ())), preferred_element_type=F32)


def _ds(start, size, align):
    return pl.ds(start if isinstance(start, int) else pl.multiple_of(start, align), size)


def _tile(x, j, n=1):
    return x[:, 128 * j:128 * (j + n)]


def _add(xs):
    return functools.reduce(lambda x, y: x + y, xs)


def _kernel(q_h, k_h, v_h, sh_h, sk_h, sd_h, wi_h, ws_h, b_h, wo_h, c_h, wm_h, o_h,
            q_v, k_v, v_v, sh_v, sk_v, sd_v, wi_v, ws_v, b_v, wo_v, c_v, wm_v, vf_v,
            au0_v, au1_v, fa_v, fb_v, ya_v, yb_v, bm0_v, bp0_v, bm1_v, bp1_v,
            y_v, x1_v, h0_v, z1_v, z2_v, wt_v, wr_v, bf_v, o_v, tie_v, zero_s,
            sems, *lists):
    au_v, zf_v, sum_v, h_v = (au0_v, au1_v), lists[:16], lists[16:32], (lists[32:41], lists[41:])
    copies = {}

    def start(group, sem, *pairs):
        copies[group] = [pltpu.make_async_copy(src, dst, sems.at[sem]) for src, dst in pairs]
        for cp in copies[group]:
            cp.start()

    def wait(*groups):
        for group in groups:
            for cp in copies[group]:
                cp.wait()

    def conv_inputs(cb, a):
        rows, lanes, sem = _ds(a * CH, CH, CH), pl.ds(cb * 128, 128), sems.at[cb % 3 * NA + a]
        return (pltpu.make_async_copy(k_h.at[rows, lanes], k_v.at[cb, _ds(PAD + a * CH, CH, PAD)], sem),
                pltpu.make_async_copy(v_h.at[rows, lanes], v_v.at[cb, rows], sem),
                pltpu.make_async_copy(sk_h.at[lanes, rows], sk_v.at[cb, a], sem))

    def fetch(stage):
        rows = lambda r, n: (q_h.at[pl.ds(r, n)], q_v.at[pl.ds(r, n)])
        if stage == 0:
            start("taps", 12, (sh_h, sh_v), (sd_h, sd_v))
        if stage < 3:
            for a in range(NA):
                for cp in conv_inputs(stage, a):
                    cp.start()
        if stage == 4:
            later = []
            for a in range(NA):
                (k3, v3, f3), (k4, v4, f4) = conv_inputs(3, a), conv_inputs(4, a)
                later.append(f4)
                for cp in (k3, k4, v3, v4, f3):
                    cp.start()
            for cp in later:
                cp.start()
        if stage == NCB:
            start("mod", 8, (c_h, c_v), (wm_h.at[:, pl.ds(0, 5 * D)], wm_v.at[:, pl.ds(0, 5 * D)]), rows(0, H))
            start("gate", 9, (wi_h.at[pl.ds(FH, FH)], wi_v.at[pl.ds(0, FH)]), rows(H, H))
            start("value", 10, (wi_h.at[pl.ds(0, FH)], wi_v.at[pl.ds(FH, FH)]), rows(RB, 2 * RB))
        if stage == NCB + 2:
            start("out", 0, rows(3 * RB, RB), (wm_h.at[:, pl.ds(5 * D, D)], wm_v.at[:, pl.ds(5 * D, D)]),
                  (b_h, b_v), (wo_h, wo_v.at[pl.ds(0, FH)]))
            start("mix", 1, *[(ws_h.at[:, pl.ds(128 * j, 128)], ws_v.at[j]) for j in range(S // 128)])

    fetch(0)
    fetch(1)
    for ref in (fb_v, ya_v, tie_v):
        ref[...] = jnp.zeros(ref.shape, ref.dtype)
    k_v[:, pl.ds(0, PAD), :] = jnp.zeros((NCB, PAD, 128), BF16)
    wo_v[pl.ds(FH, 256 * KO + 128 - FH), :] = jnp.zeros((256 * KO + 128 - FH, D), BF16)
    row, col = (lax.broadcasted_iota(jnp.int32, (128, 128), d) for d in (0, 1))
    n = (col >> 5) * 16 + (col & 7) * 2 + ((col >> 4) & 1)
    order = jnp.where(row == (n >> 3) * 16 + (col & 8) + (n & 7), 1.0, 0.0).astype(BF16)
    mats = _dft_mats()
    back = _nt(order, jnp.concatenate(mats, axis=0))
    for b in range(8):
        vf_v[b] = mats[b]
        vf_v[8 + b] = _tile(back, b).astype(BF16)
    zero_s[0] = 0
    row8 = lax.broadcasted_iota(jnp.int32, (8, 128), 0)

    def tie(after, x):
        if after is None:
            return x
        never = jnp.concatenate([tie_v[...]] * (x.shape[0] // 8), axis=0) != 0
        return jnp.where(never, after, x)

    def put(cb, slot, g, res):
        for b in range(8):
            au_v[cb % 2][b, slot, pl.ds(16 * g, 16), :] = jnp.concatenate(res[b], axis=0).astype(BF16)

    def split_filter(cb, a, after):
        kt = pltpu.bitcast(sk_v[cb, a].T, U32)
        for g in range(N2 // 8):
            u = [_phase(kt[j * N2 // 2 + g // 2 * 8:j * N2 // 2 + g // 2 * 8 + 8], g % 2) for j in range(N1)]
            if g == 0:
                u[0] = u[0] + jnp.where(row8 + a == 0, sd_v[...].astype(F32)[cb:cb + 1], 0.0)
            u[:4] = [tie(after(g), x) for x in u[:4]]
            put(cb, NA + a, g, _outer_fwd(u))

    def split_signal(cb, a, after):
        taps = [jnp.broadcast_to(sh_v[j:j + 1, pl.ds(cb * 128, 128)].astype(F32), (8, 128))
                for j in range(TAPS)]
        base = a * (CH // 2) if isinstance(a, int) else pl.multiple_of(a * (CH // 2), CH // 2)
        for g in range(N2 // 8):
            w = [tie(after(g), t) for t in taps]
            u = []
            for j in range(N1):
                r = base + j * N2 // 2 + g // 2 * 8
                lag = [_phase(_words(k_v, cb, pl.ds(r + PAD // 2 + (g % 2 - t) // 2, 8)), (g % 2 - t) % 2)
                       for t in range(TAPS)]
                u.append(_add([x * wt for x, wt in zip(lag, w)]) * _phase(_words(v_v, cb, pl.ds(r, 8)), g % 2))
            put(cb, a, g, _outer_fwd(u))

    def spectra(cb, b, half, f_ref):
        rhs = jnp.concatenate([_ld(au_v[cb % 2], b, half * NA + a) for a in range(NA)], axis=1)
        f = _nn(_ld(vf_v, b), rhs)
        for a in range(NA):
            f_ref[half * NA + a] = f[:, 128 * a:128 * a + 128]
        return f

    def product(f_ref, y_ref, plus, real_rows=None):
        for g in range(8):
            ur, ui, kr, ki = ([f_ref[o + a, pl.ds(16 * g + 8 * c, 8), :] for a in range(NA)]
                              for o in (0, NA) for c in (0, 1))
            kr, ki = ([k[0]] + [k[a] + k[a - 1] if plus else k[a] - k[a - 1] for a in range(1, NA)]
                      for k in (kr, ki))
            for a in range(NA):
                yi = _add([kr[j] * ui[a - j] + ki[j] * ur[a - j] for j in range(a + 1)])
                if real_rows is not None and g == 0:
                    rr = _add([kr[j] * ur[a - j] for j in range(a + 1)])
                    ii = _add([ki[j] * ui[a - j] for j in range(a + 1)])
                    yr = jnp.where(real_rows, 0.5 * rr, rr - ii)
                    yi = jnp.where(real_rows, 0.5 * ii, yi)
                else:
                    yr = _add([kr[j] * ur[a - j] - ki[j] * ui[a - j] for j in range(a + 1)])
                y_ref[a, pl.ds(16 * g, 16), :] = jnp.concatenate([yr, yi], axis=0).astype(BF16)

    def residues(y_ref, b, dst):
        r = _nn(_ld(vf_v, 8 + b), jnp.concatenate([_ld(y_ref, a) for a in range(NA)], axis=1))
        for a in range(NA):
            dst[a] = r[:, 128 * a:128 * a + 128]
        return r

    def stash(t):
        return ((bm0_v.at[t], bp0_v.at[t]) if t < 16 else (bm1_v.at[t - 16], bp1_v.at[t - 16]))

    def merge(cb, a, after=lambda g: None):
        src = [stash(1 + 4 * cb + b)[s] for s in (0, 1) for b in range(4)]
        for g in range(N2 // 8):
            res = [[ref[a, pl.ds(16 * g + 8 * c, 8), :] for c in (0, 1)] for ref in src]
            res[0] = [tie(after(g), x) for x in res[0]]
            res[1] = [tie(after(g), x) for x in res[1]]
            for j, y in enumerate(_outer_inv(res)):
                y_v[cb, _ds(a * CH + j * N2 + 8 * g, 8, 8), :] = y

    def transform(cb, a, dst, active=True):
        pa = (a + 3) % 4
        res = []
        if active:
            res += [spectra(cb, a, 1, fa_v), spectra(cb, a, 0, fa_v)]
        product(fb_v, yb_v, True, row8 + (3 - pa) == 0)
        res.append(residues(ya_v, pa, dst[0]))
        if active:
            res += [spectra(cb, 4 + a, 1, fb_v), spectra(cb, 4 + a, 0, fb_v)]
            product(fa_v, ya_v, False)
        res.append(residues(yb_v, 4 + pa, dst[1]))
        return res

    def conv_step(cb, a):
        if cb < NCB:
            for cp in conv_inputs(cb, a):
                cp.wait()
        if cb:
            done = transform(cb - 1, a, (bm0_v.at[4 * cb - 4 + a], bp0_v.at[4 * cb - 4 + a])
                             if cb < NCB else (bm1_v.at[a], bp1_v.at[a]))
        at = lambda p: done[p // 8][16 * (p % 8):16 * (p % 8) + 8, 0:128] if cb and p >= 0 else None
        if cb < NCB:
            split_signal(cb, a, lambda g: at(TU[g]))
            split_filter(cb, a, lambda g: at(TK[g]))
        else:
            for c in range(3):
                merge(c, a, lambda g: at(TI[8 * c + g]))

    wait("taps")
    for cb in range(NCB + 1):
        fetch(cb + 2)
        pl.loop(0, NA)(functools.partial(conv_step, cb))

    wait("mod")
    transform(NCB, 0, stash(20), active=False)
    cc = c_v[...].astype(F32)
    sc = jnp.broadcast_to(cc / (1.0 + jnp.exp(-cc)), (16, D)).astype(BF16)
    mod = _nn(sc, jnp.concatenate([wm_v[:, pl.ds(i * D, D)] for i in (0, 1, 2, 4, 3)], axis=1))[0:8]
    sa, ca, ga, cb_, sb = (mod[:, i * D:(i + 1) * D] for i in range(5))
    m1, m0 = ga * (1.0 + ca), ga * sa
    n1, n0 = _GA * (1.0 + cb_), _GA * sb
    zero = zero_s[0]
    for n, cb in enumerate((3, 4)):
        merge(cb, zero, lambda g: _tile(mod, (8 * n + g) * 3 // 4))

    TB = RB // 128

    def hidden(r0, after=(None, None)):
        out = []
        for r, a in zip((r0, r0 + 8), after):
            rows = pl.ds(r, 8)
            x = q_v[rows, :].astype(F32)
            x = jnp.concatenate([tie(a, x[:, :128]), x[:, 128:]], axis=1)
            x1 = x + (_ln_rows(x) * m1 + m0) * jnp.concatenate([y_v[j, rows, :] for j in range(NCB)], axis=1)
            x1_v[rows, :] = x1
            out.append(_ln_rows(x1) * n1 + n0)
        return jnp.concatenate(out, axis=0)

    def keep_gate(tile, z):
        zf_v[tile][pl.ds(zero, FH), :] = z

    def moments(tile, after):
        z, acc = zf_v[tile], sum_v[tile]
        s1 = s2 = None
        for n, f in enumerate(range(0, FH, SU)):
            for r in range(f, f + SU, 8):
                d = tie(after(n)[:8] if r == f else None, z[pl.ds(r, 8), :])
                s1, s2 = (d, d * d) if s1 is None else (s1 + d, s2 + d * d)
            acc[pl.ds(16 * n + zero, 16), :] = jnp.concatenate([s1, s2], axis=0)
        s1, s2 = (jnp.sum(acc[pl.ds(16 * n + r, 8), :], axis=0, keepdims=True) for r in (0, 8))
        stats[tile] = [jnp.broadcast_to(t, (8, 128)) for t in _norm_stats(s1, s2, FH, EPS * (2 * _GA) ** 2)]

    def norm_gate(pair, after):
        for n in range(FM // 8):
            means = [tie(after(n)[:8], stats[2 * pair + c][0]) for c in (0, 1)]
            quad = [(zf_v[2 * pair + c][pl.ds(r + 8 * n, 8), :] - means[c]) * stats[2 * pair + c][1]
                    for r in (0, FM) for c in (0, 1)]
            for k, a in enumerate(_lhs7(*quad)):
                z2_v[k, pair, pl.ds(8 * n, 8), :] = a

    def prepare(i, c, after):
        def put(k, n, x):
            for j in range(x.shape[1] // 128):
                h_v[i % 2][k][j, pl.ds(16 * n + zero, 16), :] = _tile(x, j).astype(BF16)

        for n in range(H // 16):
            h = hidden(i * RB + c * H + 16 * n, (after(2 * n)[:8], after(2 * n + 1)[:8]))
            top, bot = _tile(h, 0, 2), _tile(h, 2, 2)
            put(7 + c, n, _tile(h, 4))
            if c:
                half[n] = top, bot
                put(2, n, top - bot)
                put(4, n, bot)
            else:
                put(1, n, top)
                put(3, n, bot - top)
                put(0, n, top + half[n][1])
                put(5, n, top + half[n][0])
                put(6, n, bot + half[n][1])

    def turn_out(after):
        for n in range((2 * KO + 1) * NCB):
            j, t = divmod(n, NCB)
            w = _words(wo_v, pl.ds(64 * j, 64), pl.ds(128 * t, 128))
            w = jnp.concatenate([tie(pltpu.bitcast(after(n)[:8], U32), w[:8]), w[8:]], axis=0)
            wr_v[j, pl.ds(128 * t + zero, 128), :] = pltpu.bitcast(w, BF16).T

    def split_out(after):
        for n in range(KO * DM // 16):
            j, r = divmod(16 * n, DM)
            quad = [wr_v[j + KO * c, pl.ds(r + DM * b, 16), :].astype(F32) for b in (0, 1) for c in (0, 1)]
            for k, a in enumerate(_lhs7(tie(after(n), quad[0]), quad[1], quad[2], tie(after(n), quad[3]))):
                wt_v[k, j, pl.ds(r, 16), :] = a.astype(BF16)

    def side_jobs(plan, at):
        for job in plan.split(","):
            if job:
                kind, (n, *spans) = job[0], (int(x) for x in job[1:].split(":"))
                total = {"s": FH // SU, "n": FM // 8, "h": H // 8, "m": N2 // 8,
                         "t": (2 * KO + 1) * NCB, "o": KO * DM // 16}[kind]
                slots = [p for lo, hi in zip(spans[::2], spans[1::2]) for p in range(lo, hi)]
                after = lambda k: at(slots[k * len(slots) // total])
                if kind == "s":
                    moments(n, after)
                elif kind == "m":
                    merge(n // NA, n % NA + zero, lambda k: after(k)[:8])
                elif kind in "to":
                    (turn_out if kind == "t" else split_out)(after)
                elif kind == "n":
                    norm_gate(n, after)
                else:
                    prepare(n // 2, n % 2, after)

    def rows_of(z):
        per = z.shape[0] // 16
        return lambda p: z[16 * (p % per):16 * (p % per) + 16, 128 * (p // per):128 * (p // per) + 128]

    def project(i):
        def prod(*pairs):
            right = [_ld(h_v[i % 2][k], j) for _, k in pairs for j in range(2 if k < 7 else 1)]
            return _nt(jnp.concatenate([x for k, _ in pairs for x in left[k]], axis=1),
                       jnp.concatenate(right, axis=1))

        s5, s3, r12, s4, s1 = prod((4, 4)), prod((2, 2)), prod((7, 8)), prod((3, 3)), prod((0, 0))
        s7, s2, r21, s6 = prod((6, 6), (7, 7)), prod((1, 1)), prod((8, 7)), prod((5, 5), (8, 8))
        gate = [((s4 - s5) + s1) + s7, (s5 + s3) + r12]
        value = [(s4 + s2) + r21, ((s3 + s1) - s2) + s6]
        for t in range(TB):
            keep_gate(i * TB + t, _gelu_scaled(_tile(gate[t // 2], t % 2)))
            z1_v[i * TB + t] = _tile(value[t // 2], t % 2).astype(BF16)
        rounds = (s5, s3, gate[1], _tile(s4, 1), _tile(s1, 1), gate[0], s2, value[0], _tile(value[1], 1))
        return lambda p: rounds[p // (FH // 16)][16 * (p % (FH // 16)):16 * (p % (FH // 16)) + 16, 0:128]

    def first(f0, r0, n, k0, k1):
        h = jnp.concatenate([_ld(h0_v, j, pl.ds(r0 // 2, n // 2)) for j in range(k0, k1)], axis=1)
        return _nt(wi_v[pl.ds(f0, FH), pl.ds(128 * k0, 128 * (k1 - k0))], h)

    def keep_first(r, h):
        for j in range(NCB):
            h0_v[j, pl.ds(r, 16), :] = _tile(h, j).astype(BF16)

    stats, half = {}, {}
    for r in range(0, H, 16):
        keep_first(r, hidden(r))
    wait("gate")
    zero = pl.multiple_of(zero_s[0], 16)
    head = first(0, 0, H, 0, 2)
    z = _gelu_scaled(head + first(0, 0, H, 2, NCB))
    at = rows_of(jnp.concatenate([_tile(head, 0), z], axis=1))
    for n in range(H // 16):
        keep_first(H + 16 * n, hidden(H + 16 * n, [at(E0 + (2 * n + k) * ES // 8)[:8] for k in (0, 1)]))
    z = jnp.concatenate([z] + [_gelu_scaled(first(0, r, 128, 0, NCB)) for r in (H, H + 128)], axis=1)
    for t in range(TB):
        keep_gate(t, _tile(z, t))
    side_jobs(NJ[0], rows_of(z))
    wait("value")
    head = first(FH, 0, RB, NCB - 1, NCB)
    z = head + first(FH, 0, RB, 0, NCB - 1)
    for t in range(TB):
        z1_v[t] = _tile(z, t).astype(BF16)
    side_jobs(NJ[1], rows_of(jnp.concatenate([_tile(head, 0), z], axis=1)))
    sums = [_lhs7(*(wi_v[pl.ds(FH * r, FH), pl.ds(256 * c + 128 * j, 128)].astype(F32)
                    for r in (0, 1) for c in (0, 1))) for j in (0, 1)]
    left = ([[s[k].astype(BF16) for s in sums] for k in range(7)]
            + [[wi_v[pl.ds(FH * r, FH), pl.ds(512, 128)]] for r in (0, 1)])
    for i in range(1, NB):
        if i == 2:
            wait("out")
        side_jobs(NJ[i + 1], project(i))
    gb = _nn(sc, wm_v[:, pl.ds(5 * D, D)]) * (0.5 / _GA)
    bf_v[...] = b_v[...].astype(F32)

    wait("mix")

    def mix(i):
        def w(c, r):
            return [_ld(ws_v, 2 * j + c, _ds((i * RB + r * H) // 2, H // 2, H // 2))
                    for j in range(S // 256)]

        def comb(x, y, sign):
            return [(jnp.add if sign > 0 else jnp.subtract)(a.astype(F32), b.astype(F32)) for a, b in zip(x, y)]

        def prod(n, rhs):
            def left(k):
                def part(r, c, rows):
                    return jnp.concatenate([z2_v[n, 2 * j + c, pl.ds(FT * r, rows), :] for j in range(NB)], axis=1)

                def both(c, op):
                    top = part(0, c, FT)
                    return jnp.concatenate([op(top[:FB], part(1, 1, FB)), top[FB:]], axis=0)

                return (lambda: both(0, jnp.add), lambda: part(1, 0, FB) + part(1, 1, FB),
                        lambda: part(0, 0, FT), lambda: part(1, 1, FB),
                        lambda: part(0, 0, FT) + part(0, 1, FT), lambda: part(1, 0, FB) - part(0, 0, FB),
                        lambda: both(1, jnp.subtract))[k]().astype(BF16)

            b11, b12, b21, b22 = (
                jnp.concatenate([rhs[2 * j + c][128 * r:128 * r + 128] for j in range(NB)], axis=1)
                for c in (0, 1) for r in (0, 1))
            m = lambda k, x: _nt(left(k), x.astype(BF16))
            m2, m5 = m(1, b11), m(4, b22)
            b11, b12, b21, b22 = (x.astype(F32) for x in (b11, b12, b21, b22))
            m4 = m(3, b21 - b11)
            m1, m7, m3, m6 = m(0, b11 + b22), m(6, b21 + b22), m(2, b12 - b22), m(5, b11 + b12)
            c11 = jnp.concatenate([m4 - m5[:FB], -m5[FB:]], axis=0) + m1 + m7
            c22 = (m1[:FB] - m2) + m3[:FB] + m6
            return jnp.concatenate([jnp.concatenate([c11, m5 + m3], axis=1),
                                    jnp.concatenate([m2 + m4, c22], axis=1)], axis=0)

        def gate(r, c, g):
            tiles = [i * TB + c * (H // 128) + t for t in range(H // 128)]
            bias = jnp.concatenate([bf_v[pl.ds(j, 1), :] for j in tiles], axis=1)
            z1 = jnp.concatenate([z1_v[j, pl.ds(FM * r, FM), :] for j in tiles], axis=1).astype(F32)
            return _gelu_scaled(z1) * (g + bias)

        s2 = prod(1, w(0, 0))
        s5 = prod(4, w(1, 1))
        s4 = prod(3, comb(w(1, 0), w(0, 0), -1))
        p21 = gate(1, 0, s2 + s4)
        d11 = s4 - s5
        s1 = prod(0, comb(w(0, 0), w(1, 1), 1))
        d11, d22 = d11 + s1, s1 - s2
        p11 = gate(0, 0, d11 + prod(6, comb(w(1, 0), w(1, 1), 1)))
        s3 = prod(2, comb(w(0, 1), w(1, 1), -1))
        p12 = gate(0, 1, s3 + s5)
        p22 = gate(1, 1, (d22 + s3) + prod(5, comb(w(0, 0), w(0, 1), 1)))
        return [jnp.concatenate(p, axis=0) for p in ((p11, p21), (p12, p22))]

    def flush(k):
        rows = _ds(k * H, H, H)
        return [pltpu.make_async_copy(o_v.at[j, rows], o_h.at[rows, pl.ds(128 * j, 128)], sems.at[2])
                for j in range(NCB)]

    def finish(r0, tile):
        for cols in (range(DM // 128), range(DM // 128, NCB)):
            for t, j in ((t, j) for t in range(H // 128) for j in cols):
                at = _ds(r0 + 128 * t, 128, 128), pl.ds(128 * j, 128)
                o_v[j, at[0], :] = (x1_v[at] + jnp.concatenate([_tile(gb, j)] * 8, axis=0)
                           * tile(t, j).T.astype(F32)).astype(BF16)

    def mix_step(i):
        p = mix(i)
        b11, b12, b21, b22 = (p[c][128 * KO * r:128 * KO * (r + 1)] for r in (0, 1) for c in (0, 1))

        def prod(n, rhs):
            return _nn(jnp.concatenate([_ld(wt_v, n, j) for j in range(KO)], axis=1), rhs.astype(BF16))

        def rest(c):
            tail = jnp.concatenate([p[c][256 * KO:], jnp.zeros((128 + 256 * KO - FH, H), F32)], axis=0)
            return _nn(_ld(wr_v, 2 * KO), tail.astype(BF16))

        r0 = rest(0)
        s2 = prod(1, b11)
        s4 = prod(3, b21 - b11)
        s5 = prod(4, b22)
        s1 = prod(0, b11 + b22)
        s7 = prod(6, b21 + b22)
        ot = jnp.concatenate([r0[:DM] + s4 - s5 + s1 + s7, r0[DM:] + s2 + s4], axis=0)
        finish(i * RB, lambda t, j: _tile(ot, t)[128 * j:128 * j + 128].astype(BF16))
        for cp in flush(2 * i):
            cp.start()
        spot = 0, _ds(i * RB + H, 16, 16)
        o_v[spot] = jnp.zeros((16, 128), BF16)
        pin = o_v[0, _ds(i * RB + H + zero, 16, 16)].astype(F32)
        r1 = rest(1)
        s3 = prod(2, b12 - b22)
        b = b11 + b12
        b = jnp.concatenate([b[:-16], jnp.concatenate([b[-16:, :128], tie(pin, b[-16:, 128:])], axis=1)], axis=0)
        s6 = prod(5, b)
        ot = jnp.concatenate([r1[:DM] + s5 + s3, (s1 - s2) + r1[DM:] + s3 + s6], axis=0)
        finish(i * RB + H, lambda t, j: _tile(ot, t)[128 * j:128 * j + 128].astype(BF16))
        for cp in flush(2 * i + 1):
            cp.start()

    zero = pl.multiple_of(zero_s[0], 16)
    zero = zero_s[0]
    pl.loop(0, NB)(mix_step)
    for k in range(S // H):
        for cp in flush(k):
            cp.wait()


@jax.jit
def pallas_adaLN_cond__ssm_conv_h3__mixer_gmlp__prompt_kernel(
    A_q, A_k, A_v, A_shift_k, A_ssm_k, A_ssm_D, B_x, B_w_in, B_w_sp, B_b_sp, B_w_out, c, w_mod,
):
    del B_x
    vm = pltpu.VMEM
    tile = (128, 128)
    scratch = [
        vm((S, D), BF16), vm((NCB, PAD + S, 128), BF16), vm((NCB, S, 128), BF16), vm((TAPS, D), BF16),
        vm((NCB, NA, 128, CH), BF16), vm((NCB, 128), BF16), vm((2 * FH, D), BF16),
        vm((S // 128, S, 128), BF16), vm((S // 128, 128), BF16), vm((256 * KO + 128, D), BF16), vm((1, D), BF16),
        vm((D, 6 * D), BF16), vm((16, *tile), BF16),
        vm((8, 2 * NA, *tile), BF16), vm((8, 2 * NA, *tile), BF16),
        vm((2 * NA, *tile), F32), vm((2 * NA, *tile), F32), vm((NA, *tile), BF16), vm((NA, *tile), BF16),
        vm((16, NA, *tile), F32), vm((16, NA, *tile), F32), vm((5, NA, *tile), F32), vm((5, NA, *tile), F32),
        vm((NCB, S, 128), F32), vm((S, D), F32), vm((NCB, RB, 128), BF16),
        vm((S // 128, FH, 128), BF16), vm((7, S // 256, FM, 128), F32),
        vm((7, KO, DM, 128), BF16), vm((2 * KO + 1, D, 128), BF16), vm((S // 128, 128), F32),
        vm((NCB, S, 128), BF16), vm((8, 128), jnp.int32), pltpu.SMEM((1,), jnp.int32),
        pltpu.SemaphoreType.DMA((13,)),
    ]
    scratch += [vm((FH, 128), F32)] * 16 + [vm((FH // SU * 16, 128), F32)] * 16
    scratch += ([vm((2, H, 128), BF16)] * 7 + [vm((1, H, 128), BF16)] * 2) * 2
    out = pl.pallas_call(
        _kernel,
        out_shape=jax.ShapeDtypeStruct((S, D), BF16),
        in_specs=[pl.BlockSpec(memory_space=pltpu.HBM)] * 12,
        out_specs=pl.BlockSpec(memory_space=pltpu.HBM),
        scratch_shapes=scratch,
        compiler_params=pltpu.CompilerParams(vmem_limit_bytes=110 * 1024 * 1024),
    )(A_q.reshape(S, D), A_k.reshape(S, D), A_v.reshape(S, D), A_shift_k.T, A_ssm_k,
      A_ssm_D.reshape(NCB, 128), B_w_in.T, B_w_sp, B_b_sp.reshape(S // 128, 128), B_w_out, c, w_mod)
    return out.reshape(1, S, D)
```

```python
import functools
import math

import numpy as np
import jax
import jax.numpy as jnp
from jax import lax
import jax.experimental.pallas as pl
import jax.experimental.pallas.tpu as pltpu

S, D, FH = 2048, 640, 864
FM, DM = FH // 2, D // 2
KO = FH // 256
FT, FB = 224, 208
TAPS = 4
CH = 512
NA = S // CH
N2 = 64
N1 = CH // N2
NCB = D // 128
RB = 512
NB = S // RB
H = RB // 2
EPS = 1e-5
F32, BF16, U32 = jnp.float32, jnp.bfloat16, jnp.uint32
PAD = 16

_C8 = math.cos(math.pi / 8)
_T8 = math.tan(math.pi / 8)
_R2 = math.sqrt(0.5)
_G0 = math.sqrt(2 / math.pi)
_GA = (_G0 * 0.044715) ** (1 / 3)

HD = 384
E0, ES = 0, 16
TU = (-1, 0, 3, 5, 16, 32, 35, 38)
TK = (34, 38, 41, 42, 43, 44, 45, 46)
TI = (-1, -1, -1, 0, 0, 2, 3, 4, 5, 5, 7, 16, 17, 17, 32, 33, 34, 36, 37, 38, 38, 39, 40, 42)
SU = 24
NJ = [
    "s0:70:89,s1:130:180,s2:168:205,m14:100:120,m18:120:150,m15:150:180,m19:180:210,m13:38:64,m17:70:100",
    "h3:0:96,h2:118:219,s3:20:80",
    "h5:0:108:142:196,h4:182:246:314:430,s4:330:418,s6:212:266",
    "h7:22:114:162:216,h6:226:280:330:446,s5:0:70,s7:44:98,s8:324:372,s10:240:270,n0:370:486",
    "s9:6:40,s11:40:80,n1:0:56,n2:56:112,n3:112:168,n4:168:224,n5:218:280,s14:160:196,s15:220:270,n7:280:344,s12:330:378,s13:380:410,n6:414:474,t0:10:330,o0:370:470",
]


def _dft_mats():
    def turn(k):
        return [jnp.cos(((k - s) & 1023).astype(F32) * (2 * math.pi / 1024)) for s in (0, 256)]

    def times(x, y, i):
        return [x[0] * y[0][i:i + 1] - x[1] * y[1][i:i + 1], x[0] * y[1][i:i + 1] + x[1] * y[0][i:i + 1]]

    row, col = (lax.broadcasted_iota(jnp.int32, (8, 128), d) for d in (0, 1))
    n, imag = (col >> 5) * 16 + (col & 7) * 2 + ((col >> 4) & 1), (col >> 3) & 1
    root = jnp.where(row < 4, 1 + 4 * row, jnp.where(row < 6, 8 * row - 30, 4))
    root = [t * jnp.where(row < 4, _C8 / 8, 1 / 8) for t in turn(root * n + 256 * imag)]
    fine, coarse = turn(16 * row * n), turn(128 * row * n)
    rows = [[t for g in range(8) for t in times(base, coarse, g)]
            for base in (times(fine, root, b) for b in range(7))]
    n = n + 64 * imag
    fine, coarse = [t * (1 / 8) for t in turn(8 * row * n)], turn(64 * row * n)
    last = [t for g in range(8) for t in times(fine, coarse, g)]
    last[1] = jnp.where(row == 0, (1 - 2 * (n & 1)).astype(F32) * (1 / 8), last[1])
    return [jnp.concatenate(r, axis=0).astype(BF16) for r in rows + [last]]


def _outer_fwd(u):
    t0r, t0i = u[0] * (1 / _C8), u[4] * (1 / _C8)
    t2r, t2i = (u[2] - u[6]) * (_R2 / _C8), (u[2] + u[6]) * (_R2 / _C8)
    t1r, t1i = u[1] - _T8 * u[5], u[5] + _T8 * u[1]
    t3r, t3i = _T8 * u[3] - u[7], _T8 * u[7] + u[3]
    ar, ai, br, bi = t0r + t2r, t0i + t2i, t0r - t2r, t0i - t2i
    cr, ci, dr, di = t1r + t3r, t1i + t3i, t1r - t3r, t1i - t3i
    out = [(ar + cr, ai + ci), (br - di, bi + dr), (ar - cr, ai - ci), (br + di, bi - dr)]
    p = [u[j] + u[j + 4] for j in range(4)]
    q = [u[j] - u[j + 4] for j in range(4)]
    er, ei = (q[1] - q[3]) * _R2, (q[1] + q[3]) * _R2
    out += [(q[0] + er, q[2] + ei), (q[0] - er, q[2] - ei)]
    out += [(p[0] - p[2], p[1] - p[3]), (p[0] + p[2], p[1] + p[3])]
    return out


def _outer_inv(B):
    ar, ai = B[0][0] + B[2][0], B[0][1] + B[2][1]
    cr, ci = B[0][0] - B[2][0], B[0][1] - B[2][1]
    br, bi = B[1][0] + B[3][0], B[1][1] + B[3][1]
    dr, di = B[1][0] - B[3][0], B[1][1] - B[3][1]
    g0r, g0i, g2r, g2i = ar + br, ai + bi, ar - br, ai - bi
    g1r, g1i, g3r, g3i = cr + di, ci - dr, cr - di, ci + dr
    nr = [g0r * (1 / _C8), g1r + _T8 * g1i, (g2r + g2i) * (_R2 / _C8), _T8 * g3r + g3i]
    ni = [g0i * (1 / _C8), g1i - _T8 * g1r, (g2i - g2r) * (_R2 / _C8), _T8 * g3i - g3r]
    fr, fi = B[4][0] - B[5][0], B[4][1] - B[5][1]
    q = [B[4][0] + B[5][0], (fr + fi) * _R2, B[4][1] + B[5][1], (fi - fr) * _R2]
    p = [B[7][0] + B[6][0], B[7][1] + B[6][1], B[7][0] - B[6][0], B[7][1] - B[6][1]]
    return ([p[j] + q[j] + nr[j] for j in range(4)]
            + [p[j] - q[j] + ni[j] for j in range(4)])


def _gelu_scaled(x):
    t = jnp.tanh(x * (_G0 / _GA + x * x))
    return x + x * t


def _norm_stats(s1, s2, n, eps):
    m = s1 * (1.0 / n)
    return m, jnp.exp(-0.5 * jnp.log(jnp.maximum(s2 * (1.0 / n) - m * m, 0.0) + eps))


def _ln_rows(x):
    m, r = _norm_stats(jnp.sum(x, axis=-1, keepdims=True), jnp.sum(x * x, axis=-1, keepdims=True),
                       x.shape[-1], EPS)
    return (x - m) * r


def _lhs7(a11, a12, a21, a22):
    return a11 + a22, a21 + a22, a11, a22, a11 + a12, a21 - a11, a12 - a22


def _words(ref, *idx):
    return ref.bitcast(U32)[idx]


def _ld(ref, *idx):
    return pltpu.bitcast(_words(ref, *idx), BF16)


def _phase(words, odd):
    return pltpu.bitcast(words & np.uint32(0xFFFF0000) if odd else words << 16, F32)


def _nn(a, b):
    return jnp.dot(a, b, preferred_element_type=F32)


def _nt(a, b):
    return lax.dot_general(a, b, (((1,), (1,)), ((), ())), preferred_element_type=F32)


def _ds(start, size, align):
    return pl.ds(start if isinstance(start, int) else pl.multiple_of(start, align), size)


def _tile(x, j, n=1):
    return x[:, 128 * j:128 * (j + n)]


def _add(xs):
    return functools.reduce(lambda x, y: x + y, xs)


def _kernel(q_h, k_h, v_h, sh_h, sk_h, sd_h, wi_h, ws_h, b_h, wo_h, c_h, wm_h, o_h,
            q_v, k_v, v_v, sh_v, sk_v, sd_v, wi_v, ws_v, b_v, wo_v, c_v, wm_v, vf_v,
            au0_v, au1_v, fa_v, fb_v, ya_v, yb_v, bm0_v, bp0_v, bm1_v, bp1_v,
            y_v, x1_v, h0_v, z1_v, z2_v, wt_v, wr_v, bf_v, o_v, tie_v, zero_s,
            sems, *lists):
    au_v, zf_v, sum_v, h_v = (au0_v, au1_v), lists[:16], lists[16:32], (lists[32:41], lists[41:])
    copies = {}

    def start(group, sem, *pairs):
        copies[group] = [pltpu.make_async_copy(src, dst, sems.at[sem]) for src, dst in pairs]
        for cp in copies[group]:
            cp.start()

    def wait(*groups):
        for group in groups:
            for cp in copies[group]:
                cp.wait()

    def conv_inputs(cb, a):
        rows, lanes, sem = _ds(a * CH, CH, CH), pl.ds(cb * 128, 128), sems.at[cb % 3 * NA + a]
        return (pltpu.make_async_copy(k_h.at[rows, lanes], k_v.at[cb, _ds(PAD + a * CH, CH, PAD)], sem),
                pltpu.make_async_copy(v_h.at[rows, lanes], v_v.at[cb, rows], sem),
                pltpu.make_async_copy(sk_h.at[lanes, rows], sk_v.at[cb, a], sem))

    def fetch(stage):
        rows = lambda r, n: (q_h.at[pl.ds(r, n)], q_v.at[pl.ds(r, n)])
        if stage == 0:
            start("taps", 12, (sh_h, sh_v), (sd_h, sd_v))
        if stage < 3:
            for a in range(NA):
                for cp in conv_inputs(stage, a):
                    cp.start()
        if stage == 4:
            later = []
            for a in range(NA):
                (k3, v3, f3), (k4, v4, f4) = conv_inputs(3, a), conv_inputs(4, a)
                later.append(f4)
                for cp in (k3, k4, v3, v4, f3):
                    cp.start()
            for cp in later:
                cp.start()
        if stage == NCB:
            start("mod", 8, (c_h, c_v), (wm_h.at[:, pl.ds(0, 5 * D)], wm_v.at[:, pl.ds(0, 5 * D)]), rows(0, H))
            start("rows", 11, rows(H, HD - H))
            start("gate", 9, (wi_h.at[pl.ds(FH, FH)], wi_v.at[pl.ds(0, FH)]), rows(HD, RB - HD))
            start("value", 10, (wi_h.at[pl.ds(0, FH)], wi_v.at[pl.ds(FH, FH)]), rows(RB, 2 * RB))
        if stage == NCB + 2:
            start("out", 0, rows(3 * RB, RB), (wm_h.at[:, pl.ds(5 * D, D)], wm_v.at[:, pl.ds(5 * D, D)]),
                  (b_h, b_v), (wo_h, wo_v.at[pl.ds(0, FH)]))
            start("mix", 1, *[(ws_h.at[:, pl.ds(128 * j, 128)], ws_v.at[j]) for j in range(S // 128)])

    fetch(0)
    fetch(1)
    for ref in (fb_v, ya_v, tie_v):
        ref[...] = jnp.zeros(ref.shape, ref.dtype)
    k_v[:, pl.ds(0, PAD), :] = jnp.zeros((NCB, PAD, 128), BF16)
    wo_v[pl.ds(FH, 256 * KO + 128 - FH), :] = jnp.zeros((256 * KO + 128 - FH, D), BF16)
    row, col = (lax.broadcasted_iota(jnp.int32, (128, 128), d) for d in (0, 1))
    n = (col >> 5) * 16 + (col & 7) * 2 + ((col >> 4) & 1)
    order = jnp.where(row == (n >> 3) * 16 + (col & 8) + (n & 7), 1.0, 0.0).astype(BF16)
    mats = _dft_mats()
    back = _nt(order, jnp.concatenate(mats, axis=0))
    for b in range(8):
        vf_v[b] = mats[b]
        vf_v[8 + b] = _tile(back, b).astype(BF16)
    zero_s[0] = 0
    row8 = lax.broadcasted_iota(jnp.int32, (8, 128), 0)

    def tie(after, x):
        if after is None:
            return x
        never = jnp.concatenate([tie_v[...]] * (x.shape[0] // 8), axis=0) != 0
        return jnp.where(never, after, x)

    def put(cb, slot, g, res):
        for b in range(8):
            au_v[cb % 2][b, slot, pl.ds(16 * g, 16), :] = jnp.concatenate(res[b], axis=0).astype(BF16)

    def split_filter(cb, a, after):
        kt = pltpu.bitcast(sk_v[cb, a].T, U32)
        for g in range(N2 // 8):
            u = [_phase(kt[j * N2 // 2 + g // 2 * 8:j * N2 // 2 + g // 2 * 8 + 8], g % 2) for j in range(N1)]
            if g == 0:
                u[0] = u[0] + jnp.where(row8 + a == 0, sd_v[...].astype(F32)[cb:cb + 1], 0.0)
            u[:4] = [tie(after(g), x) for x in u[:4]]
            put(cb, NA + a, g, _outer_fwd(u))

    def split_signal(cb, a, after):
        taps = [jnp.broadcast_to(sh_v[j:j + 1, pl.ds(cb * 128, 128)].astype(F32), (8, 128))
                for j in range(TAPS)]
        base = a * (CH // 2) if isinstance(a, int) else pl.multiple_of(a * (CH // 2), CH // 2)
        for g in range(N2 // 8):
            w = [tie(after(g), t) for t in taps]
            u = []
            for j in range(N1):
                r = base + j * N2 // 2 + g // 2 * 8
                lag = [_phase(_words(k_v, cb, pl.ds(r + PAD // 2 + (g % 2 - t) // 2, 8)), (g % 2 - t) % 2)
                       for t in range(TAPS)]
                u.append(_add([x * wt for x, wt in zip(lag, w)]) * _phase(_words(v_v, cb, pl.ds(r, 8)), g % 2))
            put(cb, a, g, _outer_fwd(u))

    def spectra(cb, b, half, f_ref):
        rhs = jnp.concatenate([_ld(au_v[cb % 2], b, half * NA + a) for a in range(NA)], axis=1)
        f = _nn(_ld(vf_v, b), rhs)
        for a in range(NA):
            f_ref[half * NA + a] = f[:, 128 * a:128 * a + 128]
        return f

    def product(f_ref, y_ref, plus, real_rows=None):
        for g in range(8):
            ur, ui, kr, ki = ([f_ref[o + a, pl.ds(16 * g + 8 * c, 8), :] for a in range(NA)]
                              for o in (0, NA) for c in (0, 1))
            kr, ki = ([k[0]] + [k[a] + k[a - 1] if plus else k[a] - k[a - 1] for a in range(1, NA)]
                      for k in (kr, ki))
            for a in range(NA):
                yi = _add([kr[j] * ui[a - j] + ki[j] * ur[a - j] for j in range(a + 1)])
                if real_rows is not None and g == 0:
                    rr = _add([kr[j] * ur[a - j] for j in range(a + 1)])
                    ii = _add([ki[j] * ui[a - j] for j in range(a + 1)])
                    yr = jnp.where(real_rows, 0.5 * rr, rr - ii)
                    yi = jnp.where(real_rows, 0.5 * ii, yi)
                else:
                    yr = _add([kr[j] * ur[a - j] - ki[j] * ui[a - j] for j in range(a + 1)])
                y_ref[a, pl.ds(16 * g, 16), :] = jnp.concatenate([yr, yi], axis=0).astype(BF16)

    def residues(y_ref, b, dst):
        r = _nn(_ld(vf_v, 8 + b), jnp.concatenate([_ld(y_ref, a) for a in range(NA)], axis=1))
        for a in range(NA):
            dst[a] = r[:, 128 * a:128 * a + 128]
        return r

    def stash(t):
        return ((bm0_v.at[t], bp0_v.at[t]) if t < 16 else (bm1_v.at[t - 16], bp1_v.at[t - 16]))

    def merge(cb, a, after=lambda g: None):
        src = [stash(1 + 4 * cb + b)[s] for s in (0, 1) for b in range(4)]
        for g in range(N2 // 8):
            res = [[ref[a, pl.ds(16 * g + 8 * c, 8), :] for c in (0, 1)] for ref in src]
            res[0] = [tie(after(g), x) for x in res[0]]
            res[1] = [tie(after(g), x) for x in res[1]]
            for j, y in enumerate(_outer_inv(res)):
                y_v[cb, _ds(a * CH + j * N2 + 8 * g, 8, 8), :] = y

    def transform(cb, a, dst, active=True):
        pa = (a + 3) % 4
        res = []
        if active:
            res += [spectra(cb, a, 1, fa_v), spectra(cb, a, 0, fa_v)]
        product(fb_v, yb_v, True, row8 + (3 - pa) == 0)
        res.append(residues(ya_v, pa, dst[0]))
        if active:
            res += [spectra(cb, 4 + a, 1, fb_v), spectra(cb, 4 + a, 0, fb_v)]
            product(fa_v, ya_v, False)
        res.append(residues(yb_v, 4 + pa, dst[1]))
        return res

    def conv_step(cb, a):
        if cb < NCB:
            for cp in conv_inputs(cb, a):
                cp.wait()
        if cb:
            done = transform(cb - 1, a, (bm0_v.at[4 * cb - 4 + a], bp0_v.at[4 * cb - 4 + a])
                             if cb < NCB else (bm1_v.at[a], bp1_v.at[a]))
        at = lambda p: done[p // 8][16 * (p % 8):16 * (p % 8) + 8, 0:128] if cb and p >= 0 else None
        if cb < NCB:
            split_signal(cb, a, lambda g: at(TU[g]))
            split_filter(cb, a, lambda g: at(TK[g]))
        else:
            for c in range(3):
                merge(c, a, lambda g: at(TI[8 * c + g]))

    wait("taps")
    for cb in range(NCB + 1):
        fetch(cb + 2)
        pl.loop(0, NA)(functools.partial(conv_step, cb))

    wait("mod")
    transform(NCB, 0, stash(20), active=False)
    cc = c_v[...].astype(F32)
    sc = jnp.broadcast_to(cc / (1.0 + jnp.exp(-cc)), (16, D)).astype(BF16)
    mod = _nn(sc, jnp.concatenate([wm_v[:, pl.ds(i * D, D)] for i in (0, 1, 2, 4, 3)], axis=1))[0:8]
    sa, ca, ga, cb_, sb = (mod[:, i * D:(i + 1) * D] for i in range(5))
    m1, m0 = ga * (1.0 + ca), ga * sa
    n1, n0 = _GA * (1.0 + cb_), _GA * sb
    zero = zero_s[0]
    for n, cb in enumerate((3, 4)):
        merge(cb, zero, lambda g: _tile(mod, (8 * n + g) * 3 // 4))

    TB = RB // 128

    def hidden(r0, after=(None, None)):
        out = []
        for r, a in zip((r0, r0 + 8), after):
            rows = pl.ds(r, 8)
            x = q_v[rows, :].astype(F32)
            x = jnp.concatenate([tie(a, x[:, :128]), x[:, 128:]], axis=1)
            x1 = x + (_ln_rows(x) * m1 + m0) * jnp.concatenate([y_v[j, rows, :] for j in range(NCB)], axis=1)
            x1_v[rows, :] = x1
            out.append(_ln_rows(x1) * n1 + n0)
        return jnp.concatenate(out, axis=0)

    def keep_gate(tile, z):
        zf_v[tile][pl.ds(zero, FH), :] = z

    def moments(tile, after):
        z, acc = zf_v[tile], sum_v[tile]
        s1 = s2 = None
        for n, f in enumerate(range(0, FH, SU)):
            for r in range(f, f + SU, 8):
                d = tie(after(n)[:8] if r == f else None, z[pl.ds(r, 8), :])
                s1, s2 = (d, d * d) if s1 is None else (s1 + d, s2 + d * d)
            acc[pl.ds(16 * n + zero, 16), :] = jnp.concatenate([s1, s2], axis=0)
        s1, s2 = (jnp.sum(acc[pl.ds(16 * n + r, 8), :], axis=0, keepdims=True) for r in (0, 8))
        stats[tile] = [jnp.broadcast_to(t, (8, 128)) for t in _norm_stats(s1, s2, FH, EPS * (2 * _GA) ** 2)]

    def norm_gate(pair, after):
        for n in range(FM // 8):
            means = [tie(after(n)[:8], stats[2 * pair + c][0]) for c in (0, 1)]
            quad = [(zf_v[2 * pair + c][pl.ds(r + 8 * n, 8), :] - means[c]) * stats[2 * pair + c][1]
                    for r in (0, FM) for c in (0, 1)]
            for k, a in enumerate(_lhs7(*quad)):
                z2_v[k, pair, pl.ds(8 * n, 8), :] = a

    def prepare(i, c, after):
        def put(k, n, x):
            for j in range(x.shape[1] // 128):
                h_v[i % 2][k][j, pl.ds(16 * n + zero, 16), :] = _tile(x, j).astype(BF16)

        for n in range(H // 16):
            h = hidden(i * RB + c * H + 16 * n, (after(2 * n)[:8], after(2 * n + 1)[:8]))
            top, bot = _tile(h, 0, 2), _tile(h, 2, 2)
            put(7 + c, n, _tile(h, 4))
            if c:
                half[n] = top, bot
                put(2, n, top - bot)
                put(4, n, bot)
            else:
                put(1, n, top)
                put(3, n, bot - top)
                put(0, n, top + half[n][1])
                put(5, n, top + half[n][0])
                put(6, n, bot + half[n][1])

    def turn_out(after):
        for n in range((2 * KO + 1) * NCB):
            j, t = divmod(n, NCB)
            w = _words(wo_v, pl.ds(64 * j, 64), pl.ds(128 * t, 128))
            w = jnp.concatenate([tie(pltpu.bitcast(after(n)[:8], U32), w[:8]), w[8:]], axis=0)
            wr_v[j, pl.ds(128 * t + zero, 128), :] = pltpu.bitcast(w, BF16).T

    def split_out(after):
        for n in range(KO * DM // 16):
            j, r = divmod(16 * n, DM)
            quad = [wr_v[j + KO * c, pl.ds(r + DM * b, 16), :].astype(F32) for b in (0, 1) for c in (0, 1)]
            for k, a in enumerate(_lhs7(tie(after(n), quad[0]), quad[1], quad[2], tie(after(n), quad[3]))):
                wt_v[k, j, pl.ds(r, 16), :] = a.astype(BF16)

    def side_jobs(plan, at):
        for job in plan.split(","):
            if job:
                kind, (n, *spans) = job[0], (int(x) for x in job[1:].split(":"))
                total = {"s": FH // SU, "n": FM // 8, "h": H // 8, "m": N2 // 8,
                         "t": (2 * KO + 1) * NCB, "o": KO * DM // 16}[kind]
                slots = [p for lo, hi in zip(spans[::2], spans[1::2]) for p in range(lo, hi)]
                after = lambda k: at(slots[k * len(slots) // total])
                if kind == "s":
                    moments(n, after)
                elif kind == "m":
                    merge(n // NA, n % NA + zero, lambda k: after(k)[:8])
                elif kind in "to":
                    (turn_out if kind == "t" else split_out)(after)
                elif kind == "n":
                    norm_gate(n, after)
                else:
                    prepare(n // 2, n % 2, after)

    def rows_of(z):
        per = z.shape[0] // 16
        return lambda p: z[16 * (p % per):16 * (p % per) + 16, 128 * (p // per):128 * (p // per) + 128]

    def project(i):
        def prod(*pairs):
            right = [_ld(h_v[i % 2][k], j) for _, k in pairs for j in range(2 if k < 7 else 1)]
            return _nt(jnp.concatenate([x for k, _ in pairs for x in left[k]], axis=1),
                       jnp.concatenate(right, axis=1))

        s5, s3, r12, s4, s1 = prod((4, 4)), prod((2, 2)), prod((7, 8)), prod((3, 3)), prod((0, 0))
        s7, s2, r21, s6 = prod((6, 6), (7, 7)), prod((1, 1)), prod((8, 7)), prod((5, 5), (8, 8))
        gate = [((s4 - s5) + s1) + s7, (s5 + s3) + r12]
        value = [(s4 + s2) + r21, ((s3 + s1) - s2) + s6]
        for t in range(TB):
            keep_gate(i * TB + t, _gelu_scaled(_tile(gate[t // 2], t % 2)))
            z1_v[i * TB + t] = _tile(value[t // 2], t % 2).astype(BF16)
        rounds = (s5, s3, gate[1], _tile(s4, 1), _tile(s1, 1), gate[0], s2, value[0], _tile(value[1], 1))
        return lambda p: rounds[p // (FH // 16)][16 * (p % (FH // 16)):16 * (p % (FH // 16)) + 16, 0:128]

    def first(f0, r0, n, k0, k1):
        h = jnp.concatenate([_ld(h0_v, j, pl.ds(r0 // 2, n // 2)) for j in range(k0, k1)], axis=1)
        return _nt(wi_v[pl.ds(f0, FH), pl.ds(128 * k0, 128 * (k1 - k0))], h)

    def keep_first(r, h):
        for j in range(NCB):
            h0_v[j, pl.ds(r, 16), :] = _tile(h, j).astype(BF16)

    stats, half = {}, {}
    for r in range(0, HD, 16):
        if r == H:
            wait("rows")
        keep_first(r, hidden(r))
    wait("gate")
    zero = pl.multiple_of(zero_s[0], 16)
    head = first(0, 0, H, 0, 2)
    z = _gelu_scaled(head + first(0, 0, H, 2, NCB))
    third = _gelu_scaled(first(0, H, 128, 0, NCB))
    at = rows_of(jnp.concatenate([_tile(head, 0), z], axis=1))
    for n in range((RB - HD) // 16):
        keep_first(HD + 16 * n, hidden(HD + 16 * n, [at(E0 + (2 * n + k) * ES // 8)[:8] for k in (0, 1)]))
    z = jnp.concatenate([z, third, _gelu_scaled(first(0, H + 128, 128, 0, NCB))], axis=1)
    for t in range(TB):
        keep_gate(t, _tile(z, t))
    side_jobs(NJ[0], rows_of(z))
    wait("value")
    head = first(FH, 0, RB, NCB - 1, NCB)
    z = head + first(FH, 0, RB, 0, NCB - 1)
    for t in range(TB):
        z1_v[t] = _tile(z, t).astype(BF16)
    side_jobs(NJ[1], rows_of(jnp.concatenate([_tile(head, 0), z], axis=1)))
    sums = [_lhs7(*(wi_v[pl.ds(FH * r, FH), pl.ds(256 * c + 128 * j, 128)].astype(F32)
                    for r in (0, 1) for c in (0, 1))) for j in (0, 1)]
    left = ([[s[k].astype(BF16) for s in sums] for k in range(7)]
            + [[wi_v[pl.ds(FH * r, FH), pl.ds(512, 128)]] for r in (0, 1)])
    for i in range(1, NB):
        if i == 2:
            wait("out")
        side_jobs(NJ[i + 1], project(i))
    gb = _nn(sc, wm_v[:, pl.ds(5 * D, D)]) * (0.5 / _GA)
    bf_v[...] = b_v[...].astype(F32)

    wait("mix")

    def mix(i):
        def w(c, r):
            return [_ld(ws_v, 2 * j + c, _ds((i * RB + r * H) // 2, H // 2, H // 2))
                    for j in range(S // 256)]

        def comb(x, y, sign):
            return [(jnp.add if sign > 0 else jnp.subtract)(a.astype(F32), b.astype(F32)) for a, b in zip(x, y)]

        def prod(n, rhs):
            def left(k):
                def part(r, c, rows):
                    return jnp.concatenate([z2_v[n, 2 * j + c, pl.ds(FT * r, rows), :] for j in range(NB)], axis=1)

                def both(c, op):
                    top = part(0, c, FT)
                    return jnp.concatenate([op(top[:FB], part(1, 1, FB)), top[FB:]], axis=0)

                return (lambda: both(0, jnp.add), lambda: part(1, 0, FB) + part(1, 1, FB),
                        lambda: part(0, 0, FT), lambda: part(1, 1, FB),
                        lambda: part(0, 0, FT) + part(0, 1, FT), lambda: part(1, 0, FB) - part(0, 0, FB),
                        lambda: both(1, jnp.subtract))[k]().astype(BF16)

            b11, b12, b21, b22 = (
                jnp.concatenate([rhs[2 * j + c][128 * r:128 * r + 128] for j in range(NB)], axis=1)
                for c in (0, 1) for r in (0, 1))
            m = lambda k, x: _nt(left(k), x.astype(BF16))
            m2, m5 = m(1, b11), m(4, b22)
            b11, b12, b21, b22 = (x.astype(F32) for x in (b11, b12, b21, b22))
            m4 = m(3, b21 - b11)
            m1, m7, m3, m6 = m(0, b11 + b22), m(6, b21 + b22), m(2, b12 - b22), m(5, b11 + b12)
            c11 = jnp.concatenate([m4 - m5[:FB], -m5[FB:]], axis=0) + m1 + m7
            c22 = (m1[:FB] - m2) + m3[:FB] + m6
            return jnp.concatenate([jnp.concatenate([c11, m5 + m3], axis=1),
                                    jnp.concatenate([m2 + m4, c22], axis=1)], axis=0)

        def gate(r, c, g):
            tiles = [i * TB + c * (H // 128) + t for t in range(H // 128)]
            bias = jnp.concatenate([bf_v[pl.ds(j, 1), :] for j in tiles], axis=1)
            z1 = jnp.concatenate([z1_v[j, pl.ds(FM * r, FM), :] for j in tiles], axis=1).astype(F32)
            return _gelu_scaled(z1) * (g + bias)

        s2 = prod(1, w(0, 0))
        s5 = prod(4, w(1, 1))
        s4 = prod(3, comb(w(1, 0), w(0, 0), -1))
        p21 = gate(1, 0, s2 + s4)
        d11 = s4 - s5
        s1 = prod(0, comb(w(0, 0), w(1, 1), 1))
        d11, d22 = d11 + s1, s1 - s2
        p11 = gate(0, 0, d11 + prod(6, comb(w(1, 0), w(1, 1), 1)))
        s3 = prod(2, comb(w(0, 1), w(1, 1), -1))
        p12 = gate(0, 1, s3 + s5)
        p22 = gate(1, 1, (d22 + s3) + prod(5, comb(w(0, 0), w(0, 1), 1)))
        return [jnp.concatenate(p, axis=0) for p in ((p11, p21), (p12, p22))]

    def flush(k):
        rows = _ds(k * H, H, H)
        return [pltpu.make_async_copy(o_v.at[j, rows], o_h.at[rows, pl.ds(128 * j, 128)], sems.at[2])
                for j in range(NCB)]

    def finish(r0, tile):
        for cols in (range(DM // 128), range(DM // 128, NCB)):
            for t, j in ((t, j) for t in range(H // 128) for j in cols):
                at = _ds(r0 + 128 * t, 128, 128), pl.ds(128 * j, 128)
                o_v[j, at[0], :] = (x1_v[at] + jnp.concatenate([_tile(gb, j)] * 8, axis=0)
                           * tile(t, j).T.astype(F32)).astype(BF16)

    def mix_step(i):
        p = mix(i)
        b11, b12, b21, b22 = (p[c][128 * KO * r:128 * KO * (r + 1)] for r in (0, 1) for c in (0, 1))

        def prod(n, rhs):
            return _nn(jnp.concatenate([_ld(wt_v, n, j) for j in range(KO)], axis=1), rhs.astype(BF16))

        def rest(c):
            tail = jnp.concatenate([p[c][256 * KO:], jnp.zeros((128 + 256 * KO - FH, H), F32)], axis=0)
            return _nn(_ld(wr_v, 2 * KO), tail.astype(BF16))

        r0 = rest(0)
        s2 = prod(1, b11)
        s4 = prod(3, b21 - b11)
        s5 = prod(4, b22)
        s1 = prod(0, b11 + b22)
        s7 = prod(6, b21 + b22)
        ot = jnp.concatenate([r0[:DM] + s4 - s5 + s1 + s7, r0[DM:] + s2 + s4], axis=0)
        finish(i * RB, lambda t, j: _tile(ot, t)[128 * j:128 * j + 128].astype(BF16))
        for cp in flush(2 * i):
            cp.start()
        spot = 0, _ds(i * RB + H, 16, 16)
        o_v[spot] = jnp.zeros((16, 128), BF16)
        pin = o_v[0, _ds(i * RB + H + zero, 16, 16)].astype(F32)
        r1 = rest(1)
        s3 = prod(2, b12 - b22)
        b = b11 + b12
        b = jnp.concatenate([b[:-16], jnp.concatenate([b[-16:, :128], tie(pin, b[-16:, 128:])], axis=1)], axis=0)
        s6 = prod(5, b)
        ot = jnp.concatenate([r1[:DM] + s5 + s3, (s1 - s2) + r1[DM:] + s3 + s6], axis=0)
        finish(i * RB + H, lambda t, j: _tile(ot, t)[128 * j:128 * j + 128].astype(BF16))
        for cp in flush(2 * i + 1):
            cp.start()

    zero = pl.multiple_of(zero_s[0], 16)
    zero = zero_s[0]
    pl.loop(0, NB)(mix_step)
    for k in range(S // H):
        for cp in flush(k):
            cp.wait()


@jax.jit
def pallas_adaLN_cond__ssm_conv_h3__mixer_gmlp__prompt_kernel(
    A_q, A_k, A_v, A_shift_k, A_ssm_k, A_ssm_D, B_x, B_w_in, B_w_sp, B_b_sp, B_w_out, c, w_mod,
):
    del B_x
    vm = pltpu.VMEM
    tile = (128, 128)
    scratch = [
        vm((S, D), BF16), vm((NCB, PAD + S, 128), BF16), vm((NCB, S, 128), BF16), vm((TAPS, D), BF16),
        vm((NCB, NA, 128, CH), BF16), vm((NCB, 128), BF16), vm((2 * FH, D), BF16),
        vm((S // 128, S, 128), BF16), vm((S // 128, 128), BF16), vm((256 * KO + 128, D), BF16), vm((1, D), BF16),
        vm((D, 6 * D), BF16), vm((16, *tile), BF16),
        vm((8, 2 * NA, *tile), BF16), vm((8, 2 * NA, *tile), BF16),
        vm((2 * NA, *tile), F32), vm((2 * NA, *tile), F32), vm((NA, *tile), BF16), vm((NA, *tile), BF16),
        vm((16, NA, *tile), F32), vm((16, NA, *tile), F32), vm((5, NA, *tile), F32), vm((5, NA, *tile), F32),
        vm((NCB, S, 128), F32), vm((S, D), F32), vm((NCB, RB, 128), BF16),
        vm((S // 128, FH, 128), BF16), vm((7, S // 256, FM, 128), F32),
        vm((7, KO, DM, 128), BF16), vm((2 * KO + 1, D, 128), BF16), vm((S // 128, 128), F32),
        vm((NCB, S, 128), BF16), vm((8, 128), jnp.int32), pltpu.SMEM((1,), jnp.int32),
        pltpu.SemaphoreType.DMA((13,)),
    ]
    scratch += [vm((FH, 128), F32)] * 16 + [vm((FH // SU * 16, 128), F32)] * 16
    scratch += ([vm((2, H, 128), BF16)] * 7 + [vm((1, H, 128), BF16)] * 2) * 2
    out = pl.pallas_call(
        _kernel,
        out_shape=jax.ShapeDtypeStruct((S, D), BF16),
        in_specs=[pl.BlockSpec(memory_space=pltpu.HBM)] * 12,
        out_specs=pl.BlockSpec(memory_space=pltpu.HBM),
        scratch_shapes=scratch,
        compiler_params=pltpu.CompilerParams(vmem_limit_bytes=110 * 1024 * 1024),
    )(A_q.reshape(S, D), A_k.reshape(S, D), A_v.reshape(S, D), A_shift_k.T, A_ssm_k,
      A_ssm_D.reshape(NCB, 128), B_w_in.T, B_w_sp, B_b_sp.reshape(S // 128, 128), B_w_out, c, w_mod)
    return out.reshape(1, S, D)
```
